```python
import jax
import jax.numpy as jnp

def _softmax(x, axis=-1):
    return jax.nn.softmax(x, axis=axis)

def _gelu(x):
    return jax.nn.gelu(x, approximate=True)

def _silu(x):
    return jax.nn.silu(x)

def _sigmoid(x):
    return jax.nn.sigmoid(x)

def _layernorm(x, axis=-1, eps=1e-05):
    m = jnp.mean(x, axis=axis, keepdims=True)
    v = jnp.var(x, axis=axis, keepdims=True)
    return (x - m) / jnp.sqrt(v + eps)

def _scatter_add(tgt, idx, src, axis=0):
    return tgt.at[idx].add(src)

def _segment_sum(src, seg, n):
    return jax.ops.segment_sum(src, seg, n)

class _Rng:

    def __init__(self, key):
        self._k = key

    def _next(self):
        self._k, sub = jax.random.split(self._k)
        return sub

    def normal(self, shape):
        return jax.random.normal(self._next(), shape, dtype=jnp.bfloat16)

    def randint(self, lo, hi, shape):
        return jax.random.randint(self._next(), shape, lo, hi, dtype=jnp.int32)

    def uniform(self, shape, lo=0.0, hi=1.0):
        return jax.random.uniform(self._next(), shape, jnp.bfloat16, lo, hi)

    def permutation(self, n):
        return jax.random.permutation(self._next(), n)
kernel_name = 'adaLN_cond__ssm_conv_h3__glu_gated_reglu__prompt'

def setup_inputs():
    _rng = _Rng(jax.random.key(int.from_bytes(__import__("os").urandom(4), "little")))
    _w = lambda a: (lambda t: t.astype(jnp.bfloat16) if jnp.issubdtype(t.dtype, jnp.floating) else t)(jnp.asarray(a))

    def _A_setup():
        B, S, D = (1, 2048, 640)
        ks = 4
        return {'q': _w((lambda *s: _rng.normal(s) * 0.05)(B, S, D)), 'k': _w((lambda *s: _rng.normal(s) * 0.05)(B, S, D)), 'v': _w((lambda *s: _rng.normal(s) * 0.05)(B, S, D)), 'shift_k': _w((lambda *s: _rng.normal(s) * 0.05)(D, ks) * 0.5), 'ssm_k': _w((lambda *s: _rng.normal(s) * 0.05)(D, S) * (1.0 / S ** 0.5)), 'ssm_D': _w((lambda *s: _rng.normal(s) * 0.05)(D))}
    _A_in = _A_setup()

    def _B_setup():
        B, S, D, F = (1, 2048, 640, 1536)
        return {'x': _w((lambda *s: _rng.normal(s) * 0.05)(B, S, D)), 'W_gate': _w((lambda *s: _rng.normal(s) * 0.05)(D, F) * (2.0 / D) ** 0.5), 'W_up': _w((lambda *s: _rng.normal(s) * 0.05)(D, F) * (2.0 / D) ** 0.5), 'W_down': _w((lambda *s: _rng.normal(s) * 0.05)(F, D) * (1.0 / F) ** 0.5)}
    _B_in = _B_setup()
    return {'A_q': _A_in['q'], 'A_k': _A_in['k'], 'A_v': _A_in['v'], 'A_shift_k': _A_in['shift_k'], 'A_ssm_k': _A_in['ssm_k'], 'A_ssm_D': _A_in['ssm_D'], 'B_x': _B_in['x'], 'B_W_gate': _B_in['W_gate'], 'B_W_up': _B_in['W_up'], 'B_W_down': _B_in['W_down'], 'c': _w((lambda *s: _rng.normal(s) * 0.05)(1, 640)), 'w_mod': _w((lambda *s: _rng.normal(s) * 0.05)(640, 6 * 640) * 640 ** (-0.5))}

def reference(A_q, A_k, A_v, A_shift_k, A_ssm_k, A_ssm_D, B_x, B_W_gate, B_W_up, B_W_down, c, w_mod):

    def _A_ref(q, k, v, shift_k, ssm_k, ssm_D):
        B, S, D = q.shape
        ks = shift_k.shape[-1]
        k_pad = jnp.pad(k, ((0, 0), (ks - 1, 0), (0, 0)))
        k_shift = jnp.zeros_like(k)
        for t in range(ks):
            k_shift = k_shift + k_pad[:, t:t + S, :] * shift_k[:, ks - 1 - t][None, None, :]
        kv = k_shift * v
        L = 2 * S
        kv_pad = jnp.pad(kv, ((0, 0), (0, S), (0, 0)))
        kf_pad = jnp.pad(ssm_k, ((0, 0), (0, S)))
        kv_f = (lambda x, axes=(-2, -1): jnp.fft.rfft2(x.astype(jnp.float32), axes=axes))(kv_pad[:, None, :, :], axes=(1, 2))
        kf_f = (lambda x, axes=(-2, -1): jnp.fft.rfft2(x.astype(jnp.float32), axes=axes))(kf_pad[:, None, :], axes=(1, 2))
        kf_f = (lambda x, *d: x.transpose(*d))(kf_f, 1, 2, 0)
        y_f = kv_f * kf_f[None, :, :, :]
        y = (lambda x, s, axes=(-2, -1): jnp.fft.irfft2(x, s=s, axes=axes).astype(jnp.bfloat16))(y_f, (1, L), axes=(1, 2))[:, 0, :S, :]
        y = y + kv * ssm_D[None, None, :]
        return q * y

    def _B_ref(x, W_gate, W_up, W_down):
        gate = jnp.einsum('bsd,df->bsf', x, W_gate)
        up = jnp.einsum('bsd,df->bsf', x, W_up)
        gate = gate * (lambda x, dt: x.astype(dt))(gate > 0, gate.dtype)
        h = gate * up
        return jnp.einsum('bsf,fd->bsd', h, W_down)
    x = A_q
    mod = (_silu(c) @ w_mod).reshape(c.shape[0], 6, 1, -1)
    sa, ca, ga, sb, cb, gb = (mod[:, 0].copy(), mod[:, 1].copy(), mod[:, 2].copy(), mod[:, 3].copy(), mod[:, 4].copy(), mod[:, 5].copy())
    h = _layernorm(x, axis=-1) * (1 + ca) + sa
    x = x + ga * _A_ref(h, A_k, A_v, A_shift_k, A_ssm_k, A_ssm_D)
    h = _layernorm(x, axis=-1) * (1 + cb) + sb
    x = x + gb * _B_ref(h, B_W_gate, B_W_up, B_W_down)
    return x
```

```python
import functools, os
import numpy as np
import jax
import jax.numpy as jnp
from jax import lax
import jax.experimental.pallas as pl
import jax.experimental.pallas.tpu as pltpu

S, D, F = 2048, 640, 1536
BLK = 128
NB = S // BLK
TM = 256
NT = S // TM
NL = D // 128
EPS = 1e-5
f32 = jnp.float32
bf16 = jnp.bfloat16
u32 = jnp.uint32

LN_CH = int(os.environ.get("LN_CH", "8"))
KV_CH = int(os.environ.get("KV_CH", "1"))
FCH = [int(x) for x in os.environ.get("FCH", "256,256,256,256,256,256").split(",")]
SKIP = os.environ.get("SKIP", "")
FOFF = [sum(FCH[:i]) for i in range(len(FCH) + 1)]
NCH = len(FCH)
SEM_KVS0, SEM_KVS1, SEM_KVS2, SEM_M0, SEM_M1 = 0, 1, 2, 3, 4
SEM_W = 5
SEM_STEP = SEM_W + NCH
SEM_OUT = SEM_STEP + NT - 1
NSEM = SEM_OUT + 1
ZSLOT = NB


def _dft_mats():
    f = np.concatenate([np.arange(0, BLK, 2), np.arange(1, BLK, 2)]).astype(np.float64)
    n = np.arange(BLK, dtype=np.float64)
    ang = 2.0 * np.pi * np.outer(f + 0.5, n) / (2 * BLK)
    fm = np.concatenate([np.cos(ang), -np.sin(ang)], axis=0)
    gm = fm.T / BLK
    return fm.astype(np.float32), gm.astype(np.float32)


def _kernel(q_hbm, k_hbm, v_hbm, sk_hbm, ssmk_hbm, d_hbm, wg_hbm, wu_hbm, wd_hbm, c_hbm, wm_hbm,
            fm_hbm, gm_hbm, o_hbm,
            q_v, k_v, v_v, s_v, wm_v, wg_v, wu_v, wd_v, wgp, wup, wdp, o_v,
            sk_ref, d_ref, c_ref, fm_ref, gm_ref,
            u_ref, kk_ref, kprev_ref, kvb_ref, z_ref, y_ref, acc_ref, h2_ref, x1_ref, mod_ref, taps_ref,
            sems, zsem):

    def st(x):
        return isinstance(x, int)

    def rows(t, off=0, n=TM, al=8):
        r0 = t * TM + off
        return pl.ds(r0 if st(t) else pl.multiple_of(r0, al), n)

    def cp(src, dst, sem):
        return pltpu.make_async_copy(src, dst, sems.at[sem])

    def kvs(t, sem):
        rs = rows(t, al=TM)
        return [cp(k_hbm.at[rs, :], k_v.at[rs, :], sem), cp(v_hbm.at[rs, :], v_v.at[rs, :], sem),
                cp(ssmk_hbm.at[:, rs], s_v.at[:, rs], sem)]

    def qc(t, sem):
        rs = rows(t, al=TM)
        return [cp(q_hbm.at[rs, :], q_v.at[rs, :], sem)]

    def wmc(c0, c1, sem):
        cs = pl.ds(c0 * D, (c1 - c0) * D)
        return [cp(wm_hbm.at[:, cs], wm_v.at[:, cs], sem)]

    def wc(i):
        cs = pl.ds(FOFF[i], FCH[i])
        return [cp(wg_hbm.at[:, cs], wg_v.at[:, cs], SEM_W + i), cp(wu_hbm.at[:, cs], wu_v.at[:, cs], SEM_W + i),
                cp(wd_hbm.at[cs, :], wd_v.at[cs, :], SEM_W + i)]

    def step_group(s, with_kvs):
        return qc(s + 1, SEM_STEP + s) + (kvs(s + 3, SEM_STEP + s) if with_kvs else [])

    groups = {}
    groups[SEM_KVS0] = [cp(fm_hbm, fm_ref, SEM_KVS0), cp(sk_hbm, sk_ref, SEM_KVS0), cp(d_hbm, d_ref, SEM_KVS0),
                        cp(c_hbm, c_ref, SEM_KVS0), cp(gm_hbm, gm_ref, SEM_KVS0)] + kvs(0, SEM_KVS0)
    groups[SEM_KVS1] = kvs(1, SEM_KVS1)
    groups[SEM_KVS2] = kvs(2, SEM_KVS2)
    groups[SEM_M0] = qc(0, SEM_M0) + wmc(0, 3, SEM_M0)
    groups[SEM_M1] = wmc(3, 5, SEM_M1)
    for i in range(NCH):
        groups[SEM_W + i] = wc(i)
    groups[SEM_W + 1] = qc(1, SEM_W + 1) + groups[SEM_W + 1]
    groups[SEM_W + NCH - 1] = groups[SEM_W + NCH - 1] + wmc(5, 6, SEM_W + NCH - 1)
    groups[SEM_STEP] = kvs(3, SEM_STEP)
    for s in range(1, NT - 1):
        groups[SEM_STEP + s] = step_group(s, s + 3 < NT)
    for g in sorted(groups):
        for c_ in groups[g]:
            c_.start()

    def wait(g):
        for c_ in (groups[g] if st(g) else g):
            c_.wait()

    def out_copy(t):
        rs = rows(t, al=TM)
        return cp(o_v.at[rs, :], o_hbm.at[rs, :], SEM_OUT)

    z0 = pl.semaphore_read(zsem)
    pred = jnp.full((8, 128), z0, jnp.int32) != 0

    def gate(x, tok):
        return x if tok is None else jnp.where(pred, tok, x)

    def gate_first(x, tok):
        if tok is None:
            return x
        first = gate(x[0:8, 0:128], tok)
        return jnp.concatenate([first, x[0:8, 128:]], axis=1)

    def fold(*xs):
        parts = []
        for x in xs:
            if x is None:
                continue
            parts += [x[i:i + 8, j:j + 128] for i in range(0, x.shape[0], 8) for j in range(0, x.shape[1], 128)]
        if not parts:
            return None
        while len(parts) > 1:
            parts = [jnp.maximum(parts[i], parts[i + 1]) if i + 1 < len(parts) else parts[i] for i in range(0, len(parts), 2)]
        return parts[0]

    def rep(w):
        return jnp.tile(w, (TM // 8, 1))

    rowid = lax.broadcasted_iota(jnp.int32, (8, 128), 0)
    masks = [None] + [rowid < m for m in range(1, 4)]

    def kv_stage(t, ch, tok=None):
        toks = [tok] * KV_CH
        n = 0
        for (l0, l1) in [(0, 2), (2, 4), (4, 5)]:
            ls = slice(l0 * 128, l1 * 128)
            prev = None
            if not (st(t) and t == 0):
                pk = k_v[rows(t, -8, 8), ls].astype(f32)
                prev = [[None] + [pltpu.roll(pk[:, i * 128:(i + 1) * 128], m, 0) for m in range(1, 4)] for i in range(l1 - l0)]
            for g in range(TM // 8):
                rs = rows(t, 8 * g, 8)
                kf = k_v[rs, ls].astype(f32)
                vf = v_v[rs, ls].astype(f32)
                cur = []
                res = []
                for i in range(l1 - l0):
                    li = slice((l0 + i) * 128, (l0 + i + 1) * 128)
                    k0 = kf[:, i * 128:(i + 1) * 128]
                    if ch:
                        k0 = gate(k0, toks[n % KV_CH])
                    rots = [None] + [pltpu.roll(k0, m, 0) for m in range(1, 4)]
                    ks = k0 * taps_ref[0, :, li]
                    for m in range(1, 4):
                        sh = jnp.where(masks[m], prev[i][m] if prev is not None else 0.0, rots[m])
                        ks = ks + sh * taps_ref[m, :, li]
                    res.append(ks * vf[:, i * 128:(i + 1) * 128])
                    cur.append(rots)
                prev = cur
                kvb = (res[0] if len(res) == 1 else jnp.concatenate(res, axis=1)).astype(bf16)
                kvb_ref[8 * g:8 * g + 8, ls] = kvb
                if ch:
                    toks[n % KV_CH] = fold(*res)
                n += 1
        return fold(*toks) if ch else None

    def dft_u(t, b):
        a = 2 * t + b
        u = jnp.dot(fm_ref[...], kvb_ref[b * BLK:(b + 1) * BLK, :], preferred_element_type=f32)
        ur, ui = u[:BLK], u[BLK:]
        u_ref[a, 0:BLK] = ur + ui
        u_ref[a, BLK:2 * BLK] = ur
        u_ref[a, 2 * BLK:3 * BLK] = ui

    def dft_k(t, b):
        H = BLK // 2
        a = 2 * t + b
        kraw = lax.dot_general(fm_ref[...], s_v[:, rows(t, b * BLK, BLK, al=BLK)], (((1,), (1,)), ((), ())),
                               preferred_element_type=f32)
        if st(a) and a == 0:
            cr = kraw[:BLK] + d_ref[...].astype(f32).reshape(1, D)
            di = kraw[BLK:]
        else:
            kp = kprev_ref[1 - b]
            cr = jnp.concatenate([kraw[0:H] - kp[BLK:BLK + H], kraw[H:BLK] + kp[BLK + H:]], axis=0)
            di = jnp.concatenate([kraw[BLK:BLK + H] + kp[0:H], kraw[BLK + H:] - kp[H:BLK]], axis=0)
        kprev_ref[b] = kraw
        kk_ref[a, 0:BLK] = cr
        kk_ref[a, BLK:2 * BLK] = di - cr
        kk_ref[a, 2 * BLK:3 * BLK] = cr + di

    def inv_b(t, b, ls=slice(None)):
        y_ref[t % 2, b * BLK:(b + 1) * BLK, ls] = jnp.dot(gm_ref[...], z_ref[b, :, ls], preferred_element_type=f32)

    def mac_stage(t, ch, tok=None, lanes=range(NL), nlag=None):
        g0 = g1 = tok
        if st(t):
            nlag = 2 * t + 2
            kidx = list(range(nlag))
            uidx = [2 * t + 1 - j for j in range(nlag)]
        else:
            kidx = [jnp.minimum(j, 2 * t + 1) for j in range(nlag)]
            uidx = [jnp.where(2 * t + 1 - j >= 0, 2 * t + 1 - j, ZSLOT) for j in range(nlag)]
        for l in lanes:
            ls = slice(l * 128, (l + 1) * 128)
            for r in range(BLK // 8):
                rr = slice(r * 8, r * 8 + 8)
                accs = []
                for p in range(3):
                    a0 = a1 = None
                    uc = None
                    pr = slice(p * BLK + r * 8, p * BLK + r * 8 + 8)
                    for j in range(nlag - 1, -1, -1):
                        kp = kk_ref[kidx[j], pr, ls]
                        un = u_ref[uidx[j], pr, ls]
                        t1 = kp * un
                        a1 = gate(t1, g1) if a1 is None else a1 + t1
                        if uc is not None:
                            t0 = kp * uc
                            a0 = gate(t0, g0) if a0 is None else a0 + t0
                        uc = un
                    accs.append((a0, a1))
                    if ch:
                        g0, g1 = a1, a0
                outs = []
                for b in range(2):
                    re = accs[0][b] - accs[2][b]
                    im = accs[0][b] + accs[1][b]
                    z_ref[b, rr, ls] = re.astype(bf16)
                    z_ref[b, BLK + r * 8:BLK + r * 8 + 8, ls] = im.astype(bf16)
                    outs.append(jnp.maximum(re, im))
                if ch:
                    g1, g0 = outs
        return jnp.maximum(g0, g1) if ch else None

    def fin_stage(t, par, tok=None, gs=range(TM // 8)):
        toks = [tok] * LN_CH
        for g in gs:
            rr = slice(8 * g, 8 * g + 8)
            x = gate_first(q_v[rows(t, 8 * g, 8), :].astype(f32), toks[g % LN_CH])
            m = jnp.mean(x, axis=-1, keepdims=True)
            xc = x - m
            var = jnp.mean(xc * xc, axis=-1, keepdims=True)
            hg = (xc * lax.rsqrt(var + EPS)) * mod_ref[1] + mod_ref[0]
            x1 = x + hg * y_ref[par, rr, :]
            m = jnp.mean(x1, axis=-1, keepdims=True)
            xc = x1 - m
            var = jnp.mean(xc * xc, axis=-1, keepdims=True)
            h2 = (xc * lax.rsqrt(var + EPS)) * mod_ref[4] + mod_ref[3]
            x1_ref[par, rr, :] = x1
            h2_ref[par, rr, :] = h2.astype(bf16)
            toks[g % LN_CH] = fold(h2)
        return fold(*toks)

    def fin_a(t):
        x = q_v[rows(t), :].astype(f32)
        m = jnp.mean(x, axis=-1, keepdims=True)
        xc = x - m
        var = jnp.mean(xc * xc, axis=-1, keepdims=True)
        hg = (xc * lax.rsqrt(var + EPS)) * rep(mod_ref[1]) + rep(mod_ref[0])
        x1 = x + hg * y_ref[t % 2]
        m = jnp.mean(x1, axis=-1, keepdims=True)
        xc = x1 - m
        var = jnp.mean(xc * xc, axis=-1, keepdims=True)
        x1_ref[t % 2] = x1
        acc_ref[...] = xc * lax.rsqrt(var + EPS)

    def fin_b(t):
        h2_ref[t % 2] = (acc_ref[...] * rep(mod_ref[4]) + rep(mod_ref[3])).astype(bf16)

    def ffn_stage(t, h2):
        g = jnp.dot(h2, pltpu.bitcast(wgp[...], bf16), preferred_element_type=f32)
        u = jnp.dot(h2, pltpu.bitcast(wup[...], bf16), preferred_element_type=f32)
        hh = (jnp.maximum(g, 0.0) * u).astype(bf16)
        p = jnp.dot(hh, pltpu.bitcast(wdp[...], bf16), preferred_element_type=f32)
        o_v[rows(t, al=TM), :] = (x1_ref[t % 2] + rep(mod_ref[5]) * p).astype(bf16)

    def ffn0_chunk(i):
        h2 = h2_ref[0]
        cs = slice(FOFF[i], FOFF[i + 1])
        cs2 = slice(FOFF[i] // 2, FOFF[i + 1] // 2)
        wg, wu, wd = wg_v[:, cs], wu_v[:, cs], wd_v[cs, :]
        wgp[:, cs] = pltpu.bitcast(wg, u32)
        wup[:, cs] = pltpu.bitcast(wu, u32)
        wdp[cs2, :] = pltpu.bitcast(wd, u32)
        gb = modrow(5, 6) if i == NCH - 1 else None
        g = jnp.dot(h2, wg, preferred_element_type=f32)
        u = jnp.dot(h2, wu, preferred_element_type=f32)
        hh = (jnp.maximum(g, 0.0) * u).astype(bf16)
        p = jnp.dot(hh, wd, preferred_element_type=f32)
        if i > 0:
            p = p + acc_ref[...]
        if i < NCH - 1:
            acc_ref[...] = p
        else:
            mod_ref[5] = gb
            o_v[0:TM, :] = (x1_ref[0] + rep(gb) * p).astype(bf16)

    def modrow(c0, c1):
        c = c_ref[...].astype(f32)
        sc = (c * jax.nn.sigmoid(c)).astype(bf16)
        sc8 = jnp.broadcast_to(sc, (8, D))
        return jnp.dot(sc8, wm_v[:, c0 * D:c1 * D], preferred_element_type=f32)

    def region(fn, name):
        with jax.named_scope(name):
            pl.when(z0 == 0)(fn)

    u_ref[ZSLOT, 0:3 * BLK] = jnp.zeros((3 * BLK, D), f32)
    wait(SEM_KVS0)
    skf = sk_ref[...].astype(f32)
    for m in range(4):
        taps_ref[m] = jnp.broadcast_to(skf[m:m + 1, :], (8, D))
    for t in range(3):
        if t > 0:
            wait(SEM_KVS0 + t)
        def pro(t=t):
            kv_stage(t, False)
            for b in range(2):
                dft_k(t, b)
            for b in range(2):
                dft_u(t, b)
            if t < 2:
                mac_stage(t, False)
                for b in range(2):
                    inv_b(t, b)
        region(pro, f"pro{t}")
    wait(SEM_M0)
    def pm0():
        mod = modrow(0, 3)
        sa, ca, ga = [mod[:, i * D:(i + 1) * D] for i in range(3)]
        mod_ref[0] = ga * sa
        mod_ref[1] = ga * (1.0 + ca)
        fin_a(0)
    region(pm0, "pm0")
    wait(SEM_M1)
    def pm1():
        mod = modrow(3, 5)
        mod_ref[3] = mod[:, :D]
        mod_ref[4] = 1.0 + mod[:, D:]
        fin_b(0)
    region(pm1, "pm1")

    nfin = TM // 8
    lane_parts = [range(i * NL // (NCH - 1), (i + 1) * NL // (NCH - 1)) for i in range(NCH - 1)] + [range(0)]
    for i in range(NCH):
        wait(SEM_W + i)
        def st0(i=i):
            tok = None
            if i >= 1:
                for l in lane_parts[i - 1]:
                    for b in range(2):
                        inv_b(2, b, slice(l * 128, (l + 1) * 128))
                lo, hi = (i - 1) * nfin // (NCH - 1), i * nfin // (NCH - 1)
                tok = fin_stage(1, 1, tok, range(lo, hi))
            if len(lane_parts[i]):
                mac_stage(2, True, tok, lane_parts[i])
            ffn0_chunk(i)
        region(st0, f"step0_{i}")
    wait(SEM_STEP)
    def st0e():
        kv_stage(3, False)
        for b in range(2):
            dft_k(3, b)
        for b in range(2):
            dft_u(3, b)
    region(st0e, "step0_e")

    def step(s, tfin, do_mac, do_kv, nlag=None):
        h2 = h2_ref[s % 2]
        tok = fin_stage(tfin, (s + 1) % 2)
        if do_kv:
            tok = kv_stage(s + 3, True, tok)
        if do_mac:
            mac_stage(s + 2, True, tok, nlag=nlag)
        ffn_stage(s, h2)
        for b in range(2):
            if do_mac:
                inv_b(s + 2, b)
            if do_kv:
                dft_u(s + 3, b)
                dft_k(s + 3, b)

    def body_a(s, c):
        wait(step_group(s, True))
        out_copy(s - 1).start()
        step(s, s + 1, True, True, nlag=NB - 2)
        return c
    with jax.named_scope("loopA"):
        lax.fori_loop(1, NT - 3, body_a, 0)

    wait(SEM_STEP + NT - 3)
    out_copy(NT - 4).start()
    region(lambda: step(NT - 3, NT - 2, True, False), "step5")
    wait(SEM_STEP + NT - 2)

    def body_b(s, c):
        out_copy(s - 1).start()
        step(s, jnp.minimum(s + 1, NT - 1), False, False)
        return c
    with jax.named_scope("loopB"):
        lax.fori_loop(NT - 2, NT, body_b, 0)
    out_copy(NT - 1).start()
    for t in range(NT):
        out_copy(t).wait()


@jax.jit
def pallas_adaLN_cond__ssm_conv_h3__glu_gated_reglu__prompt_kernel(A_q, A_k, A_v, A_shift_k, A_ssm_k, A_ssm_D, B_x, B_W_gate, B_W_up, B_W_down, c, w_mod):
    fm, gm = _dft_mats()
    fm = jnp.asarray(fm, bf16)
    gm = jnp.asarray(gm, bf16)
    any_spec = pl.BlockSpec(memory_space=pl.ANY)
    out = pl.pallas_call(
        _kernel,
        in_specs=[any_spec] * 13,
        out_specs=any_spec,
        out_shape=jax.ShapeDtypeStruct((S, D), bf16),
        scratch_shapes=[
            pltpu.VMEM((S, D), bf16), pltpu.VMEM((S, D), bf16), pltpu.VMEM((S, D), bf16),
            pltpu.VMEM((D, S), bf16), pltpu.VMEM((D, 6 * D), bf16),
            pltpu.VMEM((D, F), bf16), pltpu.VMEM((D, F), bf16), pltpu.VMEM((F, D), bf16),
            pltpu.VMEM((D // 2, F), u32), pltpu.VMEM((D // 2, F), u32), pltpu.VMEM((F // 2, D), u32),
            pltpu.VMEM((S, D), bf16),
            pltpu.VMEM((4, D), bf16), pltpu.VMEM((D,), bf16), pltpu.VMEM((1, D), bf16),
            pltpu.VMEM((2 * BLK, BLK), bf16), pltpu.VMEM((BLK, 2 * BLK), bf16),
            pltpu.VMEM((NB + 1, 3 * BLK + 8, D), f32), pltpu.VMEM((NB, 3 * BLK + 8, D), f32),
            pltpu.VMEM((2, 2 * BLK, D), f32), pltpu.VMEM((TM, D), bf16), pltpu.VMEM((2, 2 * BLK, D), bf16),
            pltpu.VMEM((2, TM, D), f32), pltpu.VMEM((TM, D), f32),
            pltpu.VMEM((2, TM, D), bf16), pltpu.VMEM((2, TM, D), f32),
            pltpu.VMEM((6, 8, D), f32), pltpu.VMEM((4, 8, D), f32),
            pltpu.SemaphoreType.DMA((NSEM,)), pltpu.SemaphoreType.REGULAR,
        ],
        compiler_params=pltpu.CompilerParams(vmem_limit_bytes=120 * 1024 * 1024),
    )(A_q.reshape(S, D), A_k.reshape(S, D), A_v.reshape(S, D), A_shift_k.T, A_ssm_k, A_ssm_D,
      B_W_gate, B_W_up, B_W_down, c, w_mod, fm, gm)
    return out.reshape(1, S, D)
```

```python
import functools, os
import numpy as np
import jax
import jax.numpy as jnp
from jax import lax
import jax.experimental.pallas as pl
import jax.experimental.pallas.tpu as pltpu

S, D, F = 2048, 640, 1536
BLK = 128
NB = S // BLK
TM = 256
NT = S // TM
NL = D // 128
EPS = 1e-5
f32 = jnp.float32
bf16 = jnp.bfloat16
u32 = jnp.uint32

LN_CH = int(os.environ.get("LN_CH", "8"))
KV_CH = int(os.environ.get("KV_CH", "1"))
FCH = [int(x) for x in os.environ.get("FCH", "256,256,256,256,256,256").split(",")]
DYNW = int(os.environ.get("DYNW", "1"))
FOFF = [sum(FCH[:i]) for i in range(len(FCH) + 1)]
NCH = len(FCH)
SEM_KVS0, SEM_KVS1, SEM_KVS2, SEM_M0, SEM_M1 = 0, 1, 2, 3, 4
SEM_W = 5
SEM_STEP = SEM_W + NCH
SEM_OUT = SEM_STEP + NT - 1
NSEM = SEM_OUT + 1
ZPAIR = NT
PAIR_ROWS = 800
UOFF = (8, 408)
KOFF = (0, 400)


def _dft_mats():
    f = np.concatenate([np.arange(0, BLK, 2), np.arange(1, BLK, 2)]).astype(np.float64)
    n = np.arange(BLK, dtype=np.float64)
    ang = 2.0 * np.pi * np.outer(f + 0.5, n) / (2 * BLK)
    fm = np.concatenate([np.cos(ang), -np.sin(ang)], axis=0)
    gm = fm.T / BLK
    return fm.astype(np.float32), gm.astype(np.float32)


def _kernel(q_hbm, k_hbm, v_hbm, sk_hbm, ssmk_hbm, d_hbm, wg_hbm, wu_hbm, wd_hbm, c_hbm, wm_hbm,
            fm_hbm, gm_hbm, o_hbm,
            q_v, k_v, v_v, s_v, wm_v, wg_v, wu_v, wd_v, wgp, wup, wdp, o_v,
            fm_ref, gm_ref,
            u_ref, kk_ref, kprev_ref, kvb_ref, z_ref, y_ref, acc_ref, h2_ref, h2p_ref, hhp_ref, x1_ref, taps_ref, mod_ref,
            sk_ref, d_ref, c_ref,
            sems, zsem):

    def st(x):
        return isinstance(x, int)

    def rows(t, off=0, n=TM, al=8):
        r0 = t * TM + off
        return pl.ds(r0 if st(t) else pl.multiple_of(r0, al), n)

    def cp(src, dst, sem):
        return pltpu.make_async_copy(src, dst, sems.at[sem])

    def kvs(t, sem):
        rs = rows(t, al=TM)
        return [cp(k_hbm.at[rs, :], k_v.at[rs, :], sem), cp(v_hbm.at[rs, :], v_v.at[rs, :], sem),
                cp(ssmk_hbm.at[:, rs], s_v.at[:, rs], sem)]

    def qc(t, sem):
        rs = rows(t, al=TM)
        return [cp(q_hbm.at[rs, :], q_v.at[rs, :], sem)]

    def wmc(c0, c1, sem):
        cs = pl.ds(c0 * D, (c1 - c0) * D)
        return [cp(wm_hbm.at[:, cs], wm_v.at[:, cs], sem)]

    def wc(i):
        cs = pl.ds(FOFF[i], FCH[i])
        return [cp(wg_hbm.at[:, cs], wg_v.at[:, cs], SEM_W + i), cp(wu_hbm.at[:, cs], wu_v.at[:, cs], SEM_W + i),
                cp(wd_hbm.at[cs, :], wd_v.at[cs, :], SEM_W + i)]

    def step_group(s, with_kvs):
        return qc(s + 1, SEM_STEP + s) + (kvs(s + 3, SEM_STEP + s) if with_kvs else [])

    groups = {}
    groups[SEM_KVS0] = [cp(fm_hbm, fm_ref, SEM_KVS0), cp(sk_hbm, sk_ref, SEM_KVS0), cp(d_hbm, d_ref, SEM_KVS0),
                        cp(c_hbm, c_ref, SEM_KVS0), cp(gm_hbm, gm_ref, SEM_KVS0)] + kvs(0, SEM_KVS0)
    groups[SEM_KVS1] = kvs(1, SEM_KVS1)
    groups[SEM_KVS2] = kvs(2, SEM_KVS2)
    groups[SEM_M0] = qc(0, SEM_M0) + wmc(0, 3, SEM_M0)
    groups[SEM_M1] = wmc(3, 5, SEM_M1)
    for i in range(NCH):
        groups[SEM_W + i] = wc(i)
    groups[SEM_W + 1] = qc(1, SEM_W + 1) + groups[SEM_W + 1]
    groups[SEM_W + NCH - 1] = groups[SEM_W + NCH - 1] + wmc(5, 6, SEM_W + NCH - 1)
    groups[SEM_STEP] = kvs(3, SEM_STEP)
    for s in range(1, NT - 1):
        groups[SEM_STEP + s] = step_group(s, s + 3 < NT)
    for g in sorted(groups):
        for c_ in groups[g]:
            c_.start()

    def wait(g):
        for c_ in (groups[g] if st(g) else g):
            c_.wait()

    def out_copy(t):
        rs = rows(t, al=TM)
        return cp(o_v.at[rs, :], o_hbm.at[rs, :], SEM_OUT)

    z0 = pl.semaphore_read(zsem)
    pred = jnp.full((8, 128), z0, jnp.int32) != 0

    if DYNW:
        wgp, wup, wdp, h2p_ref, hhp_ref = [r.at[z0] for r in (wgp, wup, wdp, h2p_ref, hhp_ref)]
    else:
        wgp, wup, wdp, h2p_ref, hhp_ref = [r.at[0] for r in (wgp, wup, wdp, h2p_ref, hhp_ref)]

    def gate(x, tok):
        return x if tok is None else jnp.where(pred, tok, x)

    def gate_first(x, tok):
        if tok is None:
            return x
        first = gate(x[0:8, 0:128], tok)
        return jnp.concatenate([first, x[0:8, 128:]], axis=1)

    def fold(*xs):
        parts = []
        for x in xs:
            if x is None:
                continue
            parts += [x[i:i + 8, j:j + 128] for i in range(0, x.shape[0], 8) for j in range(0, x.shape[1], 128)]
        if not parts:
            return None
        while len(parts) > 1:
            parts = [jnp.maximum(parts[i], parts[i + 1]) if i + 1 < len(parts) else parts[i] for i in range(0, len(parts), 2)]
        return parts[0]

    def rep(w):
        return jnp.tile(w, (TM // 8, 1))

    rowid = lax.broadcasted_iota(jnp.int32, (8, 128), 0)
    masks = [None] + [rowid < m for m in range(1, 4)]

    def kv_stage(t, ch, tok=None):
        toks = [tok] * KV_CH
        n = 0
        for (l0, l1) in [(0, 2), (2, 4), (4, 5)]:
            ls = slice(l0 * 128, l1 * 128)
            prev = None
            if not (st(t) and t == 0):
                pk = k_v[rows(t, -8, 8), ls].astype(f32)
                prev = [[None] + [pltpu.roll(pk[:, i * 128:(i + 1) * 128], m, 0) for m in range(1, 4)] for i in range(l1 - l0)]
            for g in range(TM // 8):
                rs = rows(t, 8 * g, 8)
                kf = k_v[rs, ls].astype(f32)
                vf = v_v[rs, ls].astype(f32)
                cur = []
                res = []
                for i in range(l1 - l0):
                    li = slice((l0 + i) * 128, (l0 + i + 1) * 128)
                    k0 = kf[:, i * 128:(i + 1) * 128]
                    if ch:
                        k0 = gate(k0, toks[n % KV_CH])
                    rots = [None] + [pltpu.roll(k0, m, 0) for m in range(1, 4)]
                    ks = k0 * taps_ref[0, :, li]
                    for m in range(1, 4):
                        sh = jnp.where(masks[m], prev[i][m] if prev is not None else 0.0, rots[m])
                        ks = ks + sh * taps_ref[m, :, li]
                    res.append(ks * vf[:, i * 128:(i + 1) * 128])
                    cur.append(rots)
                prev = cur
                kvb = (res[0] if len(res) == 1 else jnp.concatenate(res, axis=1)).astype(bf16)
                kvb_ref[8 * g:8 * g + 8, ls] = kvb
                if ch:
                    toks[n % KV_CH] = fold(*res)
                n += 1
        return fold(*toks) if ch else None

    def dft_u(t, b):
        u = jnp.dot(fm_ref[...], kvb_ref[b * BLK:(b + 1) * BLK, :], preferred_element_type=f32)
        ur, ui = u[:BLK], u[BLK:]
        o = UOFF[b]
        u_ref[t, o:o + BLK] = ur + ui
        u_ref[t, o + BLK:o + 2 * BLK] = ur
        u_ref[t, o + 2 * BLK:o + 3 * BLK] = ui

    def dft_k(t, b):
        H = BLK // 2
        a = 2 * t + b
        kraw = lax.dot_general(fm_ref[...], s_v[:, rows(t, b * BLK, BLK, al=BLK)], (((1,), (1,)), ((), ())),
                               preferred_element_type=f32)
        if st(a) and a == 0:
            cr = kraw[:BLK] + d_ref[...].astype(f32).reshape(1, D)
            di = kraw[BLK:]
        else:
            kp = kprev_ref[1 - b]
            cr = jnp.concatenate([kraw[0:H] - kp[BLK:BLK + H], kraw[H:BLK] + kp[BLK + H:]], axis=0)
            di = jnp.concatenate([kraw[BLK:BLK + H] + kp[0:H], kraw[BLK + H:] - kp[H:BLK]], axis=0)
        kprev_ref[b] = kraw
        o = KOFF[b]
        kk_ref[t, o:o + BLK] = cr
        kk_ref[t, o + BLK:o + 2 * BLK] = di - cr
        kk_ref[t, o + 2 * BLK:o + 3 * BLK] = cr + di

    def inv_b(t, b, ls=slice(None)):
        y_ref[t % 2, b * BLK:(b + 1) * BLK, ls] = jnp.dot(gm_ref[...], z_ref[b, :, ls], preferred_element_type=f32)

    def mac_stage(t, ch, tok=None, lanes=range(NL), nlag=None):
        g0 = g1 = tok
        if st(t):
            nlag = 2 * t + 2
            kidx = list(range(nlag // 2))
            uidx = [t - j for j in range(nlag // 2)]
        else:
            kidx = [jnp.minimum(j, t) for j in range(nlag // 2)]
            uidx = [jnp.where(t - j >= 0, t - j, ZPAIR) for j in range(nlag // 2)]
        for l in lanes:
            ls = slice(l * 128, (l + 1) * 128)
            for r in range(BLK // 8):
                rr = slice(r * 8, r * 8 + 8)
                accs = []
                for p in range(3):
                    a0 = a1 = None
                    uc = None
                    o = p * BLK + r * 8
                    for j in range(nlag - 1, -1, -1):
                        kp = kk_ref[kidx[j // 2], KOFF[j % 2] + o:KOFF[j % 2] + o + 8, ls]
                        un = u_ref[uidx[j // 2], UOFF[1 - j % 2] + o:UOFF[1 - j % 2] + o + 8, ls]
                        t1 = kp * un
                        a1 = gate(t1, g1) if a1 is None else a1 + t1
                        if uc is not None:
                            t0 = kp * uc
                            a0 = gate(t0, g0) if a0 is None else a0 + t0
                        uc = un
                    accs.append((a0, a1))
                    if ch:
                        g0, g1 = a1, a0
                outs = []
                for b in range(2):
                    re = accs[0][b] - accs[2][b]
                    im = accs[0][b] + accs[1][b]
                    z_ref[b, rr, ls] = re.astype(bf16)
                    z_ref[b, BLK + r * 8:BLK + r * 8 + 8, ls] = im.astype(bf16)
                    outs.append(jnp.maximum(re, im))
                if ch:
                    g1, g0 = outs
        return jnp.maximum(g0, g1) if ch else None

    def fin_stage(t, par, tok=None, gs=range(TM // 8)):
        toks = [tok] * LN_CH
        for g in gs:
            rr = slice(8 * g, 8 * g + 8)
            x = gate_first(q_v[rows(t, 8 * g, 8), :].astype(f32), toks[g % LN_CH])
            m = jnp.mean(x, axis=-1, keepdims=True)
            xc = x - m
            var = jnp.mean(xc * xc, axis=-1, keepdims=True)
            hg = (xc * lax.rsqrt(var + EPS)) * mod_ref[1] + mod_ref[0]
            x1 = x + hg * y_ref[par, rr, :]
            m = jnp.mean(x1, axis=-1, keepdims=True)
            xc = x1 - m
            var = jnp.mean(xc * xc, axis=-1, keepdims=True)
            h2 = (xc * lax.rsqrt(var + EPS)) * mod_ref[4] + mod_ref[3]
            x1_ref[par, rr, :] = x1
            h2_ref[rr, :] = h2.astype(bf16)
            toks[g % LN_CH] = fold(h2)
        return fold(*toks)

    def fin_a(t):
        x = q_v[rows(t), :].astype(f32)
        m = jnp.mean(x, axis=-1, keepdims=True)
        xc = x - m
        var = jnp.mean(xc * xc, axis=-1, keepdims=True)
        hg = (xc * lax.rsqrt(var + EPS)) * rep(mod_ref[1]) + rep(mod_ref[0])
        x1 = x + hg * y_ref[t % 2]
        m = jnp.mean(x1, axis=-1, keepdims=True)
        xc = x1 - m
        var = jnp.mean(xc * xc, axis=-1, keepdims=True)
        x1_ref[t % 2] = x1
        acc_ref[...] = xc * lax.rsqrt(var + EPS)

    def fin_b(t):
        h2p_ref[...] = pltpu.bitcast((acc_ref[...] * rep(mod_ref[4]) + rep(mod_ref[3])).astype(bf16), u32)

    def ffn_stage(t, h2):
        g = jnp.dot(h2, pltpu.bitcast(wgp[...], bf16), preferred_element_type=f32)
        u = jnp.dot(h2, pltpu.bitcast(wup[...], bf16), preferred_element_type=f32)
        hhp_ref[...] = pltpu.bitcast((jnp.maximum(g, 0.0) * u).astype(bf16), u32)
        p = jnp.dot(pltpu.bitcast(hhp_ref[...], bf16), pltpu.bitcast(wdp[...], bf16), preferred_element_type=f32)
        o_v[rows(t, al=TM), :] = (x1_ref[t % 2] + rep(mod_ref[5]) * p).astype(bf16)

    def ffn0_chunk(i):
        h2 = pltpu.bitcast(h2p_ref[...], bf16)
        cs = slice(FOFF[i], FOFF[i + 1])
        cs2 = slice(FOFF[i] // 2, FOFF[i + 1] // 2)
        wg, wu, wd = wg_v[:, cs], wu_v[:, cs], wd_v[cs, :]
        wgp[:, cs] = pltpu.bitcast(wg, u32)
        wup[:, cs] = pltpu.bitcast(wu, u32)
        wdp[cs2, :] = pltpu.bitcast(wd, u32)
        gb = modrow(5, 6) if i == NCH - 1 else None
        g = jnp.dot(h2, wg, preferred_element_type=f32)
        u = jnp.dot(h2, wu, preferred_element_type=f32)
        hh = (jnp.maximum(g, 0.0) * u).astype(bf16)
        p = jnp.dot(hh, wd, preferred_element_type=f32)
        if i > 0:
            p = p + acc_ref[...]
        if i < NCH - 1:
            acc_ref[...] = p
        else:
            mod_ref[5] = gb
            o_v[0:TM, :] = (x1_ref[0] + rep(gb) * p).astype(bf16)

    def modrow(c0, c1):
        c = c_ref[...].astype(f32)
        sc = (c * jax.nn.sigmoid(c)).astype(bf16)
        sc8 = jnp.broadcast_to(sc, (8, D))
        return jnp.dot(sc8, wm_v[:, c0 * D:c1 * D], preferred_element_type=f32)

    def region(fn, name):
        with jax.named_scope(name):
            pl.when(z0 == 0)(fn)

    u_ref[ZPAIR] = jnp.zeros((PAIR_ROWS, D), f32)
    wait(SEM_KVS0)
    skf = sk_ref[...].astype(f32)
    for m in range(4):
        taps_ref[m] = jnp.broadcast_to(skf[m:m + 1, :], (8, D))
    for t in range(3):
        if t > 0:
            wait(SEM_KVS0 + t)
        def pro(t=t):
            kv_stage(t, False)
            for b in range(2):
                dft_k(t, b)
            for b in range(2):
                dft_u(t, b)
            if t < 2:
                mac_stage(t, False)
                for b in range(2):
                    inv_b(t, b)
        region(pro, f"pro{t}")
    wait(SEM_M0)
    def pm0():
        mod = modrow(0, 3)
        sa, ca, ga = [mod[:, i * D:(i + 1) * D] for i in range(3)]
        mod_ref[0] = ga * sa
        mod_ref[1] = ga * (1.0 + ca)
        fin_a(0)
    region(pm0, "pm0")
    wait(SEM_M1)
    def pm1():
        mod = modrow(3, 5)
        mod_ref[3] = mod[:, :D]
        mod_ref[4] = 1.0 + mod[:, D:]
        fin_b(0)
    region(pm1, "pm1")

    nfin = TM // 8
    lane_parts = [range(i * NL // (NCH - 1), (i + 1) * NL // (NCH - 1)) for i in range(NCH - 1)] + [range(0)]
    for i in range(NCH):
        wait(SEM_W + i)
        def st0(i=i):
            tok = None
            if i >= 1:
                for l in lane_parts[i - 1]:
                    for b in range(2):
                        inv_b(2, b, slice(l * 128, (l + 1) * 128))
                lo, hi = (i - 1) * nfin // (NCH - 1), i * nfin // (NCH - 1)
                tok = fin_stage(1, 1, tok, range(lo, hi))
            if len(lane_parts[i]):
                mac_stage(2, True, tok, lane_parts[i])
            ffn0_chunk(i)
        region(st0, f"step0_{i}")
    wait(SEM_STEP)
    def st0e():
        kv_stage(3, False)
        for b in range(2):
            dft_k(3, b)
        for b in range(2):
            dft_u(3, b)
    region(st0e, "step0_e")

    def step(s, tfin, do_mac, do_kv, nlag=None):
        h2p_ref[...] = pltpu.bitcast(h2_ref[...], u32)
        h2 = pltpu.bitcast(h2p_ref[...], bf16)
        tok = fin_stage(tfin, (s + 1) % 2)
        if do_kv:
            tok = kv_stage(s + 3, True, tok)
        if do_mac:
            mac_stage(s + 2, True, tok, nlag=nlag)
        ffn_stage(s, h2)
        for b in range(2):
            if do_mac:
                inv_b(s + 2, b)
            if do_kv:
                dft_u(s + 3, b)
                dft_k(s + 3, b)

    def body_a(s, c):
        wait(step_group(s, True))
        out_copy(s - 1).start()
        step(s, s + 1, True, True, nlag=NB - 2)
        return c
    with jax.named_scope("loopA"):
        lax.fori_loop(1, NT - 3, body_a, 0)

    wait(SEM_STEP + NT - 3)
    out_copy(NT - 4).start()
    region(lambda: step(NT - 3, NT - 2, True, False), "step5")
    wait(SEM_STEP + NT - 2)

    def body_b(s, c):
        out_copy(s - 1).start()
        step(s, jnp.minimum(s + 1, NT - 1), False, False)
        return c
    with jax.named_scope("loopB"):
        lax.fori_loop(NT - 2, NT, body_b, 0)
    out_copy(NT - 1).start()
    for t in range(NT):
        out_copy(t).wait()


@jax.jit
def pallas_adaLN_cond__ssm_conv_h3__glu_gated_reglu__prompt_kernel(A_q, A_k, A_v, A_shift_k, A_ssm_k, A_ssm_D, B_x, B_W_gate, B_W_up, B_W_down, c, w_mod):
    fm, gm = _dft_mats()
    fm = jnp.asarray(fm, bf16)
    gm = jnp.asarray(gm, bf16)
    any_spec = pl.BlockSpec(memory_space=pl.ANY)
    out = pl.pallas_call(
        _kernel,
        in_specs=[any_spec] * 13,
        out_specs=any_spec,
        out_shape=jax.ShapeDtypeStruct((S, D), bf16),
        scratch_shapes=[
            pltpu.VMEM((S, D), bf16), pltpu.VMEM((S, D), bf16), pltpu.VMEM((S, D), bf16),
            pltpu.VMEM((D, S), bf16), pltpu.VMEM((D, 6 * D), bf16),
            pltpu.VMEM((D, F), bf16), pltpu.VMEM((D, F), bf16), pltpu.VMEM((F, D), bf16),
            pltpu.VMEM((1, D // 2, F), u32), pltpu.VMEM((1, D // 2, F), u32), pltpu.VMEM((1, F // 2, D), u32),
            pltpu.VMEM((S, D), bf16),
            pltpu.VMEM((2 * BLK, BLK), bf16), pltpu.VMEM((BLK, 2 * BLK), bf16),
            pltpu.VMEM((NT + 1, PAIR_ROWS, D), f32), pltpu.VMEM((NT, PAIR_ROWS, D), f32),
            pltpu.VMEM((2, 2 * BLK, D), f32), pltpu.VMEM((TM, D), bf16), pltpu.VMEM((2, 2 * BLK, D), bf16),
            pltpu.VMEM((2, TM, D), f32), pltpu.VMEM((TM, D), f32),
            pltpu.VMEM((TM, D), bf16), pltpu.VMEM((1, TM // 2, D), u32), pltpu.VMEM((1, TM // 2, F), u32), pltpu.VMEM((2, TM, D), f32),
            pltpu.VMEM((4, 8, D), f32), pltpu.VMEM((6, 8, D), f32),
            pltpu.VMEM((4, D), bf16), pltpu.VMEM((D,), bf16), pltpu.VMEM((1, D), bf16),
            pltpu.SemaphoreType.DMA((NSEM,)), pltpu.SemaphoreType.REGULAR,
        ],
        compiler_params=pltpu.CompilerParams(vmem_limit_bytes=120 * 1024 * 1024),
    )(A_q.reshape(S, D), A_k.reshape(S, D), A_v.reshape(S, D), A_shift_k.T, A_ssm_k, A_ssm_D,
      B_W_gate, B_W_up, B_W_down, c, w_mod, fm, gm)
    return out.reshape(1, S, D)
```

```python
import os
import numpy as np
import jax
import jax.numpy as jnp
from jax import lax
import jax.experimental.pallas as pl
import jax.experimental.pallas.tpu as pltpu

S, D, F = 2048, 640, 1536
BLK = 128
TM = 256
NT = S // TM
NL = D // 128
NG = TM // 8
FC = 256
NCH = F // FC
EPS = 1e-5
f32 = jnp.float32
bf16 = jnp.bfloat16
u32 = jnp.uint32

ZPAIR = NT
PAIR_ROWS = 800
UOFF = (8, 408)
KOFF = (0, 400)

(SEM_KVS0, SEM_KVS1, SEM_KVS2, SEM_M0, SEM_M1, SEM_Q1) = range(6)
SEM_W = 6
SEM_1B = SEM_W + NCH + 1
SEM_1C = SEM_1B + 1
SEM_STEP = SEM_1C + 1 - 2
SEM_OUT = SEM_STEP + NT - 1
NSEM = SEM_OUT + 1


def _env(name, default):
    v = os.environ.get(name)
    return default if v is None else type(default)(v)


ONLY = _env("ONLY", "")
A_MODE, A_OV, A_LOCK, A_DFT = _env("A_MODE", "fkm"), _env("A_OV", 4), _env("A_LOCK", 8), _env("A_DFT", 2)
E_MODE, E_OV, E_LOCK = _env("E_MODE", "fm"), _env("E_OV", 6), _env("E_LOCK", 6)
B_LOCK = _env("B_LOCK", 0)
P_OV = _env("P_OV", -1)
S1_DFT = _env("S1_DFT", 1)
KV_ROLL, KV_SER = _env("KV_ROLL", 1), _env("KV_SER", 0)
C_LOCK = _env("C_LOCK", 4)
S1A, S1B = _env("S1A", 2), _env("S1B", 5)
S1_OV, S1_LOCK = _env("S1_OV", 0), _env("S1_LOCK", 6)
LN_W, LN_CH = _env("LN_W", 2), _env("LN_CH", 8)


def _dft_mats():
    f = np.concatenate([np.arange(0, BLK, 2), np.arange(1, BLK, 2)]).astype(np.float64)
    n = np.arange(BLK, dtype=np.float64)
    ang = 2.0 * np.pi * np.outer(f + 0.5, n) / (2 * BLK)
    fm = np.concatenate([np.cos(ang), -np.sin(ang)], axis=0)
    gm = fm.T / BLK
    return fm.astype(np.float32), gm.astype(np.float32)


def _kernel(q_hbm, k_hbm, v_hbm, sk_hbm, ssmk_hbm, d_hbm, wg_hbm, wu_hbm, wd_hbm, c_hbm, wm_hbm,
            fm_hbm, gm_hbm, o_hbm,
            q_v, k_v, v_v, s_v, wm_v, wg_v, wu_v, wd_v, wgp, wup, wdp, o_v, fm_ref, gm_ref,
            u_ref, kk_ref, kprev_ref, kf_ref, kvb_ref, z_ref, y_ref, acc_ref, h2_ref, h2p_ref, hhp_ref, x1_ref,
            taps_ref, mod_ref, sk_ref, d_ref, c_ref, sems, zsem):

    def st(x):
        return isinstance(x, int)

    def ds(i, n, off=0, size=None, al=None):
        r0 = i * n + off
        return pl.ds(r0 if st(i) else pl.multiple_of(r0, al or n), size or n)

    def cp(src, dst, sem):
        return pltpu.make_async_copy(src, dst, sems.at[sem])

    def kvs(t, sem):
        rs = ds(t, TM)
        return [cp(k_hbm.at[rs, :], k_v.at[rs, :], sem), cp(v_hbm.at[rs, :], v_v.at[rs, :], sem),
                cp(ssmk_hbm.at[:, rs], s_v.at[:, rs], sem)]

    def qc(t, sem):
        return [cp(q_hbm.at[ds(t, TM), :], q_v.at[ds(t, TM), :], sem)]

    def wmc(c0, c1, sem):
        cs = pl.ds(c0 * D, (c1 - c0) * D)
        return [cp(wm_hbm.at[:, cs], wm_v.at[:, cs], sem)]

    def wc(i, up=True, down=True):
        r = []
        if up:
            r += [cp(wg_hbm.at[:, ds(i, FC)], wg_v.at[i], SEM_W + i), cp(wu_hbm.at[:, ds(i, FC)], wu_v.at[i], SEM_W + i)]
        if down:
            r += [cp(wd_hbm.at[ds(i - 1, FC), :], wd_v.at[i - 1], SEM_W + i)]
        return r

    def step_group(s, with_kvs):
        return qc(s + 1, SEM_STEP + s) + (kvs(s + 3, SEM_STEP + s) if with_kvs else [])

    g_kvs0 = [cp(fm_hbm, fm_ref, SEM_KVS0), cp(sk_hbm, sk_ref, SEM_KVS0), cp(d_hbm, d_ref, SEM_KVS0),
              cp(c_hbm, c_ref, SEM_KVS0), cp(gm_hbm, gm_ref, SEM_KVS0)] + kvs(0, SEM_KVS0)
    g_kvs = [g_kvs0, kvs(1, SEM_KVS1), kvs(2, SEM_KVS2)]
    g_m0 = qc(0, SEM_M0) + wmc(0, 3, SEM_M0)
    g_m1 = wmc(3, 5, SEM_M1)
    g_w0 = wc(0, down=False)
    g_q1 = qc(1, SEM_Q1)
    g_we = wc(NCH, up=False) + wmc(5, 6, SEM_W + NCH)
    g_1b = kvs(3, SEM_1B) + qc(2, SEM_1B)
    g_1c = kvs(4, SEM_1C)
    order = g_kvs + [g_m0, g_m1, g_w0, g_q1] + [wc(i) for i in range(1, NCH)] + [g_we, g_1b, g_1c]
    order += [step_group(s, s + 3 < NT) for s in range(2, NT - 1)]
    for g in order:
        for c_ in g:
            c_.start()

    def wait(g):
        for c_ in g:
            c_.wait()

    def out_copy(t):
        return cp(o_v.at[ds(t, TM), :], o_hbm.at[ds(t, TM), :], SEM_OUT)

    z0 = pl.semaphore_read(zsem)
    pred = jnp.full((8, 128), z0, jnp.int32) != 0
    h2p = h2p_ref.at[z0]

    def gate(x, tok):
        return x if tok is None else jnp.where(pred, tok, x)

    def fold(*xs):
        parts = []
        for x in xs:
            if x is not None:
                parts += [x[:, j:j + 128] for j in range(0, x.shape[1], 128)]
        while len(parts) > 1:
            parts = [jnp.maximum(parts[i], parts[i + 1]) if i + 1 < len(parts) else parts[i]
                     for i in range(0, len(parts), 2)]
        return parts[0] if parts else None

    def rep(w):
        return jnp.tile(w, (NG, 1))

    def region(fn, name):
        if ONLY and not any(name.startswith(o) for o in ONLY.split(",")):
            return
        with jax.named_scope(name):
            pl.when(z0 == 0)(fn)

    def kv_stage(t, tok=None):
        kt, vt = k_v.at[ds(t, TM)], v_v.at[ds(t, TM)]
        chain = tok is not None

        def put(g, l0, l1, val, tk=None):
            for i in range(l1 - l0):
                kf_ref[l0 + i, 8 * g + 8:8 * g + 16, :] = gate(val[:, i * 128:(i + 1) * 128], tk)

        for (l0, l1) in [(0, 2), (2, 4), (4, 5)]:
            ls = slice(l0 * 128, l1 * 128)
            if st(t) and t == 0:
                put(-1, l0, l1, jnp.zeros((8, (l1 - l0) * 128), f32))
            else:
                put(-1, l0, l1, k_v[ds(t, TM, -8, 8, 8), ls].astype(f32))
            put(0, l0, l1, kt[0:8, ls].astype(f32), tok)
            for g in range(NG):
                if g + 1 < NG:
                    put(g + 1, l0, l1, kt[8 * g + 8:8 * g + 16, ls].astype(f32), tok)
                vf = vt[8 * g:8 * g + 8, ls].astype(f32)
                res = []
                for i in range(l1 - l0):
                    li = slice((l0 + i) * 128, (l0 + i + 1) * 128)
                    ks = None
                    for m in range(4):
                        term = kf_ref[l0 + i, 8 * g + 8 - m:8 * g + 16 - m, :] * taps_ref[m, :, li]
                        ks = gate(term, tok) if ks is None else ks + term
                    res.append(ks * vf[:, i * 128:(i + 1) * 128])
                kvb_ref[8 * g:8 * g + 8, ls] = (res[0] if len(res) == 1 else jnp.concatenate(res, axis=1)).astype(bf16)
                if chain:
                    tok = fold(*res)
        return tok

    rowid = lax.broadcasted_iota(jnp.int32, (8, 128), 0)
    masks = [None] + [rowid < m for m in range(1, 4)]

    def kv_roll(t, tok=None):
        kt, vt = k_v.at[ds(t, TM)], v_v.at[ds(t, TM)]
        chain = tok is not None
        for (l0, l1) in [(0, 2), (2, 4), (4, 5)]:
            ls = slice(l0 * 128, l1 * 128)
            prev = None
            if not (st(t) and t == 0):
                pk = k_v[ds(t, TM, -8, 8, 8), ls].astype(f32)
                prev = [[None] + [pltpu.roll(pk[:, i * 128:(i + 1) * 128], m, 0) for m in range(1, 4)]
                        for i in range(l1 - l0)]
            for g in range(NG):
                kf = kt[8 * g:8 * g + 8, ls].astype(f32)
                vf = vt[8 * g:8 * g + 8, ls].astype(f32)
                cur, res = [], []
                for i in range(l1 - l0):
                    li = slice((l0 + i) * 128, (l0 + i + 1) * 128)
                    k0 = gate(kf[:, i * 128:(i + 1) * 128], tok)
                    rots = [None] + [pltpu.roll(k0, m, 0) for m in range(1, 4)]
                    ks = k0 * taps_ref[0, :, li]
                    for m in range(1, 4):
                        sh = jnp.where(masks[m], prev[i][m] if prev is not None else 0.0, rots[m])
                        ks = ks + sh * taps_ref[m, :, li]
                    res.append(ks * vf[:, i * 128:(i + 1) * 128])
                    cur.append(rots)
                    if chain and KV_SER:
                        tok = res[-1]
                prev = cur
                kvb_ref[8 * g:8 * g + 8, ls] = (res[0] if len(res) == 1 else jnp.concatenate(res, axis=1)).astype(bf16)
                if chain and not KV_SER:
                    tok = fold(*res)
        return tok

    if KV_ROLL:
        kv_stage = kv_roll

    def dft_u(t, b):
        u = jnp.dot(fm_ref[...], kvb_ref[b * BLK:(b + 1) * BLK, :], preferred_element_type=f32)
        ur, ui = u[:BLK], u[BLK:]
        o = UOFF[b]
        u_ref[t, o:o + BLK] = ur + ui
        u_ref[t, o + BLK:o + 2 * BLK] = ur
        u_ref[t, o + 2 * BLK:o + 3 * BLK] = ui

    def dft_k(t, b, kp=None):
        H = BLK // 2
        kraw = lax.dot_general(fm_ref[...], s_v[:, ds(t, TM, b * BLK, BLK, BLK)], (((1,), (1,)), ((), ())),
                               preferred_element_type=f32)
        if st(t) and t == 0 and b == 0:
            cr = kraw[:BLK] + d_ref[...].astype(f32).reshape(1, D)
            di = kraw[BLK:]
        else:
            if kp is None:
                kp = kprev_ref[...]
            cr = jnp.concatenate([kraw[0:H] - kp[BLK:BLK + H], kraw[H:BLK] + kp[BLK + H:]], axis=0)
            di = jnp.concatenate([kraw[BLK:BLK + H] + kp[0:H], kraw[BLK + H:] - kp[H:BLK]], axis=0)
        if b == 1:
            kprev_ref[...] = kraw
        o = KOFF[b]
        kk_ref[t, o:o + BLK] = cr
        kk_ref[t, o + BLK:o + 2 * BLK] = di - cr
        kk_ref[t, o + 2 * BLK:o + 3 * BLK] = cr + di
        return kraw

    def dft_parts(t):
        kp = [None]

        def k0():
            kp[0] = dft_k(t, 0)
        return [k0, lambda: dft_u(t, 0), lambda: dft_k(t, 1, kp[0]), lambda: dft_u(t, 1)]

    def dft_stage(t):
        for fn in dft_parts(t):
            fn()

    def inv_stage(t, slot=None):
        for b in range(2):
            y_ref[t % 2 if slot is None else slot, b * BLK:(b + 1) * BLK, :] = jnp.dot(gm_ref[...], z_ref[b], preferred_element_type=f32)

    def mac_stage(t, chain, tok=None, late=None, nlag=None, ov=0):
        g0 = g1 = tok
        if st(t):
            nlag = 2 * t + 2
            kidx = list(range(nlag // 2))
            uidx = [t - j for j in range(nlag // 2)]
        else:
            kidx = [jnp.minimum(j, t) for j in range(nlag // 2)]
            uidx = [jnp.where(t - j >= 0, t - j, ZPAIR) for j in range(nlag // 2)]
        for l in range(NL):
            ls = slice(l * 128, (l + 1) * 128)
            for r in range(BLK // 8):
                accs = []
                for p in range(3):
                    a0 = a1 = uc = None
                    o = p * BLK + r * 8
                    for j in range(nlag - 1, -1, -1):
                        kp = kk_ref[kidx[j // 2], KOFF[j % 2] + o:KOFF[j % 2] + o + 8, ls]
                        un = u_ref[uidx[j // 2], UOFF[1 - j % 2] + o:UOFF[1 - j % 2] + o + 8, ls]
                        t1 = kp * un
                        a1 = gate(t1, g1) if a1 is None else a1 + t1
                        if uc is not None:
                            t0 = kp * uc
                            a0 = gate(t0, g0) if a0 is None else a0 + t0
                        uc = un
                        if chain and p < 2 and j == min(ov, nlag - 2):
                            n0, n1 = a1, a0
                    accs.append((a0, a1))
                    if chain and p < 2:
                        g0, g1 = n0, n1
                outs = []
                for b in range(2):
                    re = accs[0][b] - accs[2][b]
                    im = accs[0][b] + accs[1][b]
                    z_ref[b, r * 8:r * 8 + 8, ls] = re.astype(bf16)
                    z_ref[b, BLK + r * 8:BLK + r * 8 + 8, ls] = im.astype(bf16)
                    outs.append(jnp.maximum(re, im))
                if chain:
                    g1, g0 = outs
                    if late is not None and r == 5:
                        g0 = jnp.maximum(g0, late)
                        late = None
        return jnp.maximum(g0, g1) if chain else None

    def fin_piece(qrows, rr, par, toks):
        x = qrows.astype(f32)
        xs = [gate(x[:, i * 128:(i + 1) * 128], toks[i] if i < len(toks) else None) for i in range(NL)]
        x = jnp.concatenate(xs, axis=1)
        pre = ((xs[0] + xs[1]) + (xs[2] + xs[3])) + xs[4]
        xc = x - jnp.sum(pre, axis=-1, keepdims=True) * (1.0 / D)
        mid = xc[:, 0:128]
        var = jnp.mean(xc * xc, axis=-1, keepdims=True)
        hg = (xc * lax.rsqrt(var + EPS)) * mod_ref[1] + mod_ref[0]
        x1 = x + hg * y_ref[par, rr, :]
        xc = x1 - jnp.mean(x1, axis=-1, keepdims=True)
        var = jnp.mean(xc * xc, axis=-1, keepdims=True)
        h2 = (xc * lax.rsqrt(var + EPS)) * mod_ref[4] + mod_ref[3]
        x1_ref[par, rr, :] = x1
        h2_ref[rr, :] = h2.astype(bf16)
        return pre, mid, fold(h2)

    def fin_stage(t, par, lock, tok=None, base=None, n=NG):
        qt = q_v.at[ds(t, TM)]
        pres, mids, ends = [], [], []
        for g in range(n):
            rr = pl.ds(8 * g, 8) if base is None else pl.ds(pl.multiple_of(base + 8 * g, 8), 8)
            if lock:
                toks = [ends[g - lock] if g >= lock else tok]
            else:
                toks = [mids[g - LN_W] if g >= LN_W else tok, pres[g - 1] if g >= 1 else None,
                        ends[g - LN_CH] if g >= LN_CH else None]
            pre, mid, end = fin_piece(qt[rr, :], rr, par, toks)
            pres.append(pre), mids.append(mid), ends.append(end)
        if lock:
            return fold(*ends[-lock:]), None
        return mids[-1], fold(*ends[-LN_CH:])

    def fin_a():
        x = q_v[0:TM, :].astype(f32)
        xc = x - jnp.mean(x, axis=-1, keepdims=True)
        var = jnp.mean(xc * xc, axis=-1, keepdims=True)
        hg = (xc * lax.rsqrt(var + EPS)) * rep(mod_ref[1]) + rep(mod_ref[0])
        x1 = x + hg * y_ref[2]
        xc = x1 - jnp.mean(x1, axis=-1, keepdims=True)
        var = jnp.mean(xc * xc, axis=-1, keepdims=True)
        x1_ref[0] = x1
        acc_ref[...] = xc * lax.rsqrt(var + EPS)

    def fin_b():
        h2p[...] = pltpu.bitcast((acc_ref[...] * rep(mod_ref[4]) + rep(mod_ref[3])).astype(bf16), u32)
        acc_ref[...] = jnp.zeros((TM, D), f32)

    def modrow(c0, c1):
        c = c_ref[...].astype(f32)
        sc = jnp.broadcast_to((c * jax.nn.sigmoid(c)).astype(bf16), (8, D))
        return jnp.dot(sc, wm_v[:, c0 * D:c1 * D], preferred_element_type=f32)

    def cat(ref, c0, c1, axis, cs=slice(None)):
        return pltpu.bitcast(jnp.concatenate([ref[z0 + c, :, cs] for c in range(c0, c1)], axis=axis), bf16)

    def ffn_up(c0, c1):
        h2 = pltpu.bitcast(h2p[...], bf16)
        g = jnp.dot(h2, cat(wgp, c0, c1, 1), preferred_element_type=f32)
        u = jnp.dot(h2, cat(wup, c0, c1, 1), preferred_element_type=f32)
        hh = pltpu.bitcast((jnp.maximum(g, 0.0) * u).astype(bf16), u32)
        for c in range(c0, c1):
            hhp_ref[z0 + c] = hh[:, (c - c0) * FC:(c - c0 + 1) * FC]

    def ffn_down(t, inter=(), at=NL):
        hh = cat(hhp_ref, 0, NCH, 1)
        cuts = [0] + [n for n in range(max(at, 1), NL)][:len(inter)] + [NL]
        inter = list(inter)
        for n0, n1 in zip(cuts[:-1], cuts[1:]):
            cs = slice(n0 * 128, n1 * 128)
            p = jnp.dot(hh, cat(wdp, 0, NCH, 0, cs), preferred_element_type=f32)
            o_v[ds(t, TM), cs] = (x1_ref[t % 2, :, cs] + rep(mod_ref[5, :, cs]) * p).astype(bf16)
            if inter:
                inter.pop(0)()
        for fn in inter:
            fn()

    def ffn0_up(i):
        h2 = pltpu.bitcast(h2p[...], bf16)
        wg, wu = wg_v[i], wu_v[i]
        wgp[i] = pltpu.bitcast(wg, u32)
        wup[i] = pltpu.bitcast(wu, u32)
        g = jnp.dot(h2, wg, preferred_element_type=f32)
        u = jnp.dot(h2, wu, preferred_element_type=f32)
        hhp_ref[i] = pltpu.bitcast((jnp.maximum(g, 0.0) * u).astype(bf16), u32)

    def ffn0_down(i):
        wd = wd_v[i]
        wdp[i] = pltpu.bitcast(wd, u32)
        return acc_ref[...] + jnp.dot(pltpu.bitcast(hhp_ref[i], bf16), wd, preferred_element_type=f32)

    def side_work(mode, tfin, par, tkv, tmac, lock, ov, nlag=None):
        tok = late = None
        for c in mode:
            if c == "f":
                tok, late = fin_stage(tfin, par, lock, tok)
            elif c == "k":
                tok = kv_stage(tkv, jnp.zeros((8, 128), f32) if tok is None else tok)
            elif c == "m":
                tok = mac_stage(tmac, True, tok, late, nlag, ov)
                late = None

    def pack_h2():
        h2p[...] = pltpu.bitcast(h2_ref[...], u32)

    u_ref[ZPAIR] = jnp.zeros((PAIR_ROWS, D), f32)
    wait(g_kvs0)
    skf = sk_ref[...].astype(f32)
    for m in range(4):
        taps_ref[m] = jnp.broadcast_to(skf[m:m + 1, :], (8, D))

    def pro0():
        kv_stage(0)
        dft_stage(0)
        mac_stage(0, False)
        inv_stage(0, 2)
    region(pro0, "pro0")

    def body_p1(t, c):
        wait(kvs(t, SEM_KVS0 + t))
        kv_stage(t)
        dft_stage(t)
        return c

    def body_p2(t, c):
        mac_stage(t, P_OV >= 0, nlag=6, ov=P_OV)
        inv_stage(t)
        return c
    with jax.named_scope("pro1"):
        lax.fori_loop(1, 3, body_p1, 0)
    with jax.named_scope("pro2"):
        lax.fori_loop(1, 3, body_p2, 0)
    wait(g_m0)

    def pm0():
        mod = modrow(0, 3)
        sa, ca, ga = [mod[:, i * D:(i + 1) * D] for i in range(3)]
        mod_ref[0] = ga * sa
        mod_ref[1] = ga * (1.0 + ca)
        fin_a()
    region(pm0, "pm0")
    wait(g_m1)

    def pm1():
        mod = modrow(3, 5)
        mod_ref[3] = mod[:, :D]
        mod_ref[4] = 1.0 + mod[:, D:]
        fin_b()
    region(pm1, "pm1")

    wait(g_w0)
    region(lambda: ffn0_up(0), "step0_0")
    wait(g_q1)

    def body_0(i, c):
        wait(wc(i))
        acc_ref[...] = ffn0_down(i - 1)
        fin_stage(1, 1, C_LOCK, base=jnp.minimum(i - 1, 3) * (TM // 4), n=NG // 4)
        ffn0_up(i)
        return c
    with jax.named_scope("step0_l"):
        if not ONLY or "step0" in ONLY:
            lax.fori_loop(1, NCH, body_0, 0)
        else:
            for i in range(1, NCH):
                wait(wc(i))
    wait(g_we)

    def st0e():
        gb = modrow(5, 6)
        mod_ref[5] = gb
        o_v[0:TM, :] = (x1_ref[0] + rep(gb) * ffn0_down(NCH - 1)).astype(bf16)
        pack_h2()
        ffn_up(0, S1A)
    region(st0e, "step1_a")

    wait(g_1b)
    out_copy(0).start()

    def st1b():
        side_work("kf", 2, 0, 3, None, S1_LOCK, 0)
        ffn_up(S1A, S1B)
        dft_stage(3)
    region(st1b, "step1_b")
    wait(g_1c)

    def st1c():
        side_work("km", None, None, 4, 3, 0, S1_OV)
        if S1B < NCH:
            ffn_up(S1B, NCH)
        ffn_down(1, dft_parts(4), S1_DFT)
        inv_stage(3)
    region(st1c, "step1_c")

    def body_a(s, c):
        wait(step_group(s, True))
        out_copy(s - 1).start()
        pack_h2()
        side_work(A_MODE, s + 1, (s + 1) % 2, s + 3, s + 2, A_LOCK, A_OV, nlag=2 * NT - 2)
        ffn_up(0, NCH)
        ffn_down(s, dft_parts(s + 3), A_DFT)
        inv_stage(s + 2)
        return c
    with jax.named_scope("loopA"):
        if not ONLY or "A" in ONLY:
            lax.fori_loop(2, NT - 3, body_a, 0)
        else:
            for s_ in range(2, NT - 3):
                wait(step_group(s_, True))
                out_copy(s_ - 1).start()

    wait(step_group(NT - 3, False))
    out_copy(NT - 4).start()

    def st5():
        s = NT - 3
        pack_h2()
        side_work(E_MODE, s + 1, (s + 1) % 2, None, s + 2, E_LOCK, E_OV)
        ffn_up(0, NCH)
        ffn_down(s)
        inv_stage(s + 2)
    region(st5, "step5")
    wait(step_group(NT - 2, False))

    def body_b(s, c):
        out_copy(s - 1).start()
        pack_h2()
        fin_stage(jnp.minimum(s + 1, NT - 1), (s + 1) % 2, B_LOCK)
        ffn_up(0, NCH)
        ffn_down(s)
        return c
    with jax.named_scope("loopB"):
        if not ONLY or "B" in ONLY:
            lax.fori_loop(NT - 2, NT, body_b, 0)
        else:
            for s_ in range(NT - 2, NT):
                out_copy(s_ - 1).start()
    out_copy(NT - 1).start()
    for t in range(NT):
        out_copy(t).wait()


@jax.jit
def pallas_adaLN_cond__ssm_conv_h3__glu_gated_reglu__prompt_kernel(A_q, A_k, A_v, A_shift_k, A_ssm_k, A_ssm_D, B_x, B_W_gate, B_W_up, B_W_down, c, w_mod):
    fm, gm = _dft_mats()
    any_spec = pl.BlockSpec(memory_space=pl.ANY)
    V = pltpu.VMEM
    out = pl.pallas_call(
        _kernel,
        in_specs=[any_spec] * 13,
        out_specs=any_spec,
        out_shape=jax.ShapeDtypeStruct((S, D), bf16),
        scratch_shapes=[
            V((S, D), bf16), V((S, D), bf16), V((S, D), bf16), V((D, S), bf16), V((D, 6 * D), bf16),
            V((NCH, D, FC), bf16), V((NCH, D, FC), bf16), V((NCH, FC, D), bf16),
            V((NCH, D // 2, FC), u32), V((NCH, D // 2, FC), u32), V((NCH, FC // 2, D), u32),
            V((S, D), bf16), V((2 * BLK, BLK), bf16), V((BLK, 2 * BLK), bf16),
            V((NT + 1, PAIR_ROWS, D), f32), V((NT, PAIR_ROWS, D), f32),
            V((2 * BLK, D), f32), V((NL, TM + 32, 128), f32), V((TM, D), bf16), V((2, 2 * BLK, D), bf16),
            V((3, TM, D), f32), V((TM, D), f32), V((TM, D), bf16), V((1, TM // 2, D), u32),
            V((NCH, TM // 2, FC), u32), V((2, TM, D), f32),
            V((4, 8, D), f32), V((6, 8, D), f32), V((4, D), bf16), V((D,), bf16), V((1, D), bf16),
            pltpu.SemaphoreType.DMA((NSEM,)), pltpu.SemaphoreType.REGULAR,
        ],
        compiler_params=pltpu.CompilerParams(vmem_limit_bytes=120 * 1024 * 1024),
    )(A_q.reshape(S, D), A_k.reshape(S, D), A_v.reshape(S, D), A_shift_k.T, A_ssm_k, A_ssm_D,
      B_W_gate, B_W_up, B_W_down, c, w_mod, jnp.asarray(fm, bf16), jnp.asarray(gm, bf16))
    return out.reshape(1, S, D)
```

```python
import os
import numpy as np
import jax
import jax.numpy as jnp
from jax import lax
import jax.experimental.pallas as pl
import jax.experimental.pallas.tpu as pltpu

S, D, F = 2048, 640, 1536
BLK = 128
TM = 256
NT = S // TM
NL = D // 128
NG = TM // 8
FC = 256
NCH = F // FC
EPS = 1e-5
f32 = jnp.float32
bf16 = jnp.bfloat16
u32 = jnp.uint32

ZPAIR = NT
PAIR_ROWS = 800
UOFF = (8, 408)
KOFF = (0, 400)

(SEM_KVS0, SEM_KVS1, SEM_KVS2, SEM_M0, SEM_M1, SEM_Q1) = range(6)
SEM_W = 6
SEM_1B = SEM_W + NCH + 1
SEM_1C = SEM_1B + 1
SEM_STEP = SEM_1C + 1 - 2
SEM_OUT = SEM_STEP + NT - 1
NSEM = SEM_OUT + 1


def _env(name, default):
    v = os.environ.get(name)
    return default if v is None else type(default)(v)


ONLY = _env("ONLY", "")
A_MODE, A_OV, A_LOCK, A_DFT = _env("A_MODE", "fkm"), _env("A_OV", 4), _env("A_LOCK", 8), _env("A_DFT", 3)
E_MODE, E_OV, E_LOCK = _env("E_MODE", "fm"), _env("E_OV", 6), _env("E_LOCK", 6)
B_LOCK = _env("B_LOCK", 0)
P_OV = _env("P_OV", -1)
S1_DFT = _env("S1_DFT", 1)
KV_ROLL, KV_SER = _env("KV_ROLL", 1), _env("KV_SER", 0)
C_LOCK = _env("C_LOCK", 4)
S1A, S1A_DFT = _env("S1A", 3), _env("S1A_DFT", 2)
S1A_MODE, S1B_MODE = _env("S1A_MODE", "k"), _env("S1B_MODE", "fkm")
S1_OV, S1_LOCK = _env("S1_OV", 2), _env("S1_LOCK", 6)
LN_W, LN_CH = _env("LN_W", 2), _env("LN_CH", 8)


def _dft_mats():
    f = np.concatenate([np.arange(0, BLK, 2), np.arange(1, BLK, 2)]).astype(np.float64)
    n = np.arange(BLK, dtype=np.float64)
    ang = 2.0 * np.pi * np.outer(f + 0.5, n) / (2 * BLK)
    fm = np.concatenate([np.cos(ang), -np.sin(ang)], axis=0)
    gm = fm.T / BLK
    return fm.astype(np.float32), gm.astype(np.float32)


def _kernel(q_hbm, k_hbm, v_hbm, sk_hbm, ssmk_hbm, d_hbm, wg_hbm, wu_hbm, wd_hbm, c_hbm, wm_hbm,
            fm_hbm, gm_hbm, o_hbm,
            q_v, k_v, v_v, s_v, wm_v, wg_v, wu_v, wd_v, wgp, wup, wdp, o_v, fm_ref, gm_ref,
            u_ref, kk_ref, kprev_ref, kvb_ref, z_ref, y_ref, acc_ref, h2_ref, h2p_ref, hhp_ref, x1_ref,
            taps_ref, mod_ref, sk_ref, d_ref, c_ref, sems, zsem):

    def st(x):
        return isinstance(x, int)

    def ds(i, n, off=0, size=None, al=None):
        r0 = i * n + off
        return pl.ds(r0 if st(i) else pl.multiple_of(r0, al or n), size or n)

    def cp(src, dst, sem):
        return pltpu.make_async_copy(src, dst, sems.at[sem])

    def kvs(t, sem):
        rs = ds(t, TM)
        return [cp(k_hbm.at[rs, :], k_v.at[rs, :], sem), cp(v_hbm.at[rs, :], v_v.at[rs, :], sem),
                cp(ssmk_hbm.at[:, rs], s_v.at[:, rs], sem)]

    def qc(t, sem):
        return [cp(q_hbm.at[ds(t, TM), :], q_v.at[ds(t, TM), :], sem)]

    def wmc(c0, c1, sem):
        cs = pl.ds(c0 * D, (c1 - c0) * D)
        return [cp(wm_hbm.at[:, cs], wm_v.at[:, cs], sem)]

    def wc(i, up=True, down=True):
        r = []
        if up:
            r += [cp(wg_hbm.at[:, ds(i, FC)], wg_v.at[i], SEM_W + i), cp(wu_hbm.at[:, ds(i, FC)], wu_v.at[i], SEM_W + i)]
        if down:
            r += [cp(wd_hbm.at[ds(i - 1, FC), :], wd_v.at[i - 1], SEM_W + i)]
        return r

    def step_group(s, with_kvs):
        return qc(s + 1, SEM_STEP + s) + (kvs(s + 3, SEM_STEP + s) if with_kvs else [])

    g_kvs0 = [cp(fm_hbm, fm_ref, SEM_KVS0), cp(sk_hbm, sk_ref, SEM_KVS0), cp(d_hbm, d_ref, SEM_KVS0),
              cp(c_hbm, c_ref, SEM_KVS0), cp(gm_hbm, gm_ref, SEM_KVS0)] + kvs(0, SEM_KVS0)
    g_kvs = [g_kvs0, kvs(1, SEM_KVS1), kvs(2, SEM_KVS2)]
    g_m0 = qc(0, SEM_M0) + wmc(0, 3, SEM_M0)
    g_m1 = wmc(3, 5, SEM_M1)
    g_w0 = wc(0, down=False)
    g_q1 = qc(1, SEM_Q1)
    g_we = wc(NCH, up=False) + wmc(5, 6, SEM_W + NCH)
    g_1b = kvs(3, SEM_1B) + (qc(2, SEM_1B) if "f" in S1A_MODE else [])
    g_1c = kvs(4, SEM_1C) + (qc(2, SEM_1C) if "f" not in S1A_MODE else [])
    order = g_kvs + [g_m0, g_m1, g_w0, g_q1] + [wc(i) for i in range(1, NCH)] + [g_1b, g_we, g_1c]
    order += [step_group(s, s + 3 < NT) for s in range(2, NT - 1)]
    for g in order:
        for c_ in g:
            c_.start()

    def wait(g):
        for c_ in g:
            c_.wait()

    def out_copy(t):
        return cp(o_v.at[ds(t, TM), :], o_hbm.at[ds(t, TM), :], SEM_OUT)

    z0 = pl.semaphore_read(zsem)
    pred = jnp.full((8, 128), z0, jnp.int32) != 0
    h2p = h2p_ref.at[z0]

    def gate(x, tok):
        return x if tok is None else jnp.where(pred, tok, x)

    def fold(*xs):
        parts = []
        for x in xs:
            if x is not None:
                parts += [x[:, j:j + 128] for j in range(0, x.shape[1], 128)]
        while len(parts) > 1:
            parts = [jnp.maximum(parts[i], parts[i + 1]) if i + 1 < len(parts) else parts[i]
                     for i in range(0, len(parts), 2)]
        return parts[0] if parts else None

    def rep(w):
        return jnp.tile(w, (NG, 1))

    def region(fn, name):
        if ONLY and not any(name.startswith(o) for o in ONLY.split(",")):
            return
        with jax.named_scope(name):
            pl.when(z0 == 0)(fn)

    rowid = lax.broadcasted_iota(jnp.int32, (8, 128), 0)
    masks = [None] + [rowid < m for m in range(1, 4)]

    def kv_stage(t, tok=None):
        kt, vt = k_v.at[ds(t, TM)], v_v.at[ds(t, TM)]
        chain = tok is not None
        for (l0, l1) in [(0, 2), (2, 4), (4, 5)]:
            ls = slice(l0 * 128, l1 * 128)
            prev = None
            if not (st(t) and t == 0):
                pk = k_v[ds(t, TM, -8, 8, 8), ls].astype(f32)
                prev = [[None] + [pltpu.roll(pk[:, i * 128:(i + 1) * 128], m, 0) for m in range(1, 4)]
                        for i in range(l1 - l0)]
            for g in range(NG):
                kf = kt[8 * g:8 * g + 8, ls].astype(f32)
                vf = vt[8 * g:8 * g + 8, ls].astype(f32)
                cur, res = [], []
                for i in range(l1 - l0):
                    li = slice((l0 + i) * 128, (l0 + i + 1) * 128)
                    k0 = gate(kf[:, i * 128:(i + 1) * 128], tok)
                    rots = [None] + [pltpu.roll(k0, m, 0) for m in range(1, 4)]
                    ks = k0 * taps_ref[0, :, li]
                    for m in range(1, 4):
                        sh = jnp.where(masks[m], prev[i][m] if prev is not None else 0.0, rots[m])
                        ks = ks + sh * taps_ref[m, :, li]
                    res.append(ks * vf[:, i * 128:(i + 1) * 128])
                    cur.append(rots)
                    if chain and KV_SER:
                        tok = res[-1]
                prev = cur
                kvb_ref[8 * g:8 * g + 8, ls] = (res[0] if len(res) == 1 else jnp.concatenate(res, axis=1)).astype(bf16)
                if chain and not KV_SER:
                    tok = fold(*res)
        return tok

    def dft_u(t, b):
        u = jnp.dot(fm_ref[...], kvb_ref[b * BLK:(b + 1) * BLK, :], preferred_element_type=f32)
        ur, ui = u[:BLK], u[BLK:]
        o = UOFF[b]
        u_ref[t, o:o + BLK] = ur + ui
        u_ref[t, o + BLK:o + 2 * BLK] = ur
        u_ref[t, o + 2 * BLK:o + 3 * BLK] = ui

    def dft_k(t, b, kp=None):
        H = BLK // 2
        kraw = lax.dot_general(fm_ref[...], s_v[:, ds(t, TM, b * BLK, BLK, BLK)], (((1,), (1,)), ((), ())),
                               preferred_element_type=f32)
        if st(t) and t == 0 and b == 0:
            cr = kraw[:BLK] + d_ref[...].astype(f32).reshape(1, D)
            di = kraw[BLK:]
        else:
            if kp is None:
                kp = kprev_ref[...]
            cr = jnp.concatenate([kraw[0:H] - kp[BLK:BLK + H], kraw[H:BLK] + kp[BLK + H:]], axis=0)
            di = jnp.concatenate([kraw[BLK:BLK + H] + kp[0:H], kraw[BLK + H:] - kp[H:BLK]], axis=0)
        if b == 1:
            kprev_ref[...] = kraw
        o = KOFF[b]
        kk_ref[t, o:o + BLK] = cr
        kk_ref[t, o + BLK:o + 2 * BLK] = di - cr
        kk_ref[t, o + 2 * BLK:o + 3 * BLK] = cr + di
        return kraw

    def dft_parts(t):
        kp = [None]

        def k0():
            kp[0] = dft_k(t, 0)
        return [k0, lambda: dft_u(t, 0), lambda: dft_k(t, 1, kp[0]), lambda: dft_u(t, 1)]

    def dft_stage(t):
        for fn in dft_parts(t):
            fn()

    def inv_stage(t, slot=None):
        for b in range(2):
            y_ref[t % 2 if slot is None else slot, b * BLK:(b + 1) * BLK, :] = jnp.dot(gm_ref[...], z_ref[b], preferred_element_type=f32)

    def mac_stage(t, chain, tok=None, late=None, nlag=None, ov=0):
        g0 = g1 = tok
        if st(t):
            nlag = 2 * t + 2
            kidx = list(range(nlag // 2))
            uidx = [t - j for j in range(nlag // 2)]
        else:
            kidx = [jnp.minimum(j, t) for j in range(nlag // 2)]
            uidx = [jnp.where(t - j >= 0, t - j, ZPAIR) for j in range(nlag // 2)]
        for l in range(NL):
            ls = slice(l * 128, (l + 1) * 128)
            for r in range(BLK // 8):
                accs = []
                for p in range(3):
                    a0 = a1 = uc = None
                    o = p * BLK + r * 8
                    for j in range(nlag - 1, -1, -1):
                        kp = kk_ref[kidx[j // 2], KOFF[j % 2] + o:KOFF[j % 2] + o + 8, ls]
                        un = u_ref[uidx[j // 2], UOFF[1 - j % 2] + o:UOFF[1 - j % 2] + o + 8, ls]
                        t1 = kp * un
                        a1 = gate(t1, g1) if a1 is None else a1 + t1
                        if uc is not None:
                            t0 = kp * uc
                            a0 = gate(t0, g0) if a0 is None else a0 + t0
                        uc = un
                        if chain and p < 2 and j == min(ov, nlag - 2):
                            n0, n1 = a1, a0
                    accs.append((a0, a1))
                    if chain and p < 2:
                        g0, g1 = n0, n1
                outs = []
                for b in range(2):
                    re = accs[0][b] - accs[2][b]
                    im = accs[0][b] + accs[1][b]
                    z_ref[b, r * 8:r * 8 + 8, ls] = re.astype(bf16)
                    z_ref[b, BLK + r * 8:BLK + r * 8 + 8, ls] = im.astype(bf16)
                    outs.append(jnp.maximum(re, im))
                if chain:
                    g1, g0 = outs
                    if late is not None and r == 5:
                        g0 = jnp.maximum(g0, late)
                        late = None
        return jnp.maximum(g0, g1) if chain else None

    def fin_piece(qrows, rr, par, toks):
        x = qrows.astype(f32)
        xs = [gate(x[:, i * 128:(i + 1) * 128], toks[i] if i < len(toks) else None) for i in range(NL)]
        x = jnp.concatenate(xs, axis=1)
        pre = ((xs[0] + xs[1]) + (xs[2] + xs[3])) + xs[4]
        xc = x - jnp.sum(pre, axis=-1, keepdims=True) * (1.0 / D)
        mid = xc[:, 0:128]
        var = jnp.mean(xc * xc, axis=-1, keepdims=True)
        hg = (xc * lax.rsqrt(var + EPS)) * mod_ref[1] + mod_ref[0]
        x1 = x + hg * y_ref[par, rr, :]
        xc = x1 - jnp.mean(x1, axis=-1, keepdims=True)
        var = jnp.mean(xc * xc, axis=-1, keepdims=True)
        h2 = (xc * lax.rsqrt(var + EPS)) * mod_ref[4] + mod_ref[3]
        x1_ref[par, rr, :] = x1
        h2_ref[rr, :] = h2.astype(bf16)
        return pre, mid, fold(h2)

    def fin_stage(t, par, lock, tok=None, base=None, n=NG):
        qt = q_v.at[ds(t, TM)]
        pres, mids, ends = [], [], []
        for g in range(n):
            rr = pl.ds(8 * g, 8) if base is None else pl.ds(pl.multiple_of(base + 8 * g, 8), 8)
            if lock:
                toks = [ends[g - lock] if g >= lock else tok]
            else:
                toks = [mids[g - LN_W] if g >= LN_W else tok, pres[g - 1] if g >= 1 else None,
                        ends[g - LN_CH] if g >= LN_CH else None]
            pre, mid, end = fin_piece(qt[rr, :], rr, par, toks)
            pres.append(pre), mids.append(mid), ends.append(end)
        if lock:
            return fold(*ends[-lock:]), None
        return mids[-1], fold(*ends[-LN_CH:])

    def fin_a():
        x = q_v[0:TM, :].astype(f32)
        xc = x - jnp.mean(x, axis=-1, keepdims=True)
        var = jnp.mean(xc * xc, axis=-1, keepdims=True)
        hg = (xc * lax.rsqrt(var + EPS)) * rep(mod_ref[1]) + rep(mod_ref[0])
        x1 = x + hg * y_ref[2]
        xc = x1 - jnp.mean(x1, axis=-1, keepdims=True)
        var = jnp.mean(xc * xc, axis=-1, keepdims=True)
        x1_ref[2] = x1
        acc_ref[...] = xc * lax.rsqrt(var + EPS)

    def fin_b():
        h2p[...] = pltpu.bitcast((acc_ref[...] * rep(mod_ref[4]) + rep(mod_ref[3])).astype(bf16), u32)
        acc_ref[...] = jnp.zeros((TM, D), f32)

    def modrow(c0, c1):
        c = c_ref[...].astype(f32)
        sc = jnp.broadcast_to((c * jax.nn.sigmoid(c)).astype(bf16), (8, D))
        return jnp.dot(sc, wm_v[:, c0 * D:c1 * D], preferred_element_type=f32)

    def cat(ref, c0, c1, axis, cs=slice(None)):
        return pltpu.bitcast(jnp.concatenate([ref[z0 + c, :, cs] for c in range(c0, c1)], axis=axis), bf16)

    def ffn_up(c0, c1):
        h2 = pltpu.bitcast(h2p[...], bf16)
        g = jnp.dot(h2, cat(wgp, c0, c1, 1), preferred_element_type=f32)
        u = jnp.dot(h2, cat(wup, c0, c1, 1), preferred_element_type=f32)
        hh = pltpu.bitcast((jnp.maximum(g, 0.0) * u).astype(bf16), u32)
        for c in range(c0, c1):
            hhp_ref[z0 + c] = hh[:, (c - c0) * FC:(c - c0 + 1) * FC]

    def out_col(t, n):
        cs = pl.ds(n * 128, 128)
        return cp(o_v.at[ds(t, TM), cs], o_hbm.at[ds(t, TM), cs], SEM_OUT)

    def ffn_down(t, inter=(), at=NL):
        hh = cat(hhp_ref, 0, NCH, 1)
        cuts = [0] + [n for n in range(max(at, 1), NL)][:len(inter)] + [NL]
        inter = list(inter)
        for n0, n1 in zip(cuts[:-1], cuts[1:]):
            cs = slice(n0 * 128, n1 * 128)
            p = jnp.dot(hh, cat(wdp, 0, NCH, 0, cs), preferred_element_type=f32)
            o_v[ds(t, TM), cs] = (x1_ref[t % 2, :, cs] + rep(mod_ref[5, :, cs]) * p).astype(bf16)
            if inter:
                inter.pop(0)()
        for fn in inter:
            fn()

    def ffn0_up(i):
        h2 = pltpu.bitcast(h2p[...], bf16)
        wg, wu = wg_v[i], wu_v[i]
        wgp[i] = pltpu.bitcast(wg, u32)
        wup[i] = pltpu.bitcast(wu, u32)
        g = jnp.dot(h2, wg, preferred_element_type=f32)
        u = jnp.dot(h2, wu, preferred_element_type=f32)
        hhp_ref[i] = pltpu.bitcast((jnp.maximum(g, 0.0) * u).astype(bf16), u32)

    def ffn0_down(i):
        wd = wd_v[i]
        wdp[i] = pltpu.bitcast(wd, u32)
        return acc_ref[...] + jnp.dot(pltpu.bitcast(hhp_ref[i], bf16), wd, preferred_element_type=f32)

    def side_work(mode, tfin, par, tkv, tmac, lock, ov, nlag=None):
        tok = late = None
        for c in mode:
            if c == "f":
                tok, late = fin_stage(tfin, par, lock, tok)
            elif c == "k":
                tok = kv_stage(tkv, jnp.zeros((8, 128), f32) if tok is None else tok)
            elif c == "m":
                tok = mac_stage(tmac, True, tok, late, nlag, ov)
                late = None

    def pack_h2():
        h2p[...] = pltpu.bitcast(h2_ref[...], u32)

    u_ref[ZPAIR] = jnp.zeros((PAIR_ROWS, D), f32)
    wait(g_kvs0)
    skf = sk_ref[...].astype(f32)
    for m in range(4):
        taps_ref[m] = jnp.broadcast_to(skf[m:m + 1, :], (8, D))

    def pro0():
        kv_stage(0)
        dft_stage(0)
        mac_stage(0, False)
        inv_stage(0, 2)
    region(pro0, "pro0")

    def body_p1(t, c):
        wait(kvs(t, SEM_KVS0 + t))
        kv_stage(t)
        dft_stage(t)
        return c

    def body_p2(t, c):
        mac_stage(t, P_OV >= 0, nlag=6, ov=P_OV)
        inv_stage(t)
        return c
    with jax.named_scope("pro1"):
        lax.fori_loop(1, 3, body_p1, 0)
    with jax.named_scope("pro2"):
        lax.fori_loop(1, 3, body_p2, 0)
    wait(g_m0)

    def pm0():
        mod = modrow(0, 3)
        sa, ca, ga = [mod[:, i * D:(i + 1) * D] for i in range(3)]
        mod_ref[0] = ga * sa
        mod_ref[1] = ga * (1.0 + ca)
        fin_a()
    region(pm0, "pm0")
    wait(g_m1)

    def pm1():
        mod = modrow(3, 5)
        mod_ref[3] = mod[:, :D]
        mod_ref[4] = 1.0 + mod[:, D:]
        fin_b()
    region(pm1, "pm1")

    wait(g_w0)
    region(lambda: ffn0_up(0), "step0_0")
    wait(g_q1)

    def body_0(i, c):
        wait(wc(i))
        acc_ref[...] = ffn0_down(i - 1)
        fin_stage(1, 1, C_LOCK, base=jnp.minimum(i - 1, 3) * (TM // 4), n=NG // 4)
        ffn0_up(i)
        return c
    with jax.named_scope("step0_l"):
        if not ONLY or "step0" in ONLY:
            lax.fori_loop(1, NCH, body_0, 0)
        else:
            for i in range(1, NCH):
                wait(wc(i))

    wait(g_1b)

    def st1a():
        pack_h2()
        side_work(S1A_MODE, 2, 0, 3, None, S1_LOCK, 0)
        parts = dft_parts(3)
        ffn_up(0, S1A_DFT)
        for c in range(S1A_DFT, S1A):
            for fn in parts[:2]:
                fn()
            parts = parts[2:]
            ffn_up(c, c + 1)
        for fn in parts:
            fn()
    region(st1a, "step1_a")
    wait(g_we)
    wait(g_1c)

    def st1b():
        p0 = ffn0_down(NCH - 1)
        gb = modrow(5, 6)
        mod_ref[5] = gb
        o_v[0:TM, :] = (x1_ref[2] + rep(gb) * p0).astype(bf16)
        side_work(S1B_MODE, 2, 0, 4, 3, S1_LOCK, S1_OV)
        ffn_up(S1A, NCH)
        ffn_down(1, dft_parts(4), S1_DFT)
        inv_stage(3)
    region(st1b, "step1_b")
    out_copy(0).start()

    def body_a(s, c):
        wait(step_group(s, True))
        out_copy(s - 1).start()
        pack_h2()
        side_work(A_MODE, s + 1, (s + 1) % 2, s + 3, s + 2, A_LOCK, A_OV, nlag=2 * NT - 2)
        ffn_up(0, NCH)
        ffn_down(s, dft_parts(s + 3), A_DFT)
        inv_stage(s + 2)
        return c
    with jax.named_scope("loopA"):
        if not ONLY or "A" in ONLY:
            lax.fori_loop(2, NT - 3, body_a, 0)
        else:
            for s_ in range(2, NT - 3):
                wait(step_group(s_, True))
                out_copy(s_ - 1).start()

    wait(step_group(NT - 3, False))
    out_copy(NT - 4).start()

    def st5():
        s = NT - 3
        pack_h2()
        side_work(E_MODE, s + 1, (s + 1) % 2, None, s + 2, E_LOCK, E_OV)
        ffn_up(0, NCH)
        ffn_down(s)
        inv_stage(s + 2)
    region(st5, "step5")
    wait(step_group(NT - 2, False))

    out_copy(NT - 3).start()

    def body_b(s, c):
        pack_h2()
        fin_stage(jnp.minimum(s + 1, NT - 1), (s + 1) % 2, B_LOCK)
        ffn_up(0, NCH)
        ffn_down(s, [out_col(s, n).start for n in range(NL)], 1)
        return c
    with jax.named_scope("loopB"):
        if not ONLY or "B" in ONLY:
            lax.fori_loop(NT - 2, NT, body_b, 0)
        else:
            for s_ in range(NT - 2, NT):
                out_copy(s_).start()
    for t in range(NT):
        out_copy(t).wait()


@jax.jit
def pallas_adaLN_cond__ssm_conv_h3__glu_gated_reglu__prompt_kernel(A_q, A_k, A_v, A_shift_k, A_ssm_k, A_ssm_D, B_x, B_W_gate, B_W_up, B_W_down, c, w_mod):
    fm, gm = _dft_mats()
    any_spec = pl.BlockSpec(memory_space=pl.ANY)
    V = pltpu.VMEM
    out = pl.pallas_call(
        _kernel,
        in_specs=[any_spec] * 13,
        out_specs=any_spec,
        out_shape=jax.ShapeDtypeStruct((S, D), bf16),
        scratch_shapes=[
            V((S, D), bf16), V((S, D), bf16), V((S, D), bf16), V((D, S), bf16), V((D, 6 * D), bf16),
            V((NCH, D, FC), bf16), V((NCH, D, FC), bf16), V((NCH, FC, D), bf16),
            V((NCH, D // 2, FC), u32), V((NCH, D // 2, FC), u32), V((NCH, FC // 2, D), u32),
            V((S, D), bf16), V((2 * BLK, BLK), bf16), V((BLK, 2 * BLK), bf16),
            V((NT + 1, PAIR_ROWS, D), f32), V((NT, PAIR_ROWS, D), f32),
            V((2 * BLK, D), f32), V((TM, D), bf16), V((2, 2 * BLK, D), bf16),
            V((3, TM, D), f32), V((TM, D), f32), V((TM, D), bf16), V((1, TM // 2, D), u32),
            V((NCH, TM // 2, FC), u32), V((3, TM, D), f32),
            V((4, 8, D), f32), V((6, 8, D), f32), V((4, D), bf16), V((D,), bf16), V((1, D), bf16),
            pltpu.SemaphoreType.DMA((NSEM,)), pltpu.SemaphoreType.REGULAR,
        ],
        compiler_params=pltpu.CompilerParams(vmem_limit_bytes=120 * 1024 * 1024),
    )(A_q.reshape(S, D), A_k.reshape(S, D), A_v.reshape(S, D), A_shift_k.T, A_ssm_k, A_ssm_D,
      B_W_gate, B_W_up, B_W_down, c, w_mod, jnp.asarray(fm, bf16), jnp.asarray(gm, bf16))
    return out.reshape(1, S, D)
```

```python
import numpy as np
import jax
import jax.numpy as jnp
from jax import lax
import jax.experimental.pallas as pl
import jax.experimental.pallas.tpu as pltpu

S, D, F = 2048, 640, 1536
BLK = 128
TM = 256
NT = S // TM
NL = D // 128
NG = TM // 8
FC = 256
NCH = F // FC
EPS = 1e-5
f32 = jnp.float32
bf16 = jnp.bfloat16
u32 = jnp.uint32

ZPAIR = NT
PAIR_ROWS = 800
UOFF = (8, 408)
KOFF = (0, 400)

(SEM_KVS0, SEM_KVS1, SEM_KVS2, SEM_M0, SEM_M1, SEM_Q1) = range(6)
SEM_W = 6
SEM_1A = SEM_W + NCH + 1
SEM_1B = SEM_1A + 1
SEM_STEP = SEM_1B + 1 - 2
SEM_OUT = SEM_STEP + NT - 1
NSEM = SEM_OUT + 1


def _kernel(q_hbm, k_hbm, v_hbm, sk_hbm, ssmk_hbm, d_hbm, wg_hbm, wu_hbm, wd_hbm, c_hbm, wm_hbm, o_hbm,
            q_v, k_v, v_v, s_v, wm_v, wg_v, wu_v, wd_v, wgp, wup, wdp, o_v, fm_ref, gm_ref,
            u_ref, kk_ref, kprev_ref, kvb_ref, z_ref, y_ref, acc_ref, h2_ref, h2p_ref, hhp_ref, x1_ref,
            taps_ref, mod_ref, sk_ref, d_ref, c_ref, sems, zsem):

    def st(x):
        return isinstance(x, int)

    def ds(i, n, off=0, size=None, al=None):
        r0 = i * n + off
        return pl.ds(r0 if st(i) else pl.multiple_of(r0, al or n), size or n)

    def cp(src, dst, sem):
        return pltpu.make_async_copy(src, dst, sems.at[sem])

    def kvs(t, sem):
        rs = ds(t, TM)
        return [cp(k_hbm.at[rs, :], k_v.at[rs, :], sem), cp(v_hbm.at[rs, :], v_v.at[rs, :], sem),
                cp(ssmk_hbm.at[:, rs], s_v.at[:, rs], sem)]

    def qc(t, sem):
        return [cp(q_hbm.at[ds(t, TM), :], q_v.at[ds(t, TM), :], sem)]

    def wmc(c0, c1, sem):
        cs = pl.ds(c0 * D, (c1 - c0) * D)
        return [cp(wm_hbm.at[:, cs], wm_v.at[:, cs], sem)]

    def wc(i, up=True, down=True):
        r = []
        if up:
            r += [cp(wg_hbm.at[:, ds(i, FC)], wg_v.at[i], SEM_W + i),
                  cp(wu_hbm.at[:, ds(i, FC)], wu_v.at[i], SEM_W + i)]
        if down:
            r += [cp(wd_hbm.at[ds(i - 1, FC), :], wd_v.at[i - 1], SEM_W + i)]
        return r

    def step_group(s, with_kvs):
        return qc(s + 1, SEM_STEP + s) + (kvs(s + 3, SEM_STEP + s) if with_kvs else [])

    g_kvs0 = kvs(0, SEM_KVS0) + [cp(sk_hbm, sk_ref, SEM_KVS0), cp(d_hbm, d_ref, SEM_KVS0),
                                 cp(c_hbm, c_ref, SEM_KVS0)]
    g_m0 = qc(0, SEM_M0) + wmc(0, 3, SEM_M0)
    g_m1 = wmc(3, 5, SEM_M1)
    g_w0 = wc(0, down=False)
    g_q1 = qc(1, SEM_Q1)
    g_we = wc(NCH, up=False) + wmc(5, 6, SEM_W + NCH)
    g_1a = kvs(3, SEM_1A)
    g_1b = kvs(4, SEM_1B) + qc(2, SEM_1B)
    order = [g_kvs0, kvs(1, SEM_KVS1), kvs(2, SEM_KVS2), g_m0, g_m1, g_w0, g_q1]
    order += [wc(i) for i in range(1, NCH)] + [g_1a, g_we, g_1b]
    order += [step_group(s, s + 3 < NT) for s in range(2, NT - 1)]
    for g in order:
        for c_ in g:
            c_.start()

    def wait(g):
        for c_ in g:
            c_.wait()

    def out_copy(t):
        return cp(o_v.at[ds(t, TM), :], o_hbm.at[ds(t, TM), :], SEM_OUT)

    def out_col(t, n):
        cs = pl.ds(n * 128, 128)
        return cp(o_v.at[ds(t, TM), cs], o_hbm.at[ds(t, TM), cs], SEM_OUT)

    z0 = pl.semaphore_read(zsem)
    pred = jnp.full((8, 128), z0, jnp.int32) != 0
    h2p = h2p_ref.at[z0]

    def gate(x, tok):
        return x if tok is None else jnp.where(pred, tok, x)

    def fold(*xs):
        parts = []
        for x in xs:
            parts += [x[:, j:j + 128] for j in range(0, x.shape[1], 128)]
        while len(parts) > 1:
            parts = [jnp.maximum(parts[i], parts[i + 1]) if i + 1 < len(parts) else parts[i]
                     for i in range(0, len(parts), 2)]
        return parts[0]

    def rep(w):
        return jnp.tile(w, (NG, 1))

    def region(fn):
        pl.when(z0 == 0)(fn)

    rowid = lax.broadcasted_iota(jnp.int32, (8, 128), 0)
    masks = [None] + [rowid < m for m in range(1, 4)]

    def kv_stage(t, tok=None):
        kt, vt = k_v.at[ds(t, TM)], v_v.at[ds(t, TM)]
        chain = tok is not None
        for (l0, l1) in [(0, 2), (2, 4), (4, 5)]:
            ls = slice(l0 * 128, l1 * 128)
            prev = None
            if not (st(t) and t == 0):
                pk = k_v[ds(t, TM, -8, 8, 8), ls].astype(f32)
                prev = [[None] + [pltpu.roll(pk[:, i * 128:(i + 1) * 128], m, 0) for m in range(1, 4)]
                        for i in range(l1 - l0)]
            for g in range(NG):
                kf = kt[8 * g:8 * g + 8, ls].astype(f32)
                vf = vt[8 * g:8 * g + 8, ls].astype(f32)
                cur, res = [], []
                for i in range(l1 - l0):
                    li = slice((l0 + i) * 128, (l0 + i + 1) * 128)
                    k0 = gate(kf[:, i * 128:(i + 1) * 128], tok)
                    rots = [None] + [pltpu.roll(k0, m, 0) for m in range(1, 4)]
                    ks = k0 * taps_ref[0, :, li]
                    for m in range(1, 4):
                        sh = jnp.where(masks[m], prev[i][m] if prev is not None else 0.0, rots[m])
                        ks = ks + sh * taps_ref[m, :, li]
                    res.append(ks * vf[:, i * 128:(i + 1) * 128])
                    cur.append(rots)
                prev = cur
                kv = res[0] if len(res) == 1 else jnp.concatenate(res, axis=1)
                kvb_ref[8 * g:8 * g + 8, ls] = kv.astype(bf16)
                if chain:
                    tok = fold(*res)
        return tok

    def dft_u(t, b):
        u = jnp.dot(fm_ref[...], kvb_ref[b * BLK:(b + 1) * BLK, :], preferred_element_type=f32)
        ur, ui = u[:BLK], u[BLK:]
        o = UOFF[b]
        u_ref[t, o:o + BLK] = ur + ui
        u_ref[t, o + BLK:o + 2 * BLK] = ur
        u_ref[t, o + 2 * BLK:o + 3 * BLK] = ui

    def dft_k(t, l0, l1):
        H = BLK // 2
        sblk = s_v[l0 * 128:l1 * 128, ds(t, TM)]
        rhs = jnp.concatenate([sblk[i * 128:(i + 1) * 128, b * BLK:(b + 1) * BLK]
                               for i in range(l1 - l0) for b in range(2)], axis=0)
        kr = lax.dot_general(fm_ref[...], rhs, (((1,), (1,)), ((), ())), preferred_element_type=f32)
        for i in range(l1 - l0):
            ls = slice((l0 + i) * 128, (l0 + i + 1) * 128)
            raws = [kr[:, (2 * i + b) * 128:(2 * i + b + 1) * 128] for b in range(2)]
            for b in range(2):
                kraw = raws[b]
                if st(t) and t == 0 and b == 0:
                    cr = kraw[:BLK] + d_ref[...].astype(f32).reshape(1, D)[:, ls]
                    di = kraw[BLK:]
                else:
                    kp = kprev_ref[:, ls] if b == 0 else raws[0]
                    cr = jnp.concatenate([kraw[0:H] - kp[BLK:BLK + H], kraw[H:BLK] + kp[BLK + H:]], axis=0)
                    di = jnp.concatenate([kraw[BLK:BLK + H] + kp[0:H], kraw[BLK + H:] - kp[H:BLK]], axis=0)
                o = KOFF[b]
                kk_ref[t, o:o + BLK, ls] = cr
                kk_ref[t, o + BLK:o + 2 * BLK, ls] = di - cr
                kk_ref[t, o + 2 * BLK:o + 3 * BLK, ls] = cr + di
            kprev_ref[:, ls] = raws[1]

    def dft_parts(t):
        return [lambda: dft_k(t, 0, 2), lambda: dft_u(t, 0), lambda: dft_k(t, 2, 5), lambda: dft_u(t, 1)]

    def dft_stage(t):
        for fn in dft_parts(t):
            fn()

    def inv_stage(t, slot=None):
        for b in range(2):
            y_ref[t % 2 if slot is None else slot, b * BLK:(b + 1) * BLK, :] = jnp.dot(
                gm_ref[...], z_ref[b], preferred_element_type=f32)

    def mac_stage(t, chain, tok=None, nlag=None, ov=0):
        g0 = g1 = tok
        if st(t):
            nlag = 2 * t + 2
            kidx = list(range(nlag // 2))
            uidx = [t - j for j in range(nlag // 2)]
        else:
            kidx = [jnp.minimum(j, t) for j in range(nlag // 2)]
            uidx = [jnp.where(t - j >= 0, t - j, ZPAIR) for j in range(nlag // 2)]
        for l in range(NL):
            ls = slice(l * 128, (l + 1) * 128)
            for r in range(BLK // 8):
                accs = []
                for p in range(3):
                    a0 = a1 = uc = None
                    o = p * BLK + r * 8
                    for j in range(nlag - 1, -1, -1):
                        kp = kk_ref[kidx[j // 2], KOFF[j % 2] + o:KOFF[j % 2] + o + 8, ls]
                        un = u_ref[uidx[j // 2], UOFF[1 - j % 2] + o:UOFF[1 - j % 2] + o + 8, ls]
                        t1 = kp * un
                        a1 = gate(t1, g1) if a1 is None else a1 + t1
                        if uc is not None:
                            t0 = kp * uc
                            a0 = gate(t0, g0) if a0 is None else a0 + t0
                        uc = un
                        if chain and p < 2 and j == min(ov, nlag - 2):
                            n0, n1 = a1, a0
                    accs.append((a0, a1))
                    if chain and p < 2:
                        g0, g1 = n0, n1
                outs = []
                for b in range(2):
                    re = accs[0][b] - accs[2][b]
                    im = accs[0][b] + accs[1][b]
                    z_ref[b, r * 8:r * 8 + 8, ls] = re.astype(bf16)
                    z_ref[b, BLK + r * 8:BLK + r * 8 + 8, ls] = im.astype(bf16)
                    outs.append(jnp.maximum(re, im))
                if chain:
                    g1, g0 = outs

    def fin_stage(t, par, lock, base=None, n=NG):
        qt = q_v.at[ds(t, TM)]
        ends = []
        for g in range(n):
            rr = pl.ds(8 * g, 8) if base is None else pl.ds(pl.multiple_of(base + 8 * g, 8), 8)
            x = qt[rr, :].astype(f32)
            xs = [x[:, i * 128:(i + 1) * 128] for i in range(NL)]
            xs[0] = gate(xs[0], ends[g - lock] if g >= lock else None)
            x = jnp.concatenate(xs, axis=1)
            pre = ((xs[0] + xs[1]) + (xs[2] + xs[3])) + xs[4]
            xc = x - jnp.sum(pre, axis=-1, keepdims=True) * (1.0 / D)
            var = jnp.mean(xc * xc, axis=-1, keepdims=True)
            hg = (xc * lax.rsqrt(var + EPS)) * mod_ref[1] + mod_ref[0]
            x1 = x + hg * y_ref[par, rr, :]
            xc = x1 - jnp.mean(x1, axis=-1, keepdims=True)
            var = jnp.mean(xc * xc, axis=-1, keepdims=True)
            h2 = (xc * lax.rsqrt(var + EPS)) * mod_ref[4] + mod_ref[3]
            x1_ref[par, rr, :] = x1
            h2_ref[rr, :] = h2.astype(bf16)
            ends.append(fold(h2))
        return fold(*ends[-lock:])

    def modrow(c0, c1):
        c = c_ref[...].astype(f32)
        sc = jnp.broadcast_to((c * jax.nn.sigmoid(c)).astype(bf16), (8, D))
        return jnp.dot(sc, wm_v[:, c0 * D:c1 * D], preferred_element_type=f32)

    def cat(ref, c0, c1, axis, cs=slice(None)):
        return pltpu.bitcast(jnp.concatenate([ref[z0 + c, :, cs] for c in range(c0, c1)], axis=axis), bf16)

    def ffn_up(c0, c1):
        h2 = pltpu.bitcast(h2p[...], bf16)
        g = jnp.dot(h2, cat(wgp, c0, c1, 1), preferred_element_type=f32)
        u = jnp.dot(h2, cat(wup, c0, c1, 1), preferred_element_type=f32)
        hh = pltpu.bitcast((jnp.maximum(g, 0.0) * u).astype(bf16), u32)
        for c in range(c0, c1):
            hhp_ref[z0 + c] = hh[:, (c - c0) * FC:(c - c0 + 1) * FC]

    def ffn_down(t, inter=(), at=NL):
        hh = cat(hhp_ref, 0, NCH, 1)
        cuts = [0] + [n for n in range(max(at, 1), NL)][:len(inter)] + [NL]
        inter = list(inter)
        for n0, n1 in zip(cuts[:-1], cuts[1:]):
            cs = slice(n0 * 128, n1 * 128)
            p = jnp.dot(hh, cat(wdp, 0, NCH, 0, cs), preferred_element_type=f32)
            o_v[ds(t, TM), cs] = (x1_ref[t % 2, :, cs] + rep(mod_ref[5, :, cs]) * p).astype(bf16)
            if inter:
                inter.pop(0)()
        for fn in inter:
            fn()

    def ffn0_up(i):
        h2 = pltpu.bitcast(h2p[...], bf16)
        wg, wu = wg_v[i], wu_v[i]
        wgp[i] = pltpu.bitcast(wg, u32)
        wup[i] = pltpu.bitcast(wu, u32)
        g = jnp.dot(h2, wg, preferred_element_type=f32)
        u = jnp.dot(h2, wu, preferred_element_type=f32)
        hhp_ref[i] = pltpu.bitcast((jnp.maximum(g, 0.0) * u).astype(bf16), u32)

    def ffn0_down(i):
        wd = wd_v[i]
        wdp[i] = pltpu.bitcast(wd, u32)
        return acc_ref[...] + jnp.dot(pltpu.bitcast(hhp_ref[i], bf16), wd, preferred_element_type=f32)

    def pack_h2():
        h2p[...] = pltpu.bitcast(h2_ref[...], u32)

    u_ref[ZPAIR] = jnp.zeros((PAIR_ROWS, D), f32)
    ri = lax.broadcasted_iota(jnp.int32, (BLK, BLK), 0)
    ci = lax.broadcasted_iota(jnp.int32, (BLK, BLK), 1)
    f2 = jnp.where(ri < BLK // 2, 4 * ri + 1, 4 * ri - (2 * BLK - 3))
    ang = ((f2 * ci) & (4 * BLK - 1)).astype(f32) * (np.pi / (2 * BLK))
    cs_, sn_ = jnp.cos(ang), -jnp.sin(ang)
    fm_ref[0:BLK, :] = cs_.astype(bf16)
    fm_ref[BLK:, :] = sn_.astype(bf16)
    gm_ref[:, 0:BLK] = (cs_.T * (1.0 / BLK)).astype(bf16)
    gm_ref[:, BLK:] = (sn_.T * (1.0 / BLK)).astype(bf16)
    wait(g_kvs0)
    skf = sk_ref[...].astype(f32)
    for m in range(4):
        taps_ref[m] = jnp.broadcast_to(skf[m:m + 1, :], (8, D))

    @region
    def _():
        kv_stage(0)
        dft_stage(0)
        mac_stage(0, False)
        inv_stage(0, 2)

    def body_p1(t, c):
        wait(kvs(t, SEM_KVS0 + t))
        kv_stage(t)
        dft_stage(t)
        return c

    def body_p2(t, c):
        mac_stage(t, False, nlag=6)
        inv_stage(t)
        return c
    lax.fori_loop(1, 3, body_p1, 0)
    lax.fori_loop(1, 3, body_p2, 0)
    wait(g_m0)

    @region
    def _():
        mod = modrow(0, 3)
        sa, ca, ga = [mod[:, i * D:(i + 1) * D] for i in range(3)]
        mod_ref[0] = ga * sa
        mod_ref[1] = ga * (1.0 + ca)
        x = q_v[0:TM, :].astype(f32)
        xc = x - jnp.mean(x, axis=-1, keepdims=True)
        var = jnp.mean(xc * xc, axis=-1, keepdims=True)
        hg = (xc * lax.rsqrt(var + EPS)) * rep(mod_ref[1]) + rep(mod_ref[0])
        x1 = x + hg * y_ref[2]
        xc = x1 - jnp.mean(x1, axis=-1, keepdims=True)
        var = jnp.mean(xc * xc, axis=-1, keepdims=True)
        x1_ref[2] = x1
        acc_ref[...] = xc * lax.rsqrt(var + EPS)
    wait(g_m1)

    @region
    def _():
        mod = modrow(3, 5)
        mod_ref[3] = mod[:, :D]
        mod_ref[4] = 1.0 + mod[:, D:]
        h2p[...] = pltpu.bitcast((acc_ref[...] * rep(mod_ref[4]) + rep(mod_ref[3])).astype(bf16), u32)
        acc_ref[...] = jnp.zeros((TM, D), f32)

    wait(g_w0)
    region(lambda: ffn0_up(0))
    wait(g_q1)

    def body_0(i, c):
        wait(wc(i))
        acc_ref[...] = ffn0_down(i - 1)
        fin_stage(1, 1, 4, base=jnp.minimum(i - 1, 3) * (TM // 4), n=NG // 4)
        ffn0_up(i)
        return c
    lax.fori_loop(1, NCH, body_0, 0)

    wait(g_1a)

    @region
    def _():
        pack_h2()
        kv_stage(3, jnp.zeros((8, 128), f32))
        k0, u0, k1, u1 = dft_parts(3)
        for c, fn in enumerate([k0, k1, u0]):
            ffn_up(c, c + 1)
            fn()
        u1()
    wait(g_we)
    wait(g_1b)

    @region
    def _():
        p0 = ffn0_down(NCH - 1)
        gb = modrow(5, 6)
        mod_ref[5] = gb
        o_v[0:TM, :] = (x1_ref[2] + rep(gb) * p0).astype(bf16)
        mac_stage(3, True, kv_stage(4, fin_stage(2, 0, 6)), ov=2)
        ffn_up(3, NCH)
        ffn_down(1, dft_parts(4), 2)
        inv_stage(3)
    out_copy(0).start()

    def body_a(s, c):
        wait(step_group(s, True))
        out_copy(s - 1).start()
        pack_h2()
        mac_stage(s + 2, True, kv_stage(s + 3, fin_stage(s + 1, (s + 1) % 2, 6)), nlag=2 * NT - 2, ov=3)
        ffn_up(0, NCH)
        ffn_down(s, dft_parts(s + 3), 4)
        inv_stage(s + 2)
        return c
    lax.fori_loop(2, NT - 3, body_a, 0)

    wait(step_group(NT - 3, False))
    out_copy(NT - 4).start()

    @region
    def _():
        s = NT - 3
        pack_h2()
        mac_stage(s + 2, True, fin_stage(s + 1, (s + 1) % 2, 5), ov=3)
        ffn_up(0, NCH)
        ffn_down(s)
        inv_stage(s + 2)
    wait(step_group(NT - 2, False))
    out_copy(NT - 3).start()

    def body_b(s, c):
        pack_h2()
        fin_stage(jnp.minimum(s + 1, NT - 1), (s + 1) % 2, 3)
        ffn_up(0, NCH)
        ffn_down(s, [out_col(s, n).start for n in range(NL)], 1)
        return c
    lax.fori_loop(NT - 2, NT, body_b, 0)
    cp(o_v, o_hbm, SEM_OUT).wait()


@jax.jit
def pallas_adaLN_cond__ssm_conv_h3__glu_gated_reglu__prompt_kernel(
    A_q: jax.Array,
    A_k: jax.Array,
    A_v: jax.Array,
    A_shift_k: jax.Array,
    A_ssm_k: jax.Array,
    A_ssm_D: jax.Array,
    B_x: jax.Array,
    B_W_gate: jax.Array,
    B_W_up: jax.Array,
    B_W_down: jax.Array,
    c: jax.Array,
    w_mod: jax.Array,
):
    any_spec = pl.BlockSpec(memory_space=pl.ANY)
    V = pltpu.VMEM
    out = pl.pallas_call(
        _kernel,
        in_specs=[any_spec] * 11,
        out_specs=any_spec,
        out_shape=jax.ShapeDtypeStruct((S, D), bf16),
        scratch_shapes=[
            V((S, D), bf16), V((S, D), bf16), V((S, D), bf16), V((D, S), bf16), V((D, 6 * D), bf16),
            V((NCH, D, FC), bf16), V((NCH, D, FC), bf16), V((NCH, FC, D), bf16),
            V((NCH, D // 2, FC), u32), V((NCH, D // 2, FC), u32), V((NCH, FC // 2, D), u32),
            V((S, D), bf16), V((2 * BLK, BLK), bf16), V((BLK, 2 * BLK), bf16),
            V((NT + 1, PAIR_ROWS, D), f32), V((NT, PAIR_ROWS, D), f32),
            V((2 * BLK, D), f32), V((TM, D), bf16), V((2, 2 * BLK, D), bf16),
            V((3, TM, D), f32), V((TM, D), f32), V((TM, D), bf16), V((1, TM // 2, D), u32),
            V((NCH, TM // 2, FC), u32), V((3, TM, D), f32),
            V((4, 8, D), f32), V((6, 8, D), f32), V((4, D), bf16), V((D,), bf16), V((1, D), bf16),
            pltpu.SemaphoreType.DMA((NSEM,)), pltpu.SemaphoreType.REGULAR,
        ],
        compiler_params=pltpu.CompilerParams(vmem_limit_bytes=120 * 1024 * 1024),
    )(A_q.reshape(S, D), A_k.reshape(S, D), A_v.reshape(S, D), A_shift_k.T, A_ssm_k, A_ssm_D,
      B_W_gate, B_W_up, B_W_down, c, w_mod)
    return out.reshape(1, S, D)
```

```python
import numpy as np
import jax
import jax.numpy as jnp
from jax import lax
import jax.experimental.pallas as pl
import jax.experimental.pallas.tpu as pltpu

S, D, F = 2048, 640, 1536
BLK = 128
TM = 256
NT = S // TM
NL = D // 128
NG = TM // 8
FC = 256
NCH = F // FC
EPS = 1e-5
f32 = jnp.float32
bf16 = jnp.bfloat16
u32 = jnp.uint32

ZPAIR = NT
PAIR_ROWS = 800
UOFF = (8, 408)
KOFF = (0, 400)

(SEM_KVS0, SEM_KVS1, SEM_KVS2, SEM_M0, SEM_M1, SEM_Q1) = range(6)
SEM_W = 6
SEM_1A = SEM_W + NCH + 1
SEM_1B = SEM_1A + 1
SEM_STEP = SEM_1B + 1 - 2
SEM_OUT = SEM_STEP + NT - 1
NSEM = SEM_OUT + 1


def _kernel(q_hbm, k_hbm, v_hbm, sk_hbm, ssmk_hbm, d_hbm, wg_hbm, wu_hbm, wd_hbm, c_hbm, wm_hbm, o_hbm,
            q_v, k_v, v_v, s_v, wm_v, wg_v, wu_v, wd_v, wgp, wup, wdp, o_v, fm_ref, gm_ref,
            u_ref, kk_ref, kprev_ref, kvb_ref, z_ref, y_ref, acc_ref, h2_ref, h2p_ref, hhp_ref, x1_ref,
            taps_ref, mod_ref, sk_ref, d_ref, c_ref, sems, zsem):

    def st(x):
        return isinstance(x, int)

    def ds(i, n, off=0, size=None, al=None):
        r0 = i * n + off
        return pl.ds(r0 if st(i) else pl.multiple_of(r0, al or n), size or n)

    def cp(src, dst, sem):
        return pltpu.make_async_copy(src, dst, sems.at[sem])

    def kvs(t, sem):
        rs = ds(t, TM)
        return [cp(k_hbm.at[rs, :], k_v.at[rs, :], sem), cp(v_hbm.at[rs, :], v_v.at[rs, :], sem),
                cp(ssmk_hbm.at[:, rs], s_v.at[:, rs], sem)]

    def qc(t, sem):
        return [cp(q_hbm.at[ds(t, TM), :], q_v.at[ds(t, TM), :], sem)]

    def wmc(c0, c1, sem):
        cs = pl.ds(c0 * D, (c1 - c0) * D)
        return [cp(wm_hbm.at[:, cs], wm_v.at[:, cs], sem)]

    def wc(i, up=True, down=True):
        r = []
        if up:
            r += [cp(wg_hbm.at[:, ds(i, FC)], wg_v.at[i], SEM_W + i),
                  cp(wu_hbm.at[:, ds(i, FC)], wu_v.at[i], SEM_W + i)]
        if down:
            r += [cp(wd_hbm.at[ds(i - 1, FC), :], wd_v.at[i - 1], SEM_W + i)]
        return r

    def step_group(s, with_kvs):
        return qc(s + 1, SEM_STEP + s) + (kvs(s + 3, SEM_STEP + s) if with_kvs else [])

    g_kvs0 = kvs(0, SEM_KVS0) + [cp(sk_hbm, sk_ref, SEM_KVS0), cp(d_hbm, d_ref, SEM_KVS0),
                                 cp(c_hbm, c_ref, SEM_KVS0)]
    g_m0 = qc(0, SEM_M0) + wmc(0, 3, SEM_M0)
    g_m1 = wmc(3, 5, SEM_M1)
    g_w0 = wc(0, down=False)
    g_q1 = qc(1, SEM_Q1)
    g_we = wc(NCH, up=False) + wmc(5, 6, SEM_W + NCH)
    g_1a = kvs(3, SEM_1A)
    g_1b = kvs(4, SEM_1B) + qc(2, SEM_1B)
    order = [g_kvs0, kvs(1, SEM_KVS1), kvs(2, SEM_KVS2), g_m0, g_m1, g_w0, g_q1]
    order += [wc(i) for i in range(1, NCH)] + [g_1a, g_we, g_1b]
    order += [step_group(s, s + 3 < NT) for s in range(2, NT - 1)]
    for g in order:
        for c_ in g:
            c_.start()

    def wait(g):
        for c_ in g:
            c_.wait()

    def out_copy(t):
        return cp(o_v.at[ds(t, TM), :], o_hbm.at[ds(t, TM), :], SEM_OUT)

    def out_col(t, n):
        cs = pl.ds(n * 128, 128)
        return cp(o_v.at[ds(t, TM), cs], o_hbm.at[ds(t, TM), cs], SEM_OUT)

    z0 = pl.semaphore_read(zsem)
    pred = jnp.full((8, 128), z0, jnp.int32) != 0
    h2p = h2p_ref.at[z0]

    def gate(x, tok):
        return x if tok is None else jnp.where(pred, tok, x)

    def fold(*xs):
        parts = []
        for x in xs:
            parts += [x[:, j:j + 128] for j in range(0, x.shape[1], 128)]
        while len(parts) > 1:
            parts = [jnp.maximum(parts[i], parts[i + 1]) if i + 1 < len(parts) else parts[i]
                     for i in range(0, len(parts), 2)]
        return parts[0]

    def rep(w):
        return jnp.tile(w, (NG, 1))

    def region(fn):
        pl.when(z0 == 0)(fn)

    rowid = lax.broadcasted_iota(jnp.int32, (8, 128), 0)
    masks = [None] + [rowid < m for m in range(1, 4)]

    def kv_stage(t, tok=None, serial=False):
        kt, vt = k_v.at[ds(t, TM)], v_v.at[ds(t, TM)]
        chain = tok is not None
        for (l0, l1) in [(0, 2), (2, 4), (4, 5)]:
            ls = slice(l0 * 128, l1 * 128)
            prev = None
            if not (st(t) and t == 0):
                pk = k_v[ds(t, TM, -8, 8, 8), ls].astype(f32)
                prev = [[None] + [pltpu.roll(pk[:, i * 128:(i + 1) * 128], m, 0) for m in range(1, 4)]
                        for i in range(l1 - l0)]
            for g in range(NG):
                kf = kt[8 * g:8 * g + 8, ls].astype(f32)
                vf = vt[8 * g:8 * g + 8, ls].astype(f32)
                cur, res = [], []
                for i in range(l1 - l0):
                    li = slice((l0 + i) * 128, (l0 + i + 1) * 128)
                    k0 = gate(kf[:, i * 128:(i + 1) * 128], tok)
                    rots = [None] + [pltpu.roll(k0, m, 0) for m in range(1, 4)]
                    ks = k0 * taps_ref[0, :, li]
                    for m in range(1, 4):
                        sh = jnp.where(masks[m], prev[i][m] if prev is not None else 0.0, rots[m])
                        ks = ks + sh * taps_ref[m, :, li]
                    res.append(ks * vf[:, i * 128:(i + 1) * 128])
                    cur.append(rots)
                    if serial:
                        tok = res[-1]
                prev = cur
                kv = res[0] if len(res) == 1 else jnp.concatenate(res, axis=1)
                kvb_ref[8 * g:8 * g + 8, ls] = kv.astype(bf16)
                if chain and not serial:
                    tok = fold(*res)
        return tok

    def dft_u(t, b):
        u = jnp.dot(fm_ref[...], kvb_ref[b * BLK:(b + 1) * BLK, :], preferred_element_type=f32)
        ur, ui = u[:BLK], u[BLK:]
        o = UOFF[b]
        u_ref[t, o:o + BLK] = ur + ui
        u_ref[t, o + BLK:o + 2 * BLK] = ur
        u_ref[t, o + 2 * BLK:o + 3 * BLK] = ui

    def dft_k(t, l0, l1):
        H = BLK // 2
        sblk = s_v[l0 * 128:l1 * 128, ds(t, TM)]
        rhs = jnp.concatenate([sblk[i * 128:(i + 1) * 128, b * BLK:(b + 1) * BLK]
                               for i in range(l1 - l0) for b in range(2)], axis=0)
        kr = lax.dot_general(fm_ref[...], rhs, (((1,), (1,)), ((), ())), preferred_element_type=f32)
        for i in range(l1 - l0):
            ls = slice((l0 + i) * 128, (l0 + i + 1) * 128)
            raws = [kr[:, (2 * i + b) * 128:(2 * i + b + 1) * 128] for b in range(2)]
            for b in range(2):
                kraw = raws[b]
                if st(t) and t == 0 and b == 0:
                    cr = kraw[:BLK] + d_ref[...].astype(f32).reshape(1, D)[:, ls]
                    di = kraw[BLK:]
                else:
                    kp = kprev_ref[:, ls] if b == 0 else raws[0]
                    cr = jnp.concatenate([kraw[0:H] - kp[BLK:BLK + H], kraw[H:BLK] + kp[BLK + H:]], axis=0)
                    di = jnp.concatenate([kraw[BLK:BLK + H] + kp[0:H], kraw[BLK + H:] - kp[H:BLK]], axis=0)
                o = KOFF[b]
                kk_ref[t, o:o + BLK, ls] = cr
                kk_ref[t, o + BLK:o + 2 * BLK, ls] = di - cr
                kk_ref[t, o + 2 * BLK:o + 3 * BLK, ls] = cr + di
            kprev_ref[:, ls] = raws[1]

    def dft_parts(t):
        return [lambda: dft_k(t, 0, 2), lambda: dft_u(t, 0), lambda: dft_k(t, 2, 5), lambda: dft_u(t, 1)]

    def dft_stage(t):
        for fn in dft_parts(t):
            fn()

    def inv_stage(t, slot=None):
        for b in range(2):
            y_ref[t % 2 if slot is None else slot, b * BLK:(b + 1) * BLK, :] = jnp.dot(
                gm_ref[...], z_ref[b], preferred_element_type=f32)

    def mac_stage(t, chain, tok=None, nlag=None, ov=0):
        g0 = g1 = tok
        if st(t):
            nlag = 2 * t + 2
            kidx = list(range(nlag // 2))
            uidx = [t - j for j in range(nlag // 2)]
        else:
            kidx = [jnp.minimum(j, t) for j in range(nlag // 2)]
            uidx = [jnp.where(t - j >= 0, t - j, ZPAIR) for j in range(nlag // 2)]
        for l in range(NL):
            ls = slice(l * 128, (l + 1) * 128)
            for r in range(BLK // 8):
                accs = []
                for p in range(3):
                    a0 = a1 = uc = None
                    o = p * BLK + r * 8
                    for j in range(nlag - 1, -1, -1):
                        kp = kk_ref[kidx[j // 2], KOFF[j % 2] + o:KOFF[j % 2] + o + 8, ls]
                        un = u_ref[uidx[j // 2], UOFF[1 - j % 2] + o:UOFF[1 - j % 2] + o + 8, ls]
                        t1 = kp * un
                        a1 = gate(t1, g1) if a1 is None else a1 + t1
                        if uc is not None:
                            t0 = kp * uc
                            a0 = gate(t0, g0) if a0 is None else a0 + t0
                        uc = un
                        if chain and p < 2 and j == min(ov, nlag - 2):
                            n0, n1 = a1, a0
                    accs.append((a0, a1))
                    if chain and p < 2:
                        g0, g1 = n0, n1
                outs = []
                for b in range(2):
                    re = accs[0][b] - accs[2][b]
                    im = accs[0][b] + accs[1][b]
                    z_ref[b, r * 8:r * 8 + 8, ls] = re.astype(bf16)
                    z_ref[b, BLK + r * 8:BLK + r * 8 + 8, ls] = im.astype(bf16)
                    outs.append(jnp.maximum(re, im))
                if chain:
                    g1, g0 = outs

    def fin_stage(t, par, lock, base=None, n=NG):
        qt = q_v.at[ds(t, TM)]
        ends = []
        for g in range(n):
            rr = pl.ds(8 * g, 8) if base is None else pl.ds(pl.multiple_of(base + 8 * g, 8), 8)
            x = qt[rr, :].astype(f32)
            xs = [x[:, i * 128:(i + 1) * 128] for i in range(NL)]
            xs[0] = gate(xs[0], ends[g - lock] if g >= lock else None)
            x = jnp.concatenate(xs, axis=1)
            pre = ((xs[0] + xs[1]) + (xs[2] + xs[3])) + xs[4]
            xc = x - jnp.sum(pre, axis=-1, keepdims=True) * (1.0 / D)
            var = jnp.mean(xc * xc, axis=-1, keepdims=True)
            hg = (xc * lax.rsqrt(var + EPS)) * mod_ref[1] + mod_ref[0]
            x1 = x + hg * y_ref[par, rr, :]
            xc = x1 - jnp.mean(x1, axis=-1, keepdims=True)
            var = jnp.mean(xc * xc, axis=-1, keepdims=True)
            h2 = (xc * lax.rsqrt(var + EPS)) * mod_ref[4] + mod_ref[3]
            x1_ref[par, rr, :] = x1
            h2_ref[rr, :] = h2.astype(bf16)
            ends.append(fold(h2))
        return fold(*ends[-lock:])

    def modrow(c0, c1):
        c = c_ref[...].astype(f32)
        sc = jnp.broadcast_to((c * jax.nn.sigmoid(c)).astype(bf16), (8, D))
        return jnp.dot(sc, wm_v[:, c0 * D:c1 * D], preferred_element_type=f32)

    def cat(ref, c0, c1, axis, cs=slice(None)):
        return pltpu.bitcast(jnp.concatenate([ref[z0 + c, :, cs] for c in range(c0, c1)], axis=axis), bf16)

    def ffn_up(c0, c1):
        h2 = pltpu.bitcast(h2p[...], bf16)
        g = jnp.dot(h2, cat(wgp, c0, c1, 1), preferred_element_type=f32)
        u = jnp.dot(h2, cat(wup, c0, c1, 1), preferred_element_type=f32)
        hh = pltpu.bitcast((jnp.maximum(g, 0.0) * u).astype(bf16), u32)
        for c in range(c0, c1):
            hhp_ref[z0 + c] = hh[:, (c - c0) * FC:(c - c0 + 1) * FC]

    def ffn_down(t, inter=(), at=NL):
        hh = cat(hhp_ref, 0, NCH, 1)
        cuts = [0] + [n for n in range(max(at, 1), NL)][:len(inter)] + [NL]
        inter = list(inter)
        for n0, n1 in zip(cuts[:-1], cuts[1:]):
            cs = slice(n0 * 128, n1 * 128)
            p = jnp.dot(hh, cat(wdp, 0, NCH, 0, cs), preferred_element_type=f32)
            o_v[ds(t, TM), cs] = (x1_ref[t % 2, :, cs] + rep(mod_ref[5, :, cs]) * p).astype(bf16)
            if inter:
                inter.pop(0)()
        for fn in inter:
            fn()

    def ffn0_up(i):
        h2 = pltpu.bitcast(h2p[...], bf16)
        wg, wu = wg_v[i], wu_v[i]
        wgp[i] = pltpu.bitcast(wg, u32)
        wup[i] = pltpu.bitcast(wu, u32)
        g = jnp.dot(h2, wg, preferred_element_type=f32)
        u = jnp.dot(h2, wu, preferred_element_type=f32)
        hhp_ref[i] = pltpu.bitcast((jnp.maximum(g, 0.0) * u).astype(bf16), u32)

    def ffn0_down(i):
        wd = wd_v[i]
        wdp[i] = pltpu.bitcast(wd, u32)
        return acc_ref[...] + jnp.dot(pltpu.bitcast(hhp_ref[i], bf16), wd, preferred_element_type=f32)

    def pack_h2():
        h2p[...] = pltpu.bitcast(h2_ref[...], u32)

    u_ref[ZPAIR] = jnp.zeros((PAIR_ROWS, D), f32)
    ri = lax.broadcasted_iota(jnp.int32, (BLK, BLK), 0)
    ci = lax.broadcasted_iota(jnp.int32, (BLK, BLK), 1)
    f2 = jnp.where(ri < BLK // 2, 4 * ri + 1, 4 * ri - (2 * BLK - 3))
    ang = ((f2 * ci) & (4 * BLK - 1)).astype(f32) * (np.pi / (2 * BLK))
    cs_, sn_ = jnp.cos(ang), -jnp.sin(ang)
    fm_ref[0:BLK, :] = cs_.astype(bf16)
    fm_ref[BLK:, :] = sn_.astype(bf16)
    gm_ref[:, 0:BLK] = (cs_.T * (1.0 / BLK)).astype(bf16)
    gm_ref[:, BLK:] = (sn_.T * (1.0 / BLK)).astype(bf16)
    wait(g_kvs0)
    skf = sk_ref[...].astype(f32)
    for m in range(4):
        taps_ref[m] = jnp.broadcast_to(skf[m:m + 1, :], (8, D))

    @region
    def _():
        kv_stage(0)
        dft_stage(0)
        mac_stage(0, False)
        inv_stage(0, 2)

    def body_p1(t, c):
        wait(kvs(t, SEM_KVS0 + t))
        kv_stage(t)
        dft_stage(t)
        return c

    def body_p2(t, c):
        mac_stage(t, False, nlag=6)
        inv_stage(t)
        return c
    lax.fori_loop(1, 3, body_p1, 0)
    lax.fori_loop(1, 3, body_p2, 0)
    wait(g_m0)

    @region
    def _():
        mod = modrow(0, 3)
        sa, ca, ga = [mod[:, i * D:(i + 1) * D] for i in range(3)]
        mod_ref[0] = ga * sa
        mod_ref[1] = ga * (1.0 + ca)
        x = q_v[0:TM, :].astype(f32)
        xc = x - jnp.mean(x, axis=-1, keepdims=True)
        var = jnp.mean(xc * xc, axis=-1, keepdims=True)
        hg = (xc * lax.rsqrt(var + EPS)) * rep(mod_ref[1]) + rep(mod_ref[0])
        x1 = x + hg * y_ref[2]
        xc = x1 - jnp.mean(x1, axis=-1, keepdims=True)
        var = jnp.mean(xc * xc, axis=-1, keepdims=True)
        x1_ref[2] = x1
        acc_ref[...] = xc * lax.rsqrt(var + EPS)
    wait(g_m1)

    @region
    def _():
        mod = modrow(3, 5)
        mod_ref[3] = mod[:, :D]
        mod_ref[4] = 1.0 + mod[:, D:]
        h2p[...] = pltpu.bitcast((acc_ref[...] * rep(mod_ref[4]) + rep(mod_ref[3])).astype(bf16), u32)
        acc_ref[...] = jnp.zeros((TM, D), f32)

    wait(g_w0)
    region(lambda: ffn0_up(0))
    wait(g_q1)

    def body_0(i, c):
        wait(wc(i))
        acc_ref[...] = ffn0_down(i - 1)
        fin_stage(1, 1, 4, base=jnp.minimum(i - 1, 3) * (TM // 4), n=NG // 4)
        ffn0_up(i)
        return c
    lax.fori_loop(1, NCH, body_0, 0)

    wait(g_1a)

    @region
    def _():
        pack_h2()
        kv_stage(3, jnp.zeros((8, 128), f32), serial=True)
        k0, u0, k1, u1 = dft_parts(3)
        for c, fn in enumerate([k0, k1, u0]):
            ffn_up(c, c + 1)
            fn()
        u1()
    wait(g_we)
    wait(g_1b)

    @region
    def _():
        gb = modrow(5, 6)
        mod_ref[5] = gb
        o_v[0:TM, :] = (x1_ref[2] + rep(gb) * ffn0_down(NCH - 1)).astype(bf16)
        mac_stage(3, True, kv_stage(4, fin_stage(2, 0, 6)), ov=2)
        ffn_up(3, NCH)
        ffn_down(1, dft_parts(4), 2)
        inv_stage(3)
    out_copy(0).start()

    def body_a(s, c):
        wait(step_group(s, True))
        out_copy(s - 1).start()
        pack_h2()
        mac_stage(s + 2, True, kv_stage(s + 3, fin_stage(s + 1, (s + 1) % 2, 6)), nlag=2 * NT - 2, ov=3)
        ffn_up(0, NCH)
        ffn_down(s, dft_parts(s + 3), 4)
        inv_stage(s + 2)
        return c
    lax.fori_loop(2, NT - 3, body_a, 0)

    wait(step_group(NT - 3, False))
    out_copy(NT - 4).start()

    @region
    def _():
        s = NT - 3
        pack_h2()
        mac_stage(s + 2, True, fin_stage(s + 1, (s + 1) % 2, 5), ov=3)
        ffn_up(0, NCH)
        ffn_down(s)
        inv_stage(s + 2)
    wait(step_group(NT - 2, False))
    out_copy(NT - 3).start()

    def body_b(s, c):
        pack_h2()
        fin_stage(jnp.minimum(s + 1, NT - 1), (s + 1) % 2, 3)
        ffn_up(0, NCH)
        ffn_down(s, [out_col(s, n).start for n in range(NL)], 1)
        return c
    lax.fori_loop(NT - 2, NT, body_b, 0)
    cp(o_v, o_hbm, SEM_OUT).wait()


@jax.jit
def pallas_adaLN_cond__ssm_conv_h3__glu_gated_reglu__prompt_kernel(
    A_q: jax.Array,
    A_k: jax.Array,
    A_v: jax.Array,
    A_shift_k: jax.Array,
    A_ssm_k: jax.Array,
    A_ssm_D: jax.Array,
    B_x: jax.Array,
    B_W_gate: jax.Array,
    B_W_up: jax.Array,
    B_W_down: jax.Array,
    c: jax.Array,
    w_mod: jax.Array,
):
    any_spec = pl.BlockSpec(memory_space=pl.ANY)
    V = pltpu.VMEM
    out = pl.pallas_call(
        _kernel,
        in_specs=[any_spec] * 11,
        out_specs=any_spec,
        out_shape=jax.ShapeDtypeStruct((S, D), bf16),
        scratch_shapes=[
            V((S, D), bf16), V((S, D), bf16), V((S, D), bf16), V((D, S), bf16), V((D, 6 * D), bf16),
            V((NCH, D, FC), bf16), V((NCH, D, FC), bf16), V((NCH, FC, D), bf16),
            V((NCH, D // 2, FC), u32), V((NCH, D // 2, FC), u32), V((NCH, FC // 2, D), u32),
            V((S, D), bf16), V((2 * BLK, BLK), bf16), V((BLK, 2 * BLK), bf16),
            V((NT + 1, PAIR_ROWS, D), f32), V((NT, PAIR_ROWS, D), f32),
            V((2 * BLK, D), f32), V((TM, D), bf16), V((2, 2 * BLK, D), bf16),
            V((3, TM, D), f32), V((TM, D), f32), V((TM, D), bf16), V((1, TM // 2, D), u32),
            V((NCH, TM // 2, FC), u32), V((3, TM, D), f32),
            V((4, 8, D), f32), V((6, 8, D), f32), V((4, D), bf16), V((D,), bf16), V((1, D), bf16),
            pltpu.SemaphoreType.DMA((NSEM,)), pltpu.SemaphoreType.REGULAR,
        ],
        compiler_params=pltpu.CompilerParams(vmem_limit_bytes=120 * 1024 * 1024),
    )(A_q.reshape(S, D), A_k.reshape(S, D), A_v.reshape(S, D), A_shift_k.T, A_ssm_k, A_ssm_D,
      B_W_gate, B_W_up, B_W_down, c, w_mod)
    return out.reshape(1, S, D)
```

```python
import numpy as np
import jax
import jax.numpy as jnp
from jax import lax
import jax.experimental.pallas as pl
import jax.experimental.pallas.tpu as pltpu

S, D, F = 2048, 640, 1536
BLK = 128
TM = 256
NT = S // TM
NL = D // 128
NG = TM // 8
FC = 256
NCH = F // FC
EPS = 1e-5
f32 = jnp.float32
bf16 = jnp.bfloat16
u32 = jnp.uint32

ZPAIR = NT
PAIR_ROWS = 800
UOFF = (8, 408)
KOFF = (0, 400)

(SEM_KVS0, SEM_KVS1, SEM_KVS2, SEM_M0, SEM_M1) = range(5)
SEM_W = 5
SEM_1A = SEM_W + NCH + 1
SEM_1B = SEM_1A + 1
SEM_STEP = SEM_1B + 1 - 2
SEM_OUT = SEM_STEP + NT - 1
NSEM = SEM_OUT + 1


def _kernel(q_hbm, k_hbm, v_hbm, sk_hbm, ssmk_hbm, d_hbm, wg_hbm, wu_hbm, wd_hbm, c_hbm, wm_hbm, o_hbm,
            q_v, k_v, v_v, s_v, wm_v, wg_v, wu_v, wd_v, wgp, wup, wdp, o_v, fm_ref, gm_ref,
            u_ref, kk_ref, kprev_ref, kvb_ref, z_ref, y_ref, acc_ref, h2_ref, h2p_ref, hhp_ref, x1_ref,
            taps_ref, mod_ref, sk_ref, d_ref, c_ref, sems, zsem):

    def st(x):
        return isinstance(x, int)

    def ds(i, n, off=0, size=None, al=None):
        r0 = i * n + off
        return pl.ds(r0 if st(i) else pl.multiple_of(r0, al or n), size or n)

    def cp(src, dst, sem):
        return pltpu.make_async_copy(src, dst, sems.at[sem])

    def kvs(t, sem):
        rs = ds(t, TM)
        return [cp(k_hbm.at[rs, :], k_v.at[rs, :], sem), cp(v_hbm.at[rs, :], v_v.at[rs, :], sem),
                cp(ssmk_hbm.at[:, rs], s_v.at[:, rs], sem)]

    def qc(t, sem):
        return [cp(q_hbm.at[ds(t, TM), :], q_v.at[ds(t, TM), :], sem)]

    def wmc(c0, c1, sem):
        cs = pl.ds(c0 * D, (c1 - c0) * D)
        return [cp(wm_hbm.at[:, cs], wm_v.at[:, cs], sem)]

    def wc(i, up=True, down=True):
        r = []
        if up:
            r += [cp(wg_hbm.at[:, ds(i, FC)], wg_v.at[i], SEM_W + i),
                  cp(wu_hbm.at[:, ds(i, FC)], wu_v.at[i], SEM_W + i)]
        if down:
            r += [cp(wd_hbm.at[ds(i - 1, FC), :], wd_v.at[i - 1], SEM_W + i)]
        if up and down:
            rs = ds(i + 3, TM // 4)
            r += [cp(q_hbm.at[rs, :], q_v.at[rs, :], SEM_W + i)]
        return r

    def step_group(s, with_kvs):
        return qc(s + 1, SEM_STEP + s) + (kvs(s + 3, SEM_STEP + s) if with_kvs else [])

    g_kvs0 = kvs(0, SEM_KVS0) + [cp(sk_hbm, sk_ref, SEM_KVS0), cp(d_hbm, d_ref, SEM_KVS0),
                                 cp(c_hbm, c_ref, SEM_KVS0)]
    g_m0 = qc(0, SEM_M0) + wmc(0, 3, SEM_M0)
    g_m1 = wmc(3, 5, SEM_M1)
    g_w0 = wc(0, down=False)
    g_we = wc(NCH, up=False) + wmc(5, 6, SEM_W + NCH)
    g_1a = kvs(3, SEM_1A)
    rq2 = pl.ds(2 * TM + TM // 4, TM - TM // 4)
    g_1b = kvs(4, SEM_1B) + [cp(q_hbm.at[rq2, :], q_v.at[rq2, :], SEM_1B)]
    order = [g_kvs0, kvs(1, SEM_KVS1), kvs(2, SEM_KVS2), g_m0, g_m1, g_w0]
    order += [wc(i) for i in range(1, NCH)] + [g_1a, g_we, g_1b]
    order += [step_group(s, s + 3 < NT) for s in range(2, NT - 1)]
    for g in order:
        for c_ in g:
            c_.start()

    def wait(g):
        for c_ in g:
            c_.wait()

    def out_copy(t):
        return cp(o_v.at[ds(t, TM), :], o_hbm.at[ds(t, TM), :], SEM_OUT)

    def out_col(t, n):
        cs = pl.ds(n * 128, 128)
        return cp(o_v.at[ds(t, TM), cs], o_hbm.at[ds(t, TM), cs], SEM_OUT)

    z0 = pl.semaphore_read(zsem)
    pred = jnp.full((8, 128), z0, jnp.int32) != 0
    h2p = h2p_ref.at[z0]

    def gate(x, tok):
        return x if tok is None else jnp.where(pred, tok, x)

    def fold(*xs):
        parts = []
        for x in xs:
            parts += [x[:, j:j + 128] for j in range(0, x.shape[1], 128)]
        while len(parts) > 1:
            parts = [jnp.maximum(parts[i], parts[i + 1]) if i + 1 < len(parts) else parts[i]
                     for i in range(0, len(parts), 2)]
        return parts[0]

    def rep(w):
        return jnp.tile(w, (NG, 1))

    def region(fn):
        pl.when(z0 == 0)(fn)

    rowid = lax.broadcasted_iota(jnp.int32, (8, 128), 0)
    masks = [None] + [rowid < m for m in range(1, 4)]

    def kv_stage(t, tok=None, serial=False):
        kt, vt = k_v.at[ds(t, TM)], v_v.at[ds(t, TM)]
        chain = tok is not None
        for (l0, l1) in [(0, 2), (2, 4), (4, 5)]:
            ls = slice(l0 * 128, l1 * 128)
            prev = None
            if not (st(t) and t == 0):
                pk = k_v[ds(t, TM, -8, 8, 8), ls].astype(f32)
                prev = [[None] + [pltpu.roll(pk[:, i * 128:(i + 1) * 128], m, 0) for m in range(1, 4)]
                        for i in range(l1 - l0)]
            for g in range(NG):
                kf = kt[8 * g:8 * g + 8, ls].astype(f32)
                vf = vt[8 * g:8 * g + 8, ls].astype(f32)
                cur, res = [], []
                for i in range(l1 - l0):
                    li = slice((l0 + i) * 128, (l0 + i + 1) * 128)
                    k0 = gate(kf[:, i * 128:(i + 1) * 128], tok)
                    rots = [None] + [pltpu.roll(k0, m, 0) for m in range(1, 4)]
                    ks = k0 * taps_ref[0, :, li]
                    for m in range(1, 4):
                        sh = jnp.where(masks[m], prev[i][m] if prev is not None else 0.0, rots[m])
                        ks = ks + sh * taps_ref[m, :, li]
                    res.append(ks * vf[:, i * 128:(i + 1) * 128])
                    cur.append(rots)
                    if serial:
                        tok = res[-1]
                prev = cur
                kv = res[0] if len(res) == 1 else jnp.concatenate(res, axis=1)
                kvb_ref[8 * g:8 * g + 8, ls] = kv.astype(bf16)
                if chain and not serial:
                    tok = fold(*res)
        return tok

    def dft_u(t, b):
        u = jnp.dot(fm_ref[...], kvb_ref[b * BLK:(b + 1) * BLK, :], preferred_element_type=f32)
        ur, ui = u[:BLK], u[BLK:]
        o = UOFF[b]
        u_ref[t, o:o + BLK] = ur + ui
        u_ref[t, o + BLK:o + 2 * BLK] = ur
        u_ref[t, o + 2 * BLK:o + 3 * BLK] = ui

    def dft_k(t, l0, l1):
        H = BLK // 2
        sblk = s_v[l0 * 128:l1 * 128, ds(t, TM)]
        rhs = jnp.concatenate([sblk[i * 128:(i + 1) * 128, b * BLK:(b + 1) * BLK]
                               for i in range(l1 - l0) for b in range(2)], axis=0)
        kr = lax.dot_general(fm_ref[...], rhs, (((1,), (1,)), ((), ())), preferred_element_type=f32)
        for i in range(l1 - l0):
            ls = slice((l0 + i) * 128, (l0 + i + 1) * 128)
            raws = [kr[:, (2 * i + b) * 128:(2 * i + b + 1) * 128] for b in range(2)]
            for b in range(2):
                kraw = raws[b]
                if st(t) and t == 0 and b == 0:
                    cr = kraw[:BLK] + d_ref[...].astype(f32).reshape(1, D)[:, ls]
                    di = kraw[BLK:]
                else:
                    kp = kprev_ref[:, ls] if b == 0 else raws[0]
                    cr = jnp.concatenate([kraw[0:H] - kp[BLK:BLK + H], kraw[H:BLK] + kp[BLK + H:]], axis=0)
                    di = jnp.concatenate([kraw[BLK:BLK + H] + kp[0:H], kraw[BLK + H:] - kp[H:BLK]], axis=0)
                o = KOFF[b]
                kk_ref[t, o:o + BLK, ls] = cr
                kk_ref[t, o + BLK:o + 2 * BLK, ls] = di - cr
                kk_ref[t, o + 2 * BLK:o + 3 * BLK, ls] = cr + di
            kprev_ref[:, ls] = raws[1]

    def dft_parts(t):
        return [lambda: dft_k(t, 0, 2), lambda: dft_u(t, 0), lambda: dft_k(t, 2, 5), lambda: dft_u(t, 1)]

    def dft_stage(t):
        for fn in dft_parts(t):
            fn()

    def inv_stage(t, slot=None):
        for b in range(2):
            y_ref[t % 2 if slot is None else slot, b * BLK:(b + 1) * BLK, :] = jnp.dot(
                gm_ref[...], z_ref[b], preferred_element_type=f32)

    def mac_stage(t, chain, tok=None, nlag=None, ov=0):
        g0 = g1 = tok
        if st(t):
            nlag = 2 * t + 2
            kidx = list(range(nlag // 2))
            uidx = [t - j for j in range(nlag // 2)]
        else:
            kidx = [jnp.minimum(j, t) for j in range(nlag // 2)]
            uidx = [jnp.where(t - j >= 0, t - j, ZPAIR) for j in range(nlag // 2)]
        for l in range(NL):
            ls = slice(l * 128, (l + 1) * 128)
            for r in range(BLK // 8):
                accs = []
                for p in range(3):
                    a0 = a1 = uc = None
                    o = p * BLK + r * 8
                    for j in range(nlag - 1, -1, -1):
                        kp = kk_ref[kidx[j // 2], KOFF[j % 2] + o:KOFF[j % 2] + o + 8, ls]
                        un = u_ref[uidx[j // 2], UOFF[1 - j % 2] + o:UOFF[1 - j % 2] + o + 8, ls]
                        t1 = kp * un
                        a1 = gate(t1, g1) if a1 is None else a1 + t1
                        if uc is not None:
                            t0 = kp * uc
                            a0 = gate(t0, g0) if a0 is None else a0 + t0
                        uc = un
                        if chain and p < 2 and j == min(ov, nlag - 2):
                            n0, n1 = a1, a0
                    accs.append((a0, a1))
                    if chain and p < 2:
                        g0, g1 = n0, n1
                outs = []
                for b in range(2):
                    re = accs[0][b] - accs[2][b]
                    im = accs[0][b] + accs[1][b]
                    z_ref[b, r * 8:r * 8 + 8, ls] = re.astype(bf16)
                    z_ref[b, BLK + r * 8:BLK + r * 8 + 8, ls] = im.astype(bf16)
                    outs.append(jnp.maximum(re, im))
                if chain:
                    g1, g0 = outs

    def fin_stage(t, par, lock, base=None, n=NG):
        qt = q_v.at[ds(t, TM)]
        ends = []
        for g in range(n):
            rr = pl.ds(8 * g, 8) if base is None else pl.ds(pl.multiple_of(base + 8 * g, 8), 8)
            x = qt[rr, :].astype(f32)
            xs = [x[:, i * 128:(i + 1) * 128] for i in range(NL)]
            xs[0] = gate(xs[0], ends[g - lock] if g >= lock else None)
            x = jnp.concatenate(xs, axis=1)
            pre = ((xs[0] + xs[1]) + (xs[2] + xs[3])) + xs[4]
            xc = x - jnp.sum(pre, axis=-1, keepdims=True) * (1.0 / D)
            var = jnp.mean(xc * xc, axis=-1, keepdims=True)
            hg = (xc * lax.rsqrt(var + EPS)) * mod_ref[1] + mod_ref[0]
            x1 = x + hg * y_ref[par, rr, :]
            xc = x1 - jnp.mean(x1, axis=-1, keepdims=True)
            var = jnp.mean(xc * xc, axis=-1, keepdims=True)
            h2 = (xc * lax.rsqrt(var + EPS)) * mod_ref[4] + mod_ref[3]
            x1_ref[par, rr, :] = x1
            h2_ref[rr, :] = h2.astype(bf16)
            ends.append(fold(h2))
        return fold(*ends[-lock:])

    def modrow(c0, c1):
        c = c_ref[...].astype(f32)
        sc = jnp.broadcast_to((c * jax.nn.sigmoid(c)).astype(bf16), (8, D))
        return jnp.dot(sc, wm_v[:, c0 * D:c1 * D], preferred_element_type=f32)

    def cat(ref, c0, c1, axis, cs=slice(None)):
        return pltpu.bitcast(jnp.concatenate([ref[z0 + c, :, cs] for c in range(c0, c1)], axis=axis), bf16)

    def ffn_up(c0, c1):
        h2 = pltpu.bitcast(h2p[...], bf16)
        g = jnp.dot(h2, cat(wgp, c0, c1, 1), preferred_element_type=f32)
        u = jnp.dot(h2, cat(wup, c0, c1, 1), preferred_element_type=f32)
        hh = pltpu.bitcast((jnp.maximum(g, 0.0) * u).astype(bf16), u32)
        for c in range(c0, c1):
            hhp_ref[z0 + c] = hh[:, (c - c0) * FC:(c - c0 + 1) * FC]

    def ffn_down(t, inter=(), at=NL):
        hh = cat(hhp_ref, 0, NCH, 1)
        cuts = [0] + [n for n in range(max(at, 1), NL)][:len(inter)] + [NL]
        inter = list(inter)
        for n0, n1 in zip(cuts[:-1], cuts[1:]):
            cs = slice(n0 * 128, n1 * 128)
            p = jnp.dot(hh, cat(wdp, 0, NCH, 0, cs), preferred_element_type=f32)
            o_v[ds(t, TM), cs] = (x1_ref[t % 2, :, cs] + rep(mod_ref[5, :, cs]) * p).astype(bf16)
            if inter:
                inter.pop(0)()
        for fn in inter:
            fn()

    def ffn0_up(i):
        h2 = pltpu.bitcast(h2p[...], bf16)
        wg, wu = wg_v[i], wu_v[i]
        wgp[i] = pltpu.bitcast(wg, u32)
        wup[i] = pltpu.bitcast(wu, u32)
        g = jnp.dot(h2, wg, preferred_element_type=f32)
        u = jnp.dot(h2, wu, preferred_element_type=f32)
        hhp_ref[i] = pltpu.bitcast((jnp.maximum(g, 0.0) * u).astype(bf16), u32)

    def ffn0_down(i):
        wd = wd_v[i]
        wdp[i] = pltpu.bitcast(wd, u32)
        return acc_ref[...] + jnp.dot(pltpu.bitcast(hhp_ref[i], bf16), wd, preferred_element_type=f32)

    def pack_h2():
        h2p[...] = pltpu.bitcast(h2_ref[...], u32)

    u_ref[ZPAIR] = jnp.zeros((PAIR_ROWS, D), f32)
    ri = lax.broadcasted_iota(jnp.int32, (BLK, BLK), 0)
    ci = lax.broadcasted_iota(jnp.int32, (BLK, BLK), 1)
    f2 = jnp.where(ri < BLK // 2, 4 * ri + 1, 4 * ri - (2 * BLK - 3))
    ang = ((f2 * ci) & (4 * BLK - 1)).astype(f32) * (np.pi / (2 * BLK))
    cs_, sn_ = jnp.cos(ang), -jnp.sin(ang)
    fm_ref[0:BLK, :] = cs_.astype(bf16)
    fm_ref[BLK:, :] = sn_.astype(bf16)
    gm_ref[:, 0:BLK] = (cs_.T * (1.0 / BLK)).astype(bf16)
    gm_ref[:, BLK:] = (sn_.T * (1.0 / BLK)).astype(bf16)
    wait(g_kvs0)
    skf = sk_ref[...].astype(f32)
    for m in range(4):
        taps_ref[m] = jnp.broadcast_to(skf[m:m + 1, :], (8, D))

    @region
    def _():
        kv_stage(0)
        dft_stage(0)
        mac_stage(0, False)
        inv_stage(0, 2)

    def body_p1(t, c):
        wait(kvs(t, SEM_KVS0 + t))
        kv_stage(t)
        dft_stage(t)
        return c

    def body_p2(t, c):
        mac_stage(t, False, nlag=6)
        inv_stage(t)
        return c
    lax.fori_loop(1, 3, body_p1, 0)
    lax.fori_loop(1, 3, body_p2, 0)
    wait(g_m0)

    @region
    def _():
        mod = modrow(0, 3)
        sa, ca, ga = [mod[:, i * D:(i + 1) * D] for i in range(3)]
        mod_ref[0] = ga * sa
        mod_ref[1] = ga * (1.0 + ca)
        x = q_v[0:TM, :].astype(f32)
        xc = x - jnp.mean(x, axis=-1, keepdims=True)
        var = jnp.mean(xc * xc, axis=-1, keepdims=True)
        hg = (xc * lax.rsqrt(var + EPS)) * rep(mod_ref[1]) + rep(mod_ref[0])
        x1 = x + hg * y_ref[2]
        xc = x1 - jnp.mean(x1, axis=-1, keepdims=True)
        var = jnp.mean(xc * xc, axis=-1, keepdims=True)
        x1_ref[2] = x1
        acc_ref[...] = xc * lax.rsqrt(var + EPS)
    wait(g_m1)

    @region
    def _():
        mod = modrow(3, 5)
        mod_ref[3] = mod[:, :D]
        mod_ref[4] = 1.0 + mod[:, D:]
        h2p[...] = pltpu.bitcast((acc_ref[...] * rep(mod_ref[4]) + rep(mod_ref[3])).astype(bf16), u32)
        acc_ref[...] = jnp.zeros((TM, D), f32)

    wait(g_w0)
    region(lambda: ffn0_up(0))

    def body_0(i, c):
        wait(wc(i))
        acc_ref[...] = ffn0_down(i - 1)
        fin_stage(1, 1, 4, base=jnp.minimum(i - 1, 3) * (TM // 4), n=NG // 4)
        ffn0_up(i)
        return c
    lax.fori_loop(1, NCH, body_0, 0)

    wait(g_1a)

    @region
    def _():
        pack_h2()
        kv_stage(3, jnp.zeros((8, 128), f32), serial=True)
        k0, u0, k1, u1 = dft_parts(3)
        for c, fn in enumerate([k0, k1, u0]):
            ffn_up(c, c + 1)
            fn()
        u1()
    wait(g_we)
    wait(g_1b)

    @region
    def _():
        gb = modrow(5, 6)
        mod_ref[5] = gb
        o_v[0:TM, :] = (x1_ref[2] + rep(gb) * ffn0_down(NCH - 1)).astype(bf16)
        mac_stage(3, True, kv_stage(4, fin_stage(2, 0, 6)), ov=2)
        ffn_up(3, NCH)
        ffn_down(1, dft_parts(4), 2)
        inv_stage(3)
    out_copy(0).start()

    def body_a(s, c):
        wait(step_group(s, True))
        out_copy(s - 1).start()
        pack_h2()
        mac_stage(s + 2, True, kv_stage(s + 3, fin_stage(s + 1, (s + 1) % 2, 6)), nlag=2 * NT - 2, ov=3)
        ffn_up(0, NCH)
        ffn_down(s, dft_parts(s + 3), 4)
        inv_stage(s + 2)
        return c
    lax.fori_loop(2, NT - 3, body_a, 0)

    wait(step_group(NT - 3, False))
    out_copy(NT - 4).start()

    @region
    def _():
        s = NT - 3
        pack_h2()
        mac_stage(s + 2, True, fin_stage(s + 1, (s + 1) % 2, 5), ov=3)
        ffn_up(0, NCH)
        ffn_down(s)
        inv_stage(s + 2)
    wait(step_group(NT - 2, False))
    out_copy(NT - 3).start()

    def body_b(s, c):
        pack_h2()
        fin_stage(jnp.minimum(s + 1, NT - 1), (s + 1) % 2, 3)
        ffn_up(0, NCH)
        ffn_down(s, [out_col(s, n).start for n in range(NL)], 1)
        return c
    lax.fori_loop(NT - 2, NT, body_b, 0)
    cp(o_v, o_hbm, SEM_OUT).wait()


@jax.jit
def pallas_adaLN_cond__ssm_conv_h3__glu_gated_reglu__prompt_kernel(
    A_q: jax.Array,
    A_k: jax.Array,
    A_v: jax.Array,
    A_shift_k: jax.Array,
    A_ssm_k: jax.Array,
    A_ssm_D: jax.Array,
    B_x: jax.Array,
    B_W_gate: jax.Array,
    B_W_up: jax.Array,
    B_W_down: jax.Array,
    c: jax.Array,
    w_mod: jax.Array,
):
    any_spec = pl.BlockSpec(memory_space=pl.ANY)
    V = pltpu.VMEM
    out = pl.pallas_call(
        _kernel,
        in_specs=[any_spec] * 11,
        out_specs=any_spec,
        out_shape=jax.ShapeDtypeStruct((S, D), bf16),
        scratch_shapes=[
            V((S, D), bf16), V((S, D), bf16), V((S, D), bf16), V((D, S), bf16), V((D, 6 * D), bf16),
            V((NCH, D, FC), bf16), V((NCH, D, FC), bf16), V((NCH, FC, D), bf16),
            V((NCH, D // 2, FC), u32), V((NCH, D // 2, FC), u32), V((NCH, FC // 2, D), u32),
            V((S, D), bf16), V((2 * BLK, BLK), bf16), V((BLK, 2 * BLK), bf16),
            V((NT + 1, PAIR_ROWS, D), f32), V((NT, PAIR_ROWS, D), f32),
            V((2 * BLK, D), f32), V((TM, D), bf16), V((2, 2 * BLK, D), bf16),
            V((3, TM, D), f32), V((TM, D), f32), V((TM, D), bf16), V((1, TM // 2, D), u32),
            V((NCH, TM // 2, FC), u32), V((3, TM, D), f32),
            V((4, 8, D), f32), V((6, 8, D), f32), V((4, D), bf16), V((D,), bf16), V((1, D), bf16),
            pltpu.SemaphoreType.DMA((NSEM,)), pltpu.SemaphoreType.REGULAR,
        ],
        compiler_params=pltpu.CompilerParams(vmem_limit_bytes=120 * 1024 * 1024),
    )(A_q.reshape(S, D), A_k.reshape(S, D), A_v.reshape(S, D), A_shift_k.T, A_ssm_k, A_ssm_D,
      B_W_gate, B_W_up, B_W_down, c, w_mod)
    return out.reshape(1, S, D)
```

```python
import numpy as np
import jax
import jax.numpy as jnp
from jax import lax
import jax.experimental.pallas as pl
import jax.experimental.pallas.tpu as pltpu

S, D, F = 2048, 640, 1536
BLK = 128
TM = 256
NT = S // TM
NL = D // 128
NG = TM // 8
FC = 256
NCH = F // FC
EPS = 1e-5
f32 = jnp.float32
bf16 = jnp.bfloat16
u32 = jnp.uint32

ZPAIR = NT
PAIR_ROWS = 800
UOFF = (8, 408)
KOFF = (0, 400)

(SEM_KVS0, SEM_KVS1, SEM_KVS2, SEM_M0, SEM_M1) = range(5)
SEM_W = 5
SEM_1A = SEM_W + NCH
SEM_1B = SEM_1A + 1
SEM_STEP = SEM_1B + 1 - 2
SEM_OUT = SEM_STEP + NT - 1
NSEM = SEM_OUT + 1


def _kernel(q_hbm, k_hbm, v_hbm, sk_hbm, ssmk_hbm, d_hbm, wg_hbm, wu_hbm, wd_hbm, c_hbm, wm_hbm, o_hbm,
            q_v, k_v, v_v, s_v, wm_v, wg_v, wu_v, wd_v, wgp, wup, wdp, o_v, fm_ref, gm_ref,
            u_ref, kk_ref, kprev_ref, kvb_ref, z_ref, y_ref, acc_ref, h2_ref, h2p_ref, hhp_ref, hh0_ref, x1_ref,
            taps_ref, mod_ref, sk_ref, d_ref, c_ref, sems, zsem):

    def st(x):
        return isinstance(x, int)

    def ds(i, n, off=0, size=None, al=None):
        r0 = i * n + off
        return pl.ds(r0 if st(i) else pl.multiple_of(r0, al or n), size or n)

    def cp(src, dst, sem):
        return pltpu.make_async_copy(src, dst, sems.at[sem])

    def kvs(t, sem):
        rs = ds(t, TM)
        return [cp(k_hbm.at[rs, :], k_v.at[rs, :], sem), cp(v_hbm.at[rs, :], v_v.at[rs, :], sem),
                cp(ssmk_hbm.at[:, rs], s_v.at[:, rs], sem)]

    def qc(t, sem):
        return [cp(q_hbm.at[ds(t, TM), :], q_v.at[ds(t, TM), :], sem)]

    def wmc(c0, c1, sem):
        cs = pl.ds(c0 * D, (c1 - c0) * D)
        return [cp(wm_hbm.at[:, cs], wm_v.at[:, cs], sem)]

    def wc(i):
        rs = ds(i + 4, TM // 4)
        return [cp(wg_hbm.at[:, ds(i, FC)], wg_v.at[i], SEM_W + i),
                cp(wu_hbm.at[:, ds(i, FC)], wu_v.at[i], SEM_W + i),
                cp(q_hbm.at[rs, :], q_v.at[rs, :], SEM_W + i)]

    def step_group(s, with_kvs):
        return qc(s + 1, SEM_STEP + s) + (kvs(s + 3, SEM_STEP + s) if with_kvs else [])

    g_kvs0 = kvs(0, SEM_KVS0) + [cp(sk_hbm, sk_ref, SEM_KVS0), cp(d_hbm, d_ref, SEM_KVS0),
                                 cp(c_hbm, c_ref, SEM_KVS0)]
    g_m0 = qc(0, SEM_M0) + wmc(0, 3, SEM_M0)
    g_m1 = wmc(3, 5, SEM_M1)
    g_1a = kvs(3, SEM_1A)
    rq2 = pl.ds(2 * TM + TM // 2, TM // 2)
    g_1b = ([cp(wd_hbm, wd_v, SEM_1B)] + wmc(5, 6, SEM_1B) + [cp(q_hbm.at[rq2, :], q_v.at[rq2, :], SEM_1B)]
            + kvs(4, SEM_1B))
    order = [g_kvs0, kvs(1, SEM_KVS1), kvs(2, SEM_KVS2), g_m0, g_m1] + [wc(i) for i in range(NCH)] + [g_1a, g_1b]
    order += [step_group(s, s + 3 < NT) for s in range(2, NT - 1)]
    for g in order:
        for c_ in g:
            c_.start()

    def wait(g):
        for c_ in g:
            c_.wait()

    def out_copy(t):
        return cp(o_v.at[ds(t, TM), :], o_hbm.at[ds(t, TM), :], SEM_OUT)

    def out_col(t, n):
        cs = pl.ds(n * 128, 128)
        return cp(o_v.at[ds(t, TM), cs], o_hbm.at[ds(t, TM), cs], SEM_OUT)

    z0 = pl.semaphore_read(zsem)
    pred = jnp.full((8, 128), z0, jnp.int32) != 0
    h2p = h2p_ref.at[z0]

    def gate(x, tok):
        return x if tok is None else jnp.where(pred, tok, x)

    def fold(*xs):
        parts = []
        for x in xs:
            parts += [x[:, j:j + 128] for j in range(0, x.shape[1], 128)]
        while len(parts) > 1:
            parts = [jnp.maximum(parts[i], parts[i + 1]) if i + 1 < len(parts) else parts[i]
                     for i in range(0, len(parts), 2)]
        return parts[0]

    def rep(w):
        return jnp.tile(w, (NG, 1))

    def region(fn):
        pl.when(z0 == 0)(fn)

    rowid = lax.broadcasted_iota(jnp.int32, (8, 128), 0)
    masks = [None] + [rowid < m for m in range(1, 4)]

    def kv_stage(t, tok=None, serial=False):
        kt, vt = k_v.at[ds(t, TM)], v_v.at[ds(t, TM)]
        chain = tok is not None
        for (l0, l1) in [(0, 2), (2, 4), (4, 5)]:
            ls = slice(l0 * 128, l1 * 128)
            prev = None
            if not (st(t) and t == 0):
                pk = k_v[ds(t, TM, -8, 8, 8), ls].astype(f32)
                prev = [[None] + [pltpu.roll(pk[:, i * 128:(i + 1) * 128], m, 0) for m in range(1, 4)]
                        for i in range(l1 - l0)]
            for g in range(NG):
                kf = kt[8 * g:8 * g + 8, ls].astype(f32)
                vf = vt[8 * g:8 * g + 8, ls].astype(f32)
                cur, res = [], []
                for i in range(l1 - l0):
                    li = slice((l0 + i) * 128, (l0 + i + 1) * 128)
                    k0 = gate(kf[:, i * 128:(i + 1) * 128], tok)
                    rots = [None] + [pltpu.roll(k0, m, 0) for m in range(1, 4)]
                    ks = k0 * taps_ref[0, :, li]
                    for m in range(1, 4):
                        sh = jnp.where(masks[m], prev[i][m] if prev is not None else 0.0, rots[m])
                        ks = ks + sh * taps_ref[m, :, li]
                    res.append(ks * vf[:, i * 128:(i + 1) * 128])
                    cur.append(rots)
                    if serial:
                        tok = res[-1]
                prev = cur
                kv = res[0] if len(res) == 1 else jnp.concatenate(res, axis=1)
                kvb_ref[8 * g:8 * g + 8, ls] = kv.astype(bf16)
                if chain and not serial:
                    tok = fold(*res)
        return tok

    def dft_u(t, b):
        u = jnp.dot(fm_ref[...], kvb_ref[b * BLK:(b + 1) * BLK, :], preferred_element_type=f32)
        ur, ui = u[:BLK], u[BLK:]
        o = UOFF[b]
        u_ref[t, o:o + BLK] = ur + ui
        u_ref[t, o + BLK:o + 2 * BLK] = ur
        u_ref[t, o + 2 * BLK:o + 3 * BLK] = ui

    def dft_k(t, l0, l1):
        H = BLK // 2
        sblk = s_v[l0 * 128:l1 * 128, ds(t, TM)]
        rhs = jnp.concatenate([sblk[i * 128:(i + 1) * 128, b * BLK:(b + 1) * BLK]
                               for i in range(l1 - l0) for b in range(2)], axis=0)
        kr = lax.dot_general(fm_ref[...], rhs, (((1,), (1,)), ((), ())), preferred_element_type=f32)
        for i in range(l1 - l0):
            ls = slice((l0 + i) * 128, (l0 + i + 1) * 128)
            raws = [kr[:, (2 * i + b) * 128:(2 * i + b + 1) * 128] for b in range(2)]
            for b in range(2):
                kraw = raws[b]
                if st(t) and t == 0 and b == 0:
                    cr = kraw[:BLK] + d_ref[...].astype(f32).reshape(1, D)[:, ls]
                    di = kraw[BLK:]
                else:
                    kp = kprev_ref[:, ls] if b == 0 else raws[0]
                    cr = jnp.concatenate([kraw[0:H] - kp[BLK:BLK + H], kraw[H:BLK] + kp[BLK + H:]], axis=0)
                    di = jnp.concatenate([kraw[BLK:BLK + H] + kp[0:H], kraw[BLK + H:] - kp[H:BLK]], axis=0)
                o = KOFF[b]
                kk_ref[t, o:o + BLK, ls] = cr
                kk_ref[t, o + BLK:o + 2 * BLK, ls] = di - cr
                kk_ref[t, o + 2 * BLK:o + 3 * BLK, ls] = cr + di
            kprev_ref[:, ls] = raws[1]

    def dft_parts(t):
        return [lambda: dft_k(t, 0, 2), lambda: dft_u(t, 0), lambda: dft_k(t, 2, 5), lambda: dft_u(t, 1)]

    def dft_stage(t):
        for fn in dft_parts(t):
            fn()

    def inv_stage(t, slot=None):
        for b in range(2):
            y_ref[t % 2 if slot is None else slot, b * BLK:(b + 1) * BLK, :] = jnp.dot(
                gm_ref[...], z_ref[b], preferred_element_type=f32)

    def mac_stage(t, chain, tok=None, nlag=None, ov=0):
        g0 = g1 = tok
        if st(t):
            nlag = 2 * t + 2
            kidx = list(range(nlag // 2))
            uidx = [t - j for j in range(nlag // 2)]
        else:
            kidx = [jnp.minimum(j, t) for j in range(nlag // 2)]
            uidx = [jnp.where(t - j >= 0, t - j, ZPAIR) for j in range(nlag // 2)]
        for l in range(NL):
            ls = slice(l * 128, (l + 1) * 128)
            for r in range(BLK // 8):
                accs = []
                for p in range(3):
                    a0 = a1 = uc = None
                    o = p * BLK + r * 8
                    for j in range(nlag - 1, -1, -1):
                        kp = kk_ref[kidx[j // 2], KOFF[j % 2] + o:KOFF[j % 2] + o + 8, ls]
                        un = u_ref[uidx[j // 2], UOFF[1 - j % 2] + o:UOFF[1 - j % 2] + o + 8, ls]
                        t1 = kp * un
                        a1 = gate(t1, g1) if a1 is None else a1 + t1
                        if uc is not None:
                            t0 = kp * uc
                            a0 = gate(t0, g0) if a0 is None else a0 + t0
                        uc = un
                        if chain and p < 2 and j == min(ov, nlag - 2):
                            n0, n1 = a1, a0
                    accs.append((a0, a1))
                    if chain and p < 2:
                        g0, g1 = n0, n1
                outs = []
                for b in range(2):
                    re = accs[0][b] - accs[2][b]
                    im = accs[0][b] + accs[1][b]
                    z_ref[b, r * 8:r * 8 + 8, ls] = re.astype(bf16)
                    z_ref[b, BLK + r * 8:BLK + r * 8 + 8, ls] = im.astype(bf16)
                    outs.append(jnp.maximum(re, im))
                if chain:
                    g1, g0 = outs

    def fin_stage(t, par, lock, base=None, n=NG):
        qt = q_v.at[ds(t, TM)]
        ends = []
        for g in range(n):
            rr = pl.ds(8 * g, 8) if base is None else pl.ds(pl.multiple_of(base + 8 * g, 8), 8)
            x = qt[rr, :].astype(f32)
            xs = [x[:, i * 128:(i + 1) * 128] for i in range(NL)]
            xs[0] = gate(xs[0], ends[g - lock] if g >= lock else None)
            x = jnp.concatenate(xs, axis=1)
            pre = ((xs[0] + xs[1]) + (xs[2] + xs[3])) + xs[4]
            xc = x - jnp.sum(pre, axis=-1, keepdims=True) * (1.0 / D)
            var = jnp.mean(xc * xc, axis=-1, keepdims=True)
            hg = (xc * lax.rsqrt(var + EPS)) * mod_ref[1] + mod_ref[0]
            x1 = x + hg * y_ref[par, rr, :]
            xc = x1 - jnp.mean(x1, axis=-1, keepdims=True)
            var = jnp.mean(xc * xc, axis=-1, keepdims=True)
            h2 = (xc * lax.rsqrt(var + EPS)) * mod_ref[4] + mod_ref[3]
            x1_ref[par, rr, :] = x1
            h2_ref[rr, :] = h2.astype(bf16)
            ends.append(fold(h2))
        return fold(*ends[-lock:])

    def modrow(c0, c1):
        c = c_ref[...].astype(f32)
        sc = jnp.broadcast_to((c * jax.nn.sigmoid(c)).astype(bf16), (8, D))
        return jnp.dot(sc, wm_v[:, c0 * D:c1 * D], preferred_element_type=f32)

    def cat(ref, c0, c1, axis, cs=slice(None)):
        return pltpu.bitcast(jnp.concatenate([ref[z0 + c, :, cs] for c in range(c0, c1)], axis=axis), bf16)

    def ffn_up(c0, c1):
        h2 = pltpu.bitcast(h2p[...], bf16)
        g = jnp.dot(h2, cat(wgp, c0, c1, 1), preferred_element_type=f32)
        u = jnp.dot(h2, cat(wup, c0, c1, 1), preferred_element_type=f32)
        hh = pltpu.bitcast((jnp.maximum(g, 0.0) * u).astype(bf16), u32)
        for c in range(c0, c1):
            hhp_ref[z0 + c] = hh[:, (c - c0) * FC:(c - c0 + 1) * FC]

    def ffn_down(t, inter=(), at=NL):
        hh = cat(hhp_ref, 0, NCH, 1)
        cuts = [0] + [n for n in range(max(at, 1), NL)][:len(inter)] + [NL]
        inter = list(inter)
        for n0, n1 in zip(cuts[:-1], cuts[1:]):
            cs = slice(n0 * 128, n1 * 128)
            p = jnp.dot(hh, cat(wdp, 0, NCH, 0, cs), preferred_element_type=f32)
            o_v[ds(t, TM), cs] = (x1_ref[t % 2, :, cs] + rep(mod_ref[5, :, cs]) * p).astype(bf16)
            if inter:
                inter.pop(0)()
        for fn in inter:
            fn()

    def ffn0_up(i):
        h2 = pltpu.bitcast(h2p[...], bf16)
        wg, wu = wg_v[i], wu_v[i]
        wgp[i] = pltpu.bitcast(wg, u32)
        wup[i] = pltpu.bitcast(wu, u32)
        g = jnp.dot(h2, wg, preferred_element_type=f32)
        u = jnp.dot(h2, wu, preferred_element_type=f32)
        hh0_ref[i] = pltpu.bitcast((jnp.maximum(g, 0.0) * u).astype(bf16), u32)

    def ffn01_down(inter, at):
        hh = jnp.concatenate([cat(hh0_ref, 0, NCH, 1), cat(hhp_ref, 0, NCH, 1)], axis=0)
        cuts = [0] + [n for n in range(max(at, 1), NL)][:len(inter)] + [NL]
        inter = list(inter)
        for n0, n1 in zip(cuts[:-1], cuts[1:]):
            cs = slice(n0 * 128, n1 * 128)
            wd = wd_v[:, cs]
            wdu = pltpu.bitcast(wd, u32)
            for c in range(NCH):
                wdp[z0 + c, :, cs] = wdu[c * FC // 2:(c + 1) * FC // 2]
            p = jnp.dot(hh, wd, preferred_element_type=f32)
            o_v[0:TM, cs] = (x1_ref[2, :, cs] + rep(mod_ref[5, :, cs]) * p[:TM]).astype(bf16)
            o_v[TM:2 * TM, cs] = (x1_ref[1, :, cs] + rep(mod_ref[5, :, cs]) * p[TM:]).astype(bf16)
            if inter:
                inter.pop(0)()
        for fn in inter:
            fn()

    def pack_h2():
        h2p[...] = pltpu.bitcast(h2_ref[...], u32)

    u_ref[ZPAIR] = jnp.zeros((PAIR_ROWS, D), f32)
    ri = lax.broadcasted_iota(jnp.int32, (BLK, BLK), 0)
    ci = lax.broadcasted_iota(jnp.int32, (BLK, BLK), 1)
    f2 = jnp.where(ri < BLK // 2, 4 * ri + 1, 4 * ri - (2 * BLK - 3))
    ang = ((f2 * ci) & (4 * BLK - 1)).astype(f32) * (np.pi / (2 * BLK))
    cs_, sn_ = jnp.cos(ang), -jnp.sin(ang)
    fm_ref[0:BLK, :] = cs_.astype(bf16)
    fm_ref[BLK:, :] = sn_.astype(bf16)
    gm_ref[:, 0:BLK] = (cs_.T * (1.0 / BLK)).astype(bf16)
    gm_ref[:, BLK:] = (sn_.T * (1.0 / BLK)).astype(bf16)
    wait(g_kvs0)
    skf = sk_ref[...].astype(f32)
    for m in range(4):
        taps_ref[m] = jnp.broadcast_to(skf[m:m + 1, :], (8, D))

    @region
    def _():
        kv_stage(0)
        dft_stage(0)
        mac_stage(0, False)
        inv_stage(0, 2)

    def body_p1(t, c):
        wait(kvs(t, SEM_KVS0 + t))
        kv_stage(t)
        dft_stage(t)
        return c

    def body_p2(t, c):
        mac_stage(t, False, nlag=6)
        inv_stage(t)
        return c
    lax.fori_loop(1, 3, body_p1, 0)
    lax.fori_loop(1, 3, body_p2, 0)
    wait(g_m0)

    @region
    def _():
        mod = modrow(0, 3)
        sa, ca, ga = [mod[:, i * D:(i + 1) * D] for i in range(3)]
        mod_ref[0] = ga * sa
        mod_ref[1] = ga * (1.0 + ca)
        x = q_v[0:TM, :].astype(f32)
        xc = x - jnp.mean(x, axis=-1, keepdims=True)
        var = jnp.mean(xc * xc, axis=-1, keepdims=True)
        hg = (xc * lax.rsqrt(var + EPS)) * rep(mod_ref[1]) + rep(mod_ref[0])
        x1 = x + hg * y_ref[2]
        xc = x1 - jnp.mean(x1, axis=-1, keepdims=True)
        var = jnp.mean(xc * xc, axis=-1, keepdims=True)
        x1_ref[2] = x1
        acc_ref[...] = xc * lax.rsqrt(var + EPS)
    wait(g_m1)

    @region
    def _():
        mod = modrow(3, 5)
        mod_ref[3] = mod[:, :D]
        mod_ref[4] = 1.0 + mod[:, D:]
        h2p[...] = pltpu.bitcast((acc_ref[...] * rep(mod_ref[4]) + rep(mod_ref[3])).astype(bf16), u32)

    def body_0(i, c):
        wait(wc(i))
        fin_stage(1, 1, 4, base=jnp.minimum(i, 3) * (TM // 4), n=NG // 4)
        ffn0_up(i)
        return c
    lax.fori_loop(0, NCH, body_0, 0)

    wait(g_1a)

    @region
    def _():
        pack_h2()
        kv_stage(3, jnp.zeros((8, 128), f32), serial=True)
        k0, u0, k1, u1 = dft_parts(3)
        for (c0, c1), fn in zip([(0, 1), (1, 2), (2, 4), (4, 5)], [k0, k1, u0, u1]):
            ffn_up(c0, c1)
            fn()
        ffn_up(5, 6)
    wait(g_1b)

    @region
    def _():
        mod_ref[5] = modrow(5, 6)
        mac_stage(3, True, kv_stage(4, fin_stage(2, 0, 6)), ov=2)
        ffn01_down(dft_parts(4), 3)
        inv_stage(3)
    out_copy(0).start()

    def body_a(s, c):
        wait(step_group(s, True))
        out_copy(s - 1).start()
        pack_h2()
        mac_stage(s + 2, True, kv_stage(s + 3, fin_stage(s + 1, (s + 1) % 2, 6)), nlag=2 * NT - 2, ov=3)
        ffn_up(0, NCH)
        ffn_down(s, dft_parts(s + 3), 4)
        inv_stage(s + 2)
        return c
    lax.fori_loop(2, NT - 3, body_a, 0)

    wait(step_group(NT - 3, False))
    out_copy(NT - 4).start()

    @region
    def _():
        s = NT - 3
        pack_h2()
        mac_stage(s + 2, True, fin_stage(s + 1, (s + 1) % 2, 5), ov=3)
        ffn_up(0, NCH)
        ffn_down(s)
        inv_stage(s + 2)
    wait(step_group(NT - 2, False))
    out_copy(NT - 3).start()

    def body_b(s, c):
        pack_h2()
        fin_stage(jnp.minimum(s + 1, NT - 1), (s + 1) % 2, 3)
        ffn_up(0, NCH)
        ffn_down(s, [out_col(s, n).start for n in range(NL)], 1)
        return c
    lax.fori_loop(NT - 2, NT, body_b, 0)
    cp(o_v, o_hbm, SEM_OUT).wait()


@jax.jit
def pallas_adaLN_cond__ssm_conv_h3__glu_gated_reglu__prompt_kernel(
    A_q: jax.Array,
    A_k: jax.Array,
    A_v: jax.Array,
    A_shift_k: jax.Array,
    A_ssm_k: jax.Array,
    A_ssm_D: jax.Array,
    B_x: jax.Array,
    B_W_gate: jax.Array,
    B_W_up: jax.Array,
    B_W_down: jax.Array,
    c: jax.Array,
    w_mod: jax.Array,
):
    any_spec = pl.BlockSpec(memory_space=pl.ANY)
    V = pltpu.VMEM
    out = pl.pallas_call(
        _kernel,
        in_specs=[any_spec] * 11,
        out_specs=any_spec,
        out_shape=jax.ShapeDtypeStruct((S, D), bf16),
        scratch_shapes=[
            V((S, D), bf16), V((S, D), bf16), V((S, D), bf16), V((D, S), bf16), V((D, 6 * D), bf16),
            V((NCH, D, FC), bf16), V((NCH, D, FC), bf16), V((F, D), bf16),
            V((NCH, D // 2, FC), u32), V((NCH, D // 2, FC), u32), V((NCH, FC // 2, D), u32),
            V((S, D), bf16), V((2 * BLK, BLK), bf16), V((BLK, 2 * BLK), bf16),
            V((NT + 1, PAIR_ROWS, D), f32), V((NT, PAIR_ROWS, D), f32),
            V((2 * BLK, D), f32), V((TM, D), bf16), V((2, 2 * BLK, D), bf16),
            V((3, TM, D), f32), V((TM, D), f32), V((TM, D), bf16), V((1, TM // 2, D), u32),
            V((NCH, TM // 2, FC), u32), V((NCH, TM // 2, FC), u32), V((3, TM, D), f32),
            V((4, 8, D), f32), V((6, 8, D), f32), V((4, D), bf16), V((D,), bf16), V((1, D), bf16),
            pltpu.SemaphoreType.DMA((NSEM,)), pltpu.SemaphoreType.REGULAR,
        ],
        compiler_params=pltpu.CompilerParams(vmem_limit_bytes=120 * 1024 * 1024),
    )(A_q.reshape(S, D), A_k.reshape(S, D), A_v.reshape(S, D), A_shift_k.T, A_ssm_k, A_ssm_D,
      B_W_gate, B_W_up, B_W_down, c, w_mod)
    return out.reshape(1, S, D)
```

```python
import numpy as np
import jax
import jax.numpy as jnp
from jax import lax
import jax.experimental.pallas as pl
import jax.experimental.pallas.tpu as pltpu

S, D, F = 2048, 640, 1536
BLK = 128
TM = 256
NT = S // TM
NL = D // 128
NG = TM // 8
FC = 256
NCH = F // FC
EPS = 1e-5
f32 = jnp.float32
bf16 = jnp.bfloat16
u32 = jnp.uint32

ZPAIR = NT
PAIR_ROWS = 800
UOFF = (8, 408)
KOFF = (0, 400)

(SEM_KVS0, SEM_KVS1, SEM_KVS2, SEM_M0, SEM_M1, SEM_KV0) = range(6)
SEM_W = 6
SEM_1A = SEM_W + NCH
SEM_1B = SEM_1A + 1
SEM_STEP = SEM_1B + 1 - 2
SEM_OUT = SEM_STEP + NT - 1
NSEM = SEM_OUT + 1


def _kernel(q_hbm, k_hbm, v_hbm, sk_hbm, ssmk_hbm, d_hbm, wg_hbm, wu_hbm, wd_hbm, c_hbm, wm_hbm, o_hbm,
            q_v, k_v, v_v, s_v, wm_v, wg_v, wu_v, wd_v, wgp, wup, wdp, o_v, fm_ref, gm_ref,
            u_ref, kk_ref, kprev_ref, kvb_ref, z_ref, y_ref, acc_ref, h2_ref, h2p_ref, hhp_ref, hh0_ref, x1_ref,
            taps_ref, mod_ref, sk_ref, d_ref, c_ref, sems, zsem):

    def st(x):
        return isinstance(x, int)

    def ds(i, n, off=0, size=None, al=None):
        r0 = i * n + off
        return pl.ds(r0 if st(i) else pl.multiple_of(r0, al or n), size or n)

    def cp(src, dst, sem):
        return pltpu.make_async_copy(src, dst, sems.at[sem])

    def kvs(t, sem):
        rs = ds(t, TM)
        return [cp(k_hbm.at[rs, :], k_v.at[rs, :], sem), cp(v_hbm.at[rs, :], v_v.at[rs, :], sem),
                cp(ssmk_hbm.at[:, rs], s_v.at[:, rs], sem)]

    def qc(t, sem):
        return [cp(q_hbm.at[ds(t, TM), :], q_v.at[ds(t, TM), :], sem)]

    def wmc(c0, c1, sem):
        cs = pl.ds(c0 * D, (c1 - c0) * D)
        return [cp(wm_hbm.at[:, cs], wm_v.at[:, cs], sem)]

    def wc(i):
        rs = ds(i + 4, TM // 4)
        return [cp(wg_hbm.at[:, ds(i, FC)], wg_v.at[i], SEM_W + i),
                cp(wu_hbm.at[:, ds(i, FC)], wu_v.at[i], SEM_W + i),
                cp(q_hbm.at[rs, :], q_v.at[rs, :], SEM_W + i)]

    def step_group(s, with_kvs):
        return qc(s + 1, SEM_STEP + s) + (kvs(s + 3, SEM_STEP + s) if with_kvs else [])

    r0 = ds(0, TM)
    g_kv0 = [cp(sk_hbm, sk_ref, SEM_KV0), cp(k_hbm.at[r0, :], k_v.at[r0, :], SEM_KV0),
             cp(v_hbm.at[r0, :], v_v.at[r0, :], SEM_KV0)]
    g_s0 = [cp(ssmk_hbm.at[:, r0], s_v.at[:, r0], SEM_KVS0), cp(d_hbm, d_ref, SEM_KVS0), cp(c_hbm, c_ref, SEM_KVS0)]
    g_m0 = qc(0, SEM_M0) + wmc(0, 3, SEM_M0)
    g_m1 = wmc(3, 5, SEM_M1)
    g_1a = kvs(3, SEM_1A)
    rq2 = pl.ds(2 * TM + TM // 2, TM // 2)
    g_1b = ([cp(wd_hbm, wd_v, SEM_1B)] + wmc(5, 6, SEM_1B) + [cp(q_hbm.at[rq2, :], q_v.at[rq2, :], SEM_1B)]
            + kvs(4, SEM_1B))
    order = [g_kv0, g_s0, kvs(1, SEM_KVS1), kvs(2, SEM_KVS2), g_m0, g_m1] + [wc(i) for i in range(NCH)] + [g_1a, g_1b]
    order += [step_group(s, s + 3 < NT) for s in range(2, NT - 1)]
    for g in order:
        for c_ in g:
            c_.start()

    def wait(g):
        for c_ in g:
            c_.wait()

    def out_copy(t):
        return cp(o_v.at[ds(t, TM), :], o_hbm.at[ds(t, TM), :], SEM_OUT)

    def out_col(t, n):
        cs = pl.ds(n * 128, 128)
        return cp(o_v.at[ds(t, TM), cs], o_hbm.at[ds(t, TM), cs], SEM_OUT)

    z0 = pl.semaphore_read(zsem)
    pred = jnp.full((8, 128), z0, jnp.int32) != 0
    h2p = h2p_ref.at[z0]

    def gate(x, tok):
        return x if tok is None else jnp.where(pred, tok, x)

    def fold(*xs):
        parts = []
        for x in xs:
            parts += [x[:, j:j + 128] for j in range(0, x.shape[1], 128)]
        while len(parts) > 1:
            parts = [jnp.maximum(parts[i], parts[i + 1]) if i + 1 < len(parts) else parts[i]
                     for i in range(0, len(parts), 2)]
        return parts[0]

    def rep(w):
        return jnp.tile(w, (NG, 1))

    def region(fn):
        pl.when(z0 == 0)(fn)

    rowid = lax.broadcasted_iota(jnp.int32, (8, 128), 0)
    masks = [None] + [rowid < m for m in range(1, 4)]

    def kv_stage(t, tok=None, serial=False):
        kt, vt = k_v.at[ds(t, TM)], v_v.at[ds(t, TM)]
        chain = tok is not None
        for (l0, l1) in [(0, 2), (2, 4), (4, 5)]:
            ls = slice(l0 * 128, l1 * 128)
            prev = None
            if not (st(t) and t == 0):
                pk = k_v[ds(t, TM, -8, 8, 8), ls].astype(f32)
                prev = [[None] + [pltpu.roll(pk[:, i * 128:(i + 1) * 128], m, 0) for m in range(1, 4)]
                        for i in range(l1 - l0)]
            for g in range(NG):
                kf = kt[8 * g:8 * g + 8, ls].astype(f32)
                vf = vt[8 * g:8 * g + 8, ls].astype(f32)
                cur, res = [], []
                for i in range(l1 - l0):
                    li = slice((l0 + i) * 128, (l0 + i + 1) * 128)
                    k0 = gate(kf[:, i * 128:(i + 1) * 128], tok)
                    rots = [None] + [pltpu.roll(k0, m, 0) for m in range(1, 4)]
                    ks = k0 * taps_ref[0, :, li]
                    for m in range(1, 4):
                        sh = jnp.where(masks[m], prev[i][m] if prev is not None else 0.0, rots[m])
                        ks = ks + sh * taps_ref[m, :, li]
                    res.append(ks * vf[:, i * 128:(i + 1) * 128])
                    cur.append(rots)
                    if serial:
                        tok = res[-1]
                prev = cur
                kv = res[0] if len(res) == 1 else jnp.concatenate(res, axis=1)
                kvb_ref[8 * g:8 * g + 8, ls] = kv.astype(bf16)
                if chain and not serial:
                    tok = fold(*res)
        return tok

    def dft_u(t, b):
        u = jnp.dot(fm_ref[...], kvb_ref[b * BLK:(b + 1) * BLK, :], preferred_element_type=f32)
        ur, ui = u[:BLK], u[BLK:]
        o = UOFF[b]
        u_ref[t, o:o + BLK] = ur + ui
        u_ref[t, o + BLK:o + 2 * BLK] = ur
        u_ref[t, o + 2 * BLK:o + 3 * BLK] = ui

    def dft_k(t, l0, l1):
        H = BLK // 2
        sblk = s_v[l0 * 128:l1 * 128, ds(t, TM)]
        rhs = jnp.concatenate([sblk[i * 128:(i + 1) * 128, b * BLK:(b + 1) * BLK]
                               for i in range(l1 - l0) for b in range(2)], axis=0)
        kr = lax.dot_general(fm_ref[...], rhs, (((1,), (1,)), ((), ())), preferred_element_type=f32)
        for i in range(l1 - l0):
            ls = slice((l0 + i) * 128, (l0 + i + 1) * 128)
            raws = [kr[:, (2 * i + b) * 128:(2 * i + b + 1) * 128] for b in range(2)]
            for b in range(2):
                kraw = raws[b]
                if st(t) and t == 0 and b == 0:
                    cr = kraw[:BLK] + d_ref[...].astype(f32).reshape(1, D)[:, ls]
                    di = kraw[BLK:]
                else:
                    kp = kprev_ref[:, ls] if b == 0 else raws[0]
                    cr = jnp.concatenate([kraw[0:H] - kp[BLK:BLK + H], kraw[H:BLK] + kp[BLK + H:]], axis=0)
                    di = jnp.concatenate([kraw[BLK:BLK + H] + kp[0:H], kraw[BLK + H:] - kp[H:BLK]], axis=0)
                o = KOFF[b]
                kk_ref[t, o:o + BLK, ls] = cr
                kk_ref[t, o + BLK:o + 2 * BLK, ls] = di - cr
                kk_ref[t, o + 2 * BLK:o + 3 * BLK, ls] = cr + di
            kprev_ref[:, ls] = raws[1]

    def dft_parts(t):
        return [lambda: dft_k(t, 0, 2), lambda: dft_u(t, 0), lambda: dft_k(t, 2, 5), lambda: dft_u(t, 1)]

    def dft_stage(t):
        for fn in dft_parts(t):
            fn()

    def inv_stage(t, slot=None):
        for b in range(2):
            y_ref[t % 2 if slot is None else slot, b * BLK:(b + 1) * BLK, :] = jnp.dot(
                gm_ref[...], z_ref[b], preferred_element_type=f32)

    def mac_stage(t, chain, tok=None, nlag=None, ov=0):
        g0 = g1 = tok
        if st(t):
            nlag = 2 * t + 2
            kidx = list(range(nlag // 2))
            uidx = [t - j for j in range(nlag // 2)]
        else:
            kidx = [jnp.minimum(j, t) for j in range(nlag // 2)]
            uidx = [jnp.where(t - j >= 0, t - j, ZPAIR) for j in range(nlag // 2)]
        for l in range(NL):
            ls = slice(l * 128, (l + 1) * 128)
            for r in range(BLK // 8):
                accs = []
                for p in range(3):
                    a0 = a1 = uc = None
                    o = p * BLK + r * 8
                    for j in range(nlag - 1, -1, -1):
                        kp = kk_ref[kidx[j // 2], KOFF[j % 2] + o:KOFF[j % 2] + o + 8, ls]
                        un = u_ref[uidx[j // 2], UOFF[1 - j % 2] + o:UOFF[1 - j % 2] + o + 8, ls]
                        t1 = kp * un
                        a1 = gate(t1, g1) if a1 is None else a1 + t1
                        if uc is not None:
                            t0 = kp * uc
                            a0 = gate(t0, g0) if a0 is None else a0 + t0
                        uc = un
                        if chain and p < 2 and j == min(ov, nlag - 2):
                            n0, n1 = a1, a0
                    accs.append((a0, a1))
                    if chain and p < 2:
                        g0, g1 = n0, n1
                outs = []
                for b in range(2):
                    re = accs[0][b] - accs[2][b]
                    im = accs[0][b] + accs[1][b]
                    z_ref[b, r * 8:r * 8 + 8, ls] = re.astype(bf16)
                    z_ref[b, BLK + r * 8:BLK + r * 8 + 8, ls] = im.astype(bf16)
                    outs.append(jnp.maximum(re, im))
                if chain:
                    g1, g0 = outs

    def fin_stage(t, par, lock, base=None, n=NG):
        qt = q_v.at[ds(t, TM)]
        ends = []
        for g in range(n):
            rr = pl.ds(8 * g, 8) if base is None else pl.ds(pl.multiple_of(base + 8 * g, 8), 8)
            x = qt[rr, :].astype(f32)
            xs = [x[:, i * 128:(i + 1) * 128] for i in range(NL)]
            xs[0] = gate(xs[0], ends[g - lock] if g >= lock else None)
            x = jnp.concatenate(xs, axis=1)
            pre = ((xs[0] + xs[1]) + (xs[2] + xs[3])) + xs[4]
            xc = x - jnp.sum(pre, axis=-1, keepdims=True) * (1.0 / D)
            var = jnp.mean(xc * xc, axis=-1, keepdims=True)
            hg = (xc * lax.rsqrt(var + EPS)) * mod_ref[1] + mod_ref[0]
            x1 = x + hg * y_ref[par, rr, :]
            xc = x1 - jnp.mean(x1, axis=-1, keepdims=True)
            var = jnp.mean(xc * xc, axis=-1, keepdims=True)
            h2 = (xc * lax.rsqrt(var + EPS)) * mod_ref[4] + mod_ref[3]
            x1_ref[par, rr, :] = x1
            h2_ref[rr, :] = h2.astype(bf16)
            ends.append(fold(h2))
        return fold(*ends[-lock:])

    def modrow(c0, c1):
        c = c_ref[...].astype(f32)
        sc = jnp.broadcast_to((c * jax.nn.sigmoid(c)).astype(bf16), (8, D))
        return jnp.dot(sc, wm_v[:, c0 * D:c1 * D], preferred_element_type=f32)

    def cat(ref, c0, c1, axis, cs=slice(None)):
        return pltpu.bitcast(jnp.concatenate([ref[z0 + c, :, cs] for c in range(c0, c1)], axis=axis), bf16)

    def ffn_up(c0, c1):
        h2 = pltpu.bitcast(h2p[...], bf16)
        g = jnp.dot(h2, cat(wgp, c0, c1, 1), preferred_element_type=f32)
        u = jnp.dot(h2, cat(wup, c0, c1, 1), preferred_element_type=f32)
        hh = pltpu.bitcast((jnp.maximum(g, 0.0) * u).astype(bf16), u32)
        for c in range(c0, c1):
            hhp_ref[z0 + c] = hh[:, (c - c0) * FC:(c - c0 + 1) * FC]

    def ffn_down(t, inter=(), at=NL):
        hh = cat(hhp_ref, 0, NCH, 1)
        cuts = [0] + [n for n in range(max(at, 1), NL)][:len(inter)] + [NL]
        inter = list(inter)
        for n0, n1 in zip(cuts[:-1], cuts[1:]):
            cs = slice(n0 * 128, n1 * 128)
            p = jnp.dot(hh, cat(wdp, 0, NCH, 0, cs), preferred_element_type=f32)
            o_v[ds(t, TM), cs] = (x1_ref[t % 2, :, cs] + rep(mod_ref[5, :, cs]) * p).astype(bf16)
            if inter:
                inter.pop(0)()
        for fn in inter:
            fn()

    def ffn0_up(i):
        h2 = pltpu.bitcast(h2p[...], bf16)
        wg, wu = wg_v[i], wu_v[i]
        wgp[i] = pltpu.bitcast(wg, u32)
        wup[i] = pltpu.bitcast(wu, u32)
        g = jnp.dot(h2, wg, preferred_element_type=f32)
        u = jnp.dot(h2, wu, preferred_element_type=f32)
        hh0_ref[i] = pltpu.bitcast((jnp.maximum(g, 0.0) * u).astype(bf16), u32)

    def ffn01_down(inter, at):
        hh = jnp.concatenate([cat(hh0_ref, 0, NCH, 1), cat(hhp_ref, 0, NCH, 1)], axis=0)
        cuts = [0] + [n for n in range(max(at, 1), NL)][:len(inter)] + [NL]
        inter = list(inter)
        for n0, n1 in zip(cuts[:-1], cuts[1:]):
            cs = slice(n0 * 128, n1 * 128)
            wd = wd_v[:, cs]
            wdu = pltpu.bitcast(wd, u32)
            for c in range(NCH):
                wdp[z0 + c, :, cs] = wdu[c * FC // 2:(c + 1) * FC // 2]
            p = jnp.dot(hh, wd, preferred_element_type=f32)
            o_v[0:TM, cs] = (x1_ref[2, :, cs] + rep(mod_ref[5, :, cs]) * p[:TM]).astype(bf16)
            o_v[TM:2 * TM, cs] = (x1_ref[1, :, cs] + rep(mod_ref[5, :, cs]) * p[TM:]).astype(bf16)
            if inter:
                inter.pop(0)()
        for fn in inter:
            fn()

    def pack_h2():
        h2p[...] = pltpu.bitcast(h2_ref[...], u32)

    def zero_rows(i, c):
        u_ref[ZPAIR, ds(i, 40, al=8), :] = jnp.zeros((40, D), f32)
        return c
    lax.fori_loop(0, PAIR_ROWS // 40, zero_rows, 0)
    ri = lax.broadcasted_iota(jnp.int32, (BLK, BLK), 0)
    ci = lax.broadcasted_iota(jnp.int32, (BLK, BLK), 1)
    f2 = jnp.where(ri < BLK // 2, 4 * ri + 1, 4 * ri - (2 * BLK - 3))
    ang = ((f2 * ci) & (4 * BLK - 1)).astype(f32) * (np.pi / (2 * BLK))
    cs_, sn_ = jnp.cos(ang), -jnp.sin(ang)
    fm_ref[0:BLK, :] = cs_.astype(bf16)
    fm_ref[BLK:, :] = sn_.astype(bf16)
    gm_ref[:, 0:BLK] = (cs_.T * (1.0 / BLK)).astype(bf16)
    gm_ref[:, BLK:] = (sn_.T * (1.0 / BLK)).astype(bf16)
    wait(g_kv0)
    skf = sk_ref[...].astype(f32)
    for m in range(4):
        taps_ref[m] = jnp.broadcast_to(skf[m:m + 1, :], (8, D))

    kv_stage(0)
    wait(g_s0)

    @region
    def _():
        dft_stage(0)
        mac_stage(0, False)
        inv_stage(0, 2)

    def body_p1(t, c):
        wait(kvs(t, SEM_KVS0 + t))
        kv_stage(t)
        dft_stage(t)
        return c

    def body_p2(t, c):
        mac_stage(t, True, nlag=6, ov=4)
        inv_stage(t)
        return c
    lax.fori_loop(1, 3, body_p1, 0)
    lax.fori_loop(1, 3, body_p2, 0)
    wait(g_m0)

    @region
    def _():
        mod = modrow(0, 3)
        sa, ca, ga = [mod[:, i * D:(i + 1) * D] for i in range(3)]
        mod_ref[0] = ga * sa
        mod_ref[1] = ga * (1.0 + ca)
        x = q_v[0:TM, :].astype(f32)
        xc = x - jnp.mean(x, axis=-1, keepdims=True)
        var = jnp.mean(xc * xc, axis=-1, keepdims=True)
        hg = (xc * lax.rsqrt(var + EPS)) * rep(mod_ref[1]) + rep(mod_ref[0])
        x1 = x + hg * y_ref[2]
        xc = x1 - jnp.mean(x1, axis=-1, keepdims=True)
        var = jnp.mean(xc * xc, axis=-1, keepdims=True)
        x1_ref[2] = x1
        acc_ref[...] = xc * lax.rsqrt(var + EPS)
    wait(g_m1)

    @region
    def _():
        mod = modrow(3, 5)
        mod_ref[3] = mod[:, :D]
        mod_ref[4] = 1.0 + mod[:, D:]
        h2p[...] = pltpu.bitcast((acc_ref[...] * rep(mod_ref[4]) + rep(mod_ref[3])).astype(bf16), u32)

    def body_0(i, c):
        wait(wc(i))
        fin_stage(1, 1, 4, base=jnp.minimum(i, 3) * (TM // 4), n=NG // 4)
        ffn0_up(i)
        return c
    lax.fori_loop(0, NCH, body_0, 0)

    wait(g_1a)

    @region
    def _():
        pack_h2()
        kv_stage(3, jnp.zeros((8, 128), f32), serial=True)
        k0, u0, k1, u1 = dft_parts(3)
        for (c0, c1), fn in zip([(0, 1), (1, 2), (2, 4), (4, 5)], [k0, k1, u0, u1]):
            ffn_up(c0, c1)
            fn()
        ffn_up(5, 6)
    wait(g_1b)

    @region
    def _():
        mod_ref[5] = modrow(5, 6)
        mac_stage(3, True, kv_stage(4, fin_stage(2, 0, 6)), ov=2)
        ffn01_down(dft_parts(4), 3)
        inv_stage(3)
    out_copy(0).start()

    def body_a(s, c):
        wait(step_group(s, True))
        out_copy(s - 1).start()
        pack_h2()
        mac_stage(s + 2, True, kv_stage(s + 3, fin_stage(s + 1, (s + 1) % 2, 6)), nlag=2 * NT - 2, ov=3)
        ffn_up(0, NCH)
        ffn_down(s, dft_parts(s + 3), 4)
        inv_stage(s + 2)
        return c
    lax.fori_loop(2, NT - 3, body_a, 0)

    wait(step_group(NT - 3, False))
    out_copy(NT - 4).start()

    @region
    def _():
        s = NT - 3
        pack_h2()
        mac_stage(s + 2, True, fin_stage(s + 1, (s + 1) % 2, 5), ov=3)
        ffn_up(0, NCH)
        ffn_down(s)
        inv_stage(s + 2)
    wait(step_group(NT - 2, False))
    out_copy(NT - 3).start()

    def body_b(s, c):
        pack_h2()
        fin_stage(jnp.minimum(s + 1, NT - 1), (s + 1) % 2, 3)
        ffn_up(0, NCH)
        ffn_down(s, [out_col(s, n).start for n in range(NL)], 1)
        return c
    lax.fori_loop(NT - 2, NT, body_b, 0)
    cp(o_v, o_hbm, SEM_OUT).wait()


@jax.jit
def pallas_adaLN_cond__ssm_conv_h3__glu_gated_reglu__prompt_kernel(
    A_q: jax.Array,
    A_k: jax.Array,
    A_v: jax.Array,
    A_shift_k: jax.Array,
    A_ssm_k: jax.Array,
    A_ssm_D: jax.Array,
    B_x: jax.Array,
    B_W_gate: jax.Array,
    B_W_up: jax.Array,
    B_W_down: jax.Array,
    c: jax.Array,
    w_mod: jax.Array,
):
    any_spec = pl.BlockSpec(memory_space=pl.ANY)
    V = pltpu.VMEM
    out = pl.pallas_call(
        _kernel,
        in_specs=[any_spec] * 11,
        out_specs=any_spec,
        out_shape=jax.ShapeDtypeStruct((S, D), bf16),
        scratch_shapes=[
            V((S, D), bf16), V((S, D), bf16), V((S, D), bf16), V((D, S), bf16), V((D, 6 * D), bf16),
            V((NCH, D, FC), bf16), V((NCH, D, FC), bf16), V((F, D), bf16),
            V((NCH, D // 2, FC), u32), V((NCH, D // 2, FC), u32), V((NCH, FC // 2, D), u32),
            V((S, D), bf16), V((2 * BLK, BLK), bf16), V((BLK, 2 * BLK), bf16),
            V((NT + 1, PAIR_ROWS, D), f32), V((NT, PAIR_ROWS, D), f32),
            V((2 * BLK, D), f32), V((TM, D), bf16), V((2, 2 * BLK, D), bf16),
            V((3, TM, D), f32), V((TM, D), f32), V((TM, D), bf16), V((1, TM // 2, D), u32),
            V((NCH, TM // 2, FC), u32), V((NCH, TM // 2, FC), u32), V((3, TM, D), f32),
            V((4, 8, D), f32), V((6, 8, D), f32), V((4, D), bf16), V((D,), bf16), V((1, D), bf16),
            pltpu.SemaphoreType.DMA((NSEM,)), pltpu.SemaphoreType.REGULAR,
        ],
        compiler_params=pltpu.CompilerParams(vmem_limit_bytes=120 * 1024 * 1024),
    )(A_q.reshape(S, D), A_k.reshape(S, D), A_v.reshape(S, D), A_shift_k.T, A_ssm_k, A_ssm_D,
      B_W_gate, B_W_up, B_W_down, c, w_mod)
    return out.reshape(1, S, D)
```

```python
import numpy as np
import jax
import jax.numpy as jnp
from jax import lax
import jax.experimental.pallas as pl
import jax.experimental.pallas.tpu as pltpu

S, D, F = 2048, 640, 1536
BLK = 128
TM = 256
NT = S // TM
NL = D // 128
NG = TM // 8
FC = 256
NCH = F // FC
EPS = 1e-5
f32 = jnp.float32
bf16 = jnp.bfloat16
u32 = jnp.uint32

ZPAIR = NT
PAIR_ROWS = 800
UOFF = (8, 408)
KOFF = (0, 400)

(SEM_KVS0, SEM_KVS1, SEM_KVS2, SEM_M0, SEM_M1, SEM_KV0) = range(6)
SEM_W = 6
SEM_1A = SEM_W + NCH
SEM_1B = SEM_1A + 1
SEM_REST = SEM_1B + 1
SEM_OUT = SEM_REST + 1
NSEM = SEM_OUT + 1


def _kernel(q_hbm, k_hbm, v_hbm, sk_hbm, ssmk_hbm, d_hbm, wg_hbm, wu_hbm, wd_hbm, c_hbm, wm_hbm, o_hbm,
            q_v, k_v, v_v, s_v, wm_v, wg_v, wu_v, wd_v, wgp, wup, wdp, o_v, fm_ref, gm_ref,
            u_ref, kk_ref, kprev_ref, kvb_ref, z_ref, y_ref, acc_ref, h2_ref, h2p_ref, hhp_ref, hh0_ref, x1_ref,
            taps_ref, mod_ref, sk_ref, d_ref, c_ref, sems, zsem):

    def st(x):
        return isinstance(x, int)

    def ds(i, n, off=0, size=None, al=None):
        r0 = i * n + off
        return pl.ds(r0 if st(i) else pl.multiple_of(r0, al or n), size or n)

    def cp(src, dst, sem):
        return pltpu.make_async_copy(src, dst, sems.at[sem])

    def kvs(t, sem):
        rs = ds(t, TM)
        return [cp(k_hbm.at[rs, :], k_v.at[rs, :], sem), cp(v_hbm.at[rs, :], v_v.at[rs, :], sem),
                cp(ssmk_hbm.at[:, rs], s_v.at[:, rs], sem)]

    def qc(t, sem):
        return [cp(q_hbm.at[ds(t, TM), :], q_v.at[ds(t, TM), :], sem)]

    def wmc(c0, c1, sem):
        cs = pl.ds(c0 * D, (c1 - c0) * D)
        return [cp(wm_hbm.at[:, cs], wm_v.at[:, cs], sem)]

    def wc(i):
        rs = ds(i + 4, TM // 4)
        return [cp(wg_hbm.at[:, ds(i, FC)], wg_v.at[i], SEM_W + i),
                cp(wu_hbm.at[:, ds(i, FC)], wu_v.at[i], SEM_W + i),
                cp(q_hbm.at[rs, :], q_v.at[rs, :], SEM_W + i)]

    r0 = ds(0, TM)
    g_kv0 = [cp(sk_hbm, sk_ref, SEM_KV0), cp(k_hbm.at[r0, :], k_v.at[r0, :], SEM_KV0),
             cp(v_hbm.at[r0, :], v_v.at[r0, :], SEM_KV0)]
    g_s0 = [cp(ssmk_hbm.at[:, r0], s_v.at[:, r0], SEM_KVS0), cp(d_hbm, d_ref, SEM_KVS0), cp(c_hbm, c_ref, SEM_KVS0)]
    g_m0 = qc(0, SEM_M0) + wmc(0, 3, SEM_M0)
    g_m1 = wmc(3, 5, SEM_M1)
    g_1a = kvs(3, SEM_1A)
    rq2 = pl.ds(2 * TM + TM // 2, TM // 2)
    g_1b = ([cp(wd_hbm, wd_v, SEM_1B)] + wmc(5, 6, SEM_1B) + [cp(q_hbm.at[rq2, :], q_v.at[rq2, :], SEM_1B)]
            + kvs(4, SEM_1B))
    order = [g_kv0, g_s0, kvs(1, SEM_KVS1), kvs(2, SEM_KVS2), g_m0, g_m1] + [wc(i) for i in range(NCH)] + [g_1a, g_1b]
    rq, rk = pl.ds(3 * TM, S - 3 * TM), pl.ds(5 * TM, S - 5 * TM)
    g_rest = [cp(q_hbm.at[rq, :], q_v.at[rq, :], SEM_REST), cp(k_hbm.at[rk, :], k_v.at[rk, :], SEM_REST),
              cp(v_hbm.at[rk, :], v_v.at[rk, :], SEM_REST), cp(ssmk_hbm.at[:, rk], s_v.at[:, rk], SEM_REST)]
    order += [g_rest]
    for g in order:
        for c_ in g:
            c_.start()

    def wait(g):
        for c_ in g:
            c_.wait()

    def out_copy(t):
        return cp(o_v.at[ds(t, TM), :], o_hbm.at[ds(t, TM), :], SEM_OUT)

    def out_col(t, n):
        cs = pl.ds(n * 128, 128)
        return cp(o_v.at[ds(t, TM), cs], o_hbm.at[ds(t, TM), cs], SEM_OUT)

    z0 = pl.semaphore_read(zsem)
    pred = jnp.full((8, 128), z0, jnp.int32) != 0
    h2p = h2p_ref.at[z0]

    def gate(x, tok):
        return x if tok is None else jnp.where(pred, tok, x)

    def fold(*xs):
        parts = []
        for x in xs:
            parts += [x[:, j:j + 128] for j in range(0, x.shape[1], 128)]
        while len(parts) > 1:
            parts = [jnp.maximum(parts[i], parts[i + 1]) if i + 1 < len(parts) else parts[i]
                     for i in range(0, len(parts), 2)]
        return parts[0]

    def rep(w):
        return jnp.tile(w, (NG, 1))

    def region(fn):
        pl.when(z0 == 0)(fn)

    rowid = lax.broadcasted_iota(jnp.int32, (8, 128), 0)
    masks = [None] + [rowid < m for m in range(1, 4)]

    def kv_stage(t, tok=None, serial=False):
        kt, vt = k_v.at[ds(t, TM)], v_v.at[ds(t, TM)]
        chain = tok is not None
        for (l0, l1) in [(0, 2), (2, 4), (4, 5)]:
            ls = slice(l0 * 128, l1 * 128)
            prev = None
            if not (st(t) and t == 0):
                pk = k_v[ds(t, TM, -8, 8, 8), ls].astype(f32)
                prev = [[None] + [pltpu.roll(pk[:, i * 128:(i + 1) * 128], m, 0) for m in range(1, 4)]
                        for i in range(l1 - l0)]
            for g in range(NG):
                kf = kt[8 * g:8 * g + 8, ls].astype(f32)
                vf = vt[8 * g:8 * g + 8, ls].astype(f32)
                cur, res = [], []
                for i in range(l1 - l0):
                    li = slice((l0 + i) * 128, (l0 + i + 1) * 128)
                    k0 = gate(kf[:, i * 128:(i + 1) * 128], tok)
                    rots = [None] + [pltpu.roll(k0, m, 0) for m in range(1, 4)]
                    ks = k0 * taps_ref[0, :, li]
                    for m in range(1, 4):
                        sh = jnp.where(masks[m], prev[i][m] if prev is not None else 0.0, rots[m])
                        ks = ks + sh * taps_ref[m, :, li]
                    res.append(ks * vf[:, i * 128:(i + 1) * 128])
                    cur.append(rots)
                    if serial:
                        tok = res[-1]
                prev = cur
                kv = res[0] if len(res) == 1 else jnp.concatenate(res, axis=1)
                kvb_ref[8 * g:8 * g + 8, ls] = kv.astype(bf16)
                if chain and not serial:
                    tok = fold(*res)
        return tok

    def dft_u(t, b):
        u = jnp.dot(fm_ref[...], kvb_ref[b * BLK:(b + 1) * BLK, :], preferred_element_type=f32)
        ur, ui = u[:BLK], u[BLK:]
        o = UOFF[b]
        u_ref[t, o:o + BLK] = ur + ui
        u_ref[t, o + BLK:o + 2 * BLK] = ur
        u_ref[t, o + 2 * BLK:o + 3 * BLK] = ui

    def dft_k(t, l0, l1):
        H = BLK // 2
        sblk = s_v[l0 * 128:l1 * 128, ds(t, TM)]
        rhs = jnp.concatenate([sblk[i * 128:(i + 1) * 128, b * BLK:(b + 1) * BLK]
                               for i in range(l1 - l0) for b in range(2)], axis=0)
        kr = lax.dot_general(fm_ref[...], rhs, (((1,), (1,)), ((), ())), preferred_element_type=f32)
        for i in range(l1 - l0):
            ls = slice((l0 + i) * 128, (l0 + i + 1) * 128)
            raws = [kr[:, (2 * i + b) * 128:(2 * i + b + 1) * 128] for b in range(2)]
            for b in range(2):
                kraw = raws[b]
                if st(t) and t == 0 and b == 0:
                    cr = kraw[:BLK] + d_ref[...].astype(f32).reshape(1, D)[:, ls]
                    di = kraw[BLK:]
                else:
                    kp = kprev_ref[:, ls] if b == 0 else raws[0]
                    cr = jnp.concatenate([kraw[0:H] - kp[BLK:BLK + H], kraw[H:BLK] + kp[BLK + H:]], axis=0)
                    di = jnp.concatenate([kraw[BLK:BLK + H] + kp[0:H], kraw[BLK + H:] - kp[H:BLK]], axis=0)
                o = KOFF[b]
                kk_ref[t, o:o + BLK, ls] = cr
                kk_ref[t, o + BLK:o + 2 * BLK, ls] = di - cr
                kk_ref[t, o + 2 * BLK:o + 3 * BLK, ls] = cr + di
            kprev_ref[:, ls] = raws[1]

    def dft_parts(t):
        return [lambda: dft_k(t, 0, 2), lambda: dft_u(t, 0), lambda: dft_k(t, 2, 5), lambda: dft_u(t, 1)]

    def dft_stage(t):
        for fn in dft_parts(t):
            fn()

    def inv_stage(t, slot=None):
        for b in range(2):
            y_ref[t % 2 if slot is None else slot, b * BLK:(b + 1) * BLK, :] = jnp.dot(
                gm_ref[...], z_ref[b], preferred_element_type=f32)

    def mac_stage(t, chain, tok=None, nlag=None, ov=0):
        g0 = g1 = tok
        if st(t):
            nlag = 2 * t + 2
            kidx = list(range(nlag // 2))
            uidx = [t - j for j in range(nlag // 2)]
        else:
            kidx = [jnp.minimum(j, t) for j in range(nlag // 2)]
            uidx = [jnp.where(t - j >= 0, t - j, ZPAIR) for j in range(nlag // 2)]
        for l in range(NL):
            ls = slice(l * 128, (l + 1) * 128)
            for r in range(BLK // 8):
                accs = []
                for p in range(3):
                    a0 = a1 = uc = None
                    o = p * BLK + r * 8
                    for j in range(nlag - 1, -1, -1):
                        kp = kk_ref[kidx[j // 2], KOFF[j % 2] + o:KOFF[j % 2] + o + 8, ls]
                        un = u_ref[uidx[j // 2], UOFF[1 - j % 2] + o:UOFF[1 - j % 2] + o + 8, ls]
                        t1 = kp * un
                        a1 = gate(t1, g1) if a1 is None else a1 + t1
                        if uc is not None:
                            t0 = kp * uc
                            a0 = gate(t0, g0) if a0 is None else a0 + t0
                        uc = un
                        if chain and p < 2 and j == min(ov, nlag - 2):
                            n0, n1 = a1, a0
                    accs.append((a0, a1))
                    if chain and p < 2:
                        g0, g1 = n0, n1
                outs = []
                for b in range(2):
                    re = accs[0][b] - accs[2][b]
                    im = accs[0][b] + accs[1][b]
                    z_ref[b, r * 8:r * 8 + 8, ls] = re.astype(bf16)
                    z_ref[b, BLK + r * 8:BLK + r * 8 + 8, ls] = im.astype(bf16)
                    outs.append(jnp.maximum(re, im))
                if chain:
                    g1, g0 = outs

    def fin_stage(t, par, lock, base=None, n=NG):
        qt = q_v.at[ds(t, TM)]
        ends = []
        for g in range(n):
            rr = pl.ds(8 * g, 8) if base is None else pl.ds(pl.multiple_of(base + 8 * g, 8), 8)
            x = qt[rr, :].astype(f32)
            xs = [x[:, i * 128:(i + 1) * 128] for i in range(NL)]
            xs[0] = gate(xs[0], ends[g - lock] if g >= lock else None)
            x = jnp.concatenate(xs, axis=1)
            pre = ((xs[0] + xs[1]) + (xs[2] + xs[3])) + xs[4]
            xc = x - jnp.sum(pre, axis=-1, keepdims=True) * (1.0 / D)
            var = jnp.mean(xc * xc, axis=-1, keepdims=True)
            hg = (xc * lax.rsqrt(var + EPS)) * mod_ref[1] + mod_ref[0]
            x1 = x + hg * y_ref[par, rr, :]
            xc = x1 - jnp.mean(x1, axis=-1, keepdims=True)
            var = jnp.mean(xc * xc, axis=-1, keepdims=True)
            h2 = (xc * lax.rsqrt(var + EPS)) * mod_ref[4] + mod_ref[3]
            x1_ref[par, rr, :] = x1
            h2_ref[rr, :] = h2.astype(bf16)
            ends.append(fold(h2))
        return fold(*ends[-lock:])

    def modrow(c0, c1):
        c = c_ref[...].astype(f32)
        sc = jnp.broadcast_to((c * jax.nn.sigmoid(c)).astype(bf16), (8, D))
        return jnp.dot(sc, wm_v[:, c0 * D:c1 * D], preferred_element_type=f32)

    def cat(ref, c0, c1, axis, cs=slice(None)):
        return pltpu.bitcast(jnp.concatenate([ref[z0 + c, :, cs] for c in range(c0, c1)], axis=axis), bf16)

    def ffn_up(c0, c1):
        h2 = pltpu.bitcast(h2p[...], bf16)
        g = jnp.dot(h2, cat(wgp, c0, c1, 1), preferred_element_type=f32)
        u = jnp.dot(h2, cat(wup, c0, c1, 1), preferred_element_type=f32)
        hh = pltpu.bitcast((jnp.maximum(g, 0.0) * u).astype(bf16), u32)
        for c in range(c0, c1):
            hhp_ref[z0 + c] = hh[:, (c - c0) * FC:(c - c0 + 1) * FC]

    def ffn_down(t, inter=(), at=NL):
        hh = cat(hhp_ref, 0, NCH, 1)
        cuts = [0] + [n for n in range(max(at, 1), NL)][:len(inter)] + [NL]
        inter = list(inter)
        for n0, n1 in zip(cuts[:-1], cuts[1:]):
            cs = slice(n0 * 128, n1 * 128)
            p = jnp.dot(hh, cat(wdp, 0, NCH, 0, cs), preferred_element_type=f32)
            o_v[ds(t, TM), cs] = (x1_ref[t % 2, :, cs] + rep(mod_ref[5, :, cs]) * p).astype(bf16)
            if inter:
                inter.pop(0)()
        for fn in inter:
            fn()

    def ffn0_up(i):
        h2 = pltpu.bitcast(h2p[...], bf16)
        wg, wu = wg_v[i], wu_v[i]
        wgp[i] = pltpu.bitcast(wg, u32)
        wup[i] = pltpu.bitcast(wu, u32)
        g = jnp.dot(h2, wg, preferred_element_type=f32)
        u = jnp.dot(h2, wu, preferred_element_type=f32)
        hh0_ref[i] = pltpu.bitcast((jnp.maximum(g, 0.0) * u).astype(bf16), u32)

    def ffn01_down(inter, at):
        hh = jnp.concatenate([cat(hh0_ref, 0, NCH, 1), cat(hhp_ref, 0, NCH, 1)], axis=0)
        cuts = [0] + [n for n in range(max(at, 1), NL)][:len(inter)] + [NL]
        inter = list(inter)
        for n0, n1 in zip(cuts[:-1], cuts[1:]):
            cs = slice(n0 * 128, n1 * 128)
            wd = wd_v[:, cs]
            wdu = pltpu.bitcast(wd, u32)
            for c in range(NCH):
                wdp[z0 + c, :, cs] = wdu[c * FC // 2:(c + 1) * FC // 2]
            p = jnp.dot(hh, wd, preferred_element_type=f32)
            o_v[0:TM, cs] = (x1_ref[2, :, cs] + rep(mod_ref[5, :, cs]) * p[:TM]).astype(bf16)
            o_v[TM:2 * TM, cs] = (x1_ref[1, :, cs] + rep(mod_ref[5, :, cs]) * p[TM:]).astype(bf16)
            if inter:
                inter.pop(0)()
        for fn in inter:
            fn()

    def pack_h2():
        h2p[...] = pltpu.bitcast(h2_ref[...], u32)

    def zero_rows(i, c):
        u_ref[ZPAIR, ds(i, 40, al=8), :] = jnp.zeros((40, D), f32)
        return c
    lax.fori_loop(0, PAIR_ROWS // 40, zero_rows, 0)
    ri = lax.broadcasted_iota(jnp.int32, (BLK, BLK), 0)
    ci = lax.broadcasted_iota(jnp.int32, (BLK, BLK), 1)
    f2 = jnp.where(ri < BLK // 2, 4 * ri + 1, 4 * ri - (2 * BLK - 3))
    ang = ((f2 * ci) & (4 * BLK - 1)).astype(f32) * (np.pi / (2 * BLK))
    cs_, sn_ = jnp.cos(ang), -jnp.sin(ang)
    fm_ref[0:BLK, :] = cs_.astype(bf16)
    fm_ref[BLK:, :] = sn_.astype(bf16)
    gm_ref[:, 0:BLK] = (cs_.T * (1.0 / BLK)).astype(bf16)
    gm_ref[:, BLK:] = (sn_.T * (1.0 / BLK)).astype(bf16)
    wait(g_kv0)
    skf = sk_ref[...].astype(f32)
    for m in range(4):
        taps_ref[m] = jnp.broadcast_to(skf[m:m + 1, :], (8, D))

    kv_stage(0)
    wait(g_s0)

    @region
    def _():
        dft_stage(0)
        mac_stage(0, False)
        inv_stage(0, 2)

    def body_p1(t, c):
        wait(kvs(t, SEM_KVS0 + t))
        kv_stage(t)
        dft_stage(t)
        return c

    def body_p2(t, c):
        mac_stage(t, True, nlag=6, ov=4)
        inv_stage(t)
        return c
    lax.fori_loop(1, 3, body_p1, 0)
    lax.fori_loop(1, 3, body_p2, 0)
    wait(g_m0)

    @region
    def _():
        mod = modrow(0, 3)
        sa, ca, ga = [mod[:, i * D:(i + 1) * D] for i in range(3)]
        mod_ref[0] = ga * sa
        mod_ref[1] = ga * (1.0 + ca)
        x = q_v[0:TM, :].astype(f32)
        xc = x - jnp.mean(x, axis=-1, keepdims=True)
        var = jnp.mean(xc * xc, axis=-1, keepdims=True)
        hg = (xc * lax.rsqrt(var + EPS)) * rep(mod_ref[1]) + rep(mod_ref[0])
        x1 = x + hg * y_ref[2]
        xc = x1 - jnp.mean(x1, axis=-1, keepdims=True)
        var = jnp.mean(xc * xc, axis=-1, keepdims=True)
        x1_ref[2] = x1
        acc_ref[...] = xc * lax.rsqrt(var + EPS)
    wait(g_m1)

    @region
    def _():
        mod = modrow(3, 5)
        mod_ref[3] = mod[:, :D]
        mod_ref[4] = 1.0 + mod[:, D:]
        h2p[...] = pltpu.bitcast((acc_ref[...] * rep(mod_ref[4]) + rep(mod_ref[3])).astype(bf16), u32)

    def body_0(i, c):
        wait(wc(i))
        fin_stage(1, 1, 4, base=jnp.minimum(i, 3) * (TM // 4), n=NG // 4)
        ffn0_up(i)
        return c
    lax.fori_loop(0, NCH, body_0, 0)

    wait(g_1a)

    @region
    def _():
        pack_h2()
        kv_stage(3, jnp.zeros((8, 128), f32), serial=True)
        k0, u0, k1, u1 = dft_parts(3)
        for (c0, c1), fn in zip([(0, 1), (1, 2), (2, 4), (4, 5)], [k0, k1, u0, u1]):
            ffn_up(c0, c1)
            fn()
        ffn_up(5, 6)
    wait(g_1b)

    @region
    def _():
        mod_ref[5] = modrow(5, 6)
        mac_stage(3, True, kv_stage(4, fin_stage(2, 0, 6)), ov=2)
        ffn01_down(dft_parts(4), 3)
        inv_stage(3)
    out_copy(0).start()

    def body_a(s, c):
        out_copy(s - 1).start()
        pack_h2()
        mac_stage(s + 2, True, kv_stage(s + 3, fin_stage(s + 1, (s + 1) % 2, 6)), nlag=2 * NT - 2, ov=3)
        ffn_up(0, NCH)
        ffn_down(s, dft_parts(s + 3), 4)
        inv_stage(s + 2)
        return c
    wait(g_rest)
    lax.fori_loop(2, NT - 3, body_a, 0)
    out_copy(NT - 4).start()

    @region
    def _():
        s = NT - 3
        pack_h2()
        mac_stage(s + 2, True, fin_stage(s + 1, (s + 1) % 2, 5), ov=3)
        ffn_up(0, NCH)
        ffn_down(s)
        inv_stage(s + 2)
    out_copy(NT - 3).start()

    def body_b(s, c):
        pack_h2()
        fin_stage(jnp.minimum(s + 1, NT - 1), (s + 1) % 2, 3)
        ffn_up(0, NCH)
        ffn_down(s, [out_col(s, n).start for n in range(NL)], 1)
        return c
    lax.fori_loop(NT - 2, NT, body_b, 0)
    cp(o_v, o_hbm, SEM_OUT).wait()


@jax.jit
def pallas_adaLN_cond__ssm_conv_h3__glu_gated_reglu__prompt_kernel(
    A_q: jax.Array,
    A_k: jax.Array,
    A_v: jax.Array,
    A_shift_k: jax.Array,
    A_ssm_k: jax.Array,
    A_ssm_D: jax.Array,
    B_x: jax.Array,
    B_W_gate: jax.Array,
    B_W_up: jax.Array,
    B_W_down: jax.Array,
    c: jax.Array,
    w_mod: jax.Array,
):
    any_spec = pl.BlockSpec(memory_space=pl.ANY)
    V = pltpu.VMEM
    out = pl.pallas_call(
        _kernel,
        in_specs=[any_spec] * 11,
        out_specs=any_spec,
        out_shape=jax.ShapeDtypeStruct((S, D), bf16),
        scratch_shapes=[
            V((S, D), bf16), V((S, D), bf16), V((S, D), bf16), V((D, S), bf16), V((D, 6 * D), bf16),
            V((NCH, D, FC), bf16), V((NCH, D, FC), bf16), V((F, D), bf16),
            V((NCH, D // 2, FC), u32), V((NCH, D // 2, FC), u32), V((NCH, FC // 2, D), u32),
            V((S, D), bf16), V((2 * BLK, BLK), bf16), V((BLK, 2 * BLK), bf16),
            V((NT + 1, PAIR_ROWS, D), f32), V((NT, PAIR_ROWS, D), f32),
            V((2 * BLK, D), f32), V((TM, D), bf16), V((2, 2 * BLK, D), bf16),
            V((3, TM, D), f32), V((TM, D), f32), V((TM, D), bf16), V((1, TM // 2, D), u32),
            V((NCH, TM // 2, FC), u32), V((NCH, TM // 2, FC), u32), V((3, TM, D), f32),
            V((4, 8, D), f32), V((6, 8, D), f32), V((4, D), bf16), V((D,), bf16), V((1, D), bf16),
            pltpu.SemaphoreType.DMA((NSEM,)), pltpu.SemaphoreType.REGULAR,
        ],
        compiler_params=pltpu.CompilerParams(vmem_limit_bytes=120 * 1024 * 1024),
    )(A_q.reshape(S, D), A_k.reshape(S, D), A_v.reshape(S, D), A_shift_k.T, A_ssm_k, A_ssm_D,
      B_W_gate, B_W_up, B_W_down, c, w_mod)
    return out.reshape(1, S, D)
```
